```python
import jax
import jax.numpy as jnp

def _softmax(x, axis=-1):
    return jax.nn.softmax(x, axis=axis)

def _gelu(x):
    return jax.nn.gelu(x, approximate=True)

def _silu(x):
    return jax.nn.silu(x)

def _sigmoid(x):
    return jax.nn.sigmoid(x)

def _layernorm(x, axis=-1, eps=1e-05):
    m = jnp.mean(x, axis=axis, keepdims=True)
    v = jnp.var(x, axis=axis, keepdims=True)
    return (x - m) / jnp.sqrt(v + eps)

def _scatter_add(tgt, idx, src, axis=0):
    return tgt.at[idx].add(src)

def _segment_sum(src, seg, n):
    return jax.ops.segment_sum(src, seg, n)

class _Rng:

    def __init__(self, key):
        self._k = key

    def _next(self):
        self._k, sub = jax.random.split(self._k)
        return sub

    def normal(self, shape):
        return jax.random.normal(self._next(), shape, dtype=jnp.bfloat16)

    def randint(self, lo, hi, shape):
        return jax.random.randint(self._next(), shape, lo, hi, dtype=jnp.int32)

    def uniform(self, shape, lo=0.0, hi=1.0):
        return jax.random.uniform(self._next(), shape, jnp.bfloat16, lo, hi)

    def permutation(self, n):
        return jax.random.permutation(self._next(), n)
kernel_name = 'parallel_sum__memory_aug_infini_attn__moe_arch_mod__prompt'

def setup_inputs():
    _rng = _Rng(jax.random.key(int.from_bytes(__import__("os").urandom(4), "little")))
    _w = lambda a: (lambda t: t.astype(jnp.bfloat16) if jnp.issubdtype(t.dtype, jnp.floating) else t)(jnp.asarray(a))

    def _A_setup():
        B, S, D, H = (1, 2048, 576, 32)
        N = 4
        L = max(1, S // N)
        sc = D ** (-0.5)
        return {'x': _w((lambda *s: _rng.normal(s) * 0.05)(B, N * L, D)), 'wq': _w((lambda *s: _rng.normal(s) * 0.05)(D, D) * sc), 'wk': _w((lambda *s: _rng.normal(s) * 0.05)(D, D) * sc), 'wv': _w((lambda *s: _rng.normal(s) * 0.05)(D, D) * sc), 'wo': _w((lambda *s: _rng.normal(s) * 0.05)(D, D) * sc), 'beta': _w((lambda *s: _rng.normal(s) * 0.05)(H))}
    _A_in = _A_setup()

    def _B_setup():
        B, S, D, F, C = (1, 2048, 576, 4608, 2)
        return {'x': _w((lambda *s: _rng.normal(s) * 0.05)(B, S, D)), 'w_r': _w((lambda *s: _rng.normal(s) * 0.05)(D)), 'w_gate': _w((lambda *s: _rng.normal(s) * 0.05)(D, F)), 'w_up': _w((lambda *s: _rng.normal(s) * 0.05)(D, F)), 'w_down': _w((lambda *s: _rng.normal(s) * 0.05)(F, D))}
    _B_in = _B_setup()
    return {'A_x': _A_in['x'], 'A_wq': _A_in['wq'], 'A_wk': _A_in['wk'], 'A_wv': _A_in['wv'], 'A_wo': _A_in['wo'], 'A_beta': _A_in['beta'], 'B_x': _B_in['x'], 'B_w_r': _B_in['w_r'], 'B_w_gate': _B_in['w_gate'], 'B_w_up': _B_in['w_up'], 'B_w_down': _B_in['w_down']}

def reference(A_x, A_wq, A_wk, A_wv, A_wo, A_beta, B_x, B_w_r, B_w_gate, B_w_up, B_w_down):

    def _A_ref(x, wq, wk, wv, wo, beta):
        B, S, D = x.shape
        H = 32
        Dh = D // H
        N = 4
        L = S // N
        q = (lambda x, *d: x.transpose(*d))((x @ wq).reshape(B, S, H, Dh), 0, 2, 1, 3).reshape(B, H, N, L, Dh)
        k = (lambda x, *d: x.transpose(*d))((x @ wk).reshape(B, S, H, Dh), 0, 2, 1, 3).reshape(B, H, N, L, Dh)
        v = (lambda x, *d: x.transpose(*d))((x @ wv).reshape(B, S, H, Dh), 0, 2, 1, 3).reshape(B, H, N, L, Dh)
        phi = lambda t: jnp.where(t > 0, t + 1.0, jnp.exp(t))
        scale = Dh ** (-0.5)
        ar = jnp.arange(L)
        mask = (lambda x, dt: x.astype(dt))(ar[:, None] < ar[None, :], x.dtype) * -1000000000.0
        g = _sigmoid(beta).reshape(1, H, 1, 1)
        M = jnp.einsum('bhd,bhe->bhde', q[:, :, 0, 0, :] * 0.0, q[:, :, 0, 0, :] * 0.0)
        z = q[:, :, 0, 0, :] * 0.0
        outs = []
        for s in range(N):
            qs, ks, vs = (q[:, :, s].copy(), k[:, :, s].copy(), v[:, :, s].copy())
            logits = jnp.einsum('bhqd,bhkd->bhqk', qs, ks) * scale + mask
            p = _softmax(logits, axis=-1)
            a_dot = jnp.einsum('bhqk,bhkd->bhqd', p, vs)
            pq = phi(qs)
            num = jnp.einsum('bhld,bhde->bhle', pq, M)
            den = jnp.einsum('bhld,bhd->bhl', pq, z)[..., None] + 1e-06
            a_mem = num / den
            o = g * a_mem + (1.0 - g) * a_dot
            outs.append(o)
            pk = phi(ks)
            M = M + jnp.einsum('bhld,bhle->bhde', pk, vs)
            z = z + jnp.einsum('bhld->bhd', pk)
        o = (lambda x, *d: x.transpose(*d))(jnp.stack(outs, 2).reshape(B, H, S, Dh), 0, 2, 1, 3).reshape(B, S, D)
        return o @ wo

    def _B_ref(x, w_r, w_gate, w_up, w_down):
        B, S, D = x.shape
        C = 2
        r = x @ w_r
        idx = jnp.argsort(-r, axis=-1)[:, :C]
        idx_e = jnp.repeat(idx.reshape(B, C, 1), D, axis=2)
        x_sel = jnp.take_along_axis(x, idx_e, axis=1)
        g = _silu(x_sel @ w_gate)
        u = x_sel @ w_up
        y = g * u @ w_down
        r_sel = _sigmoid(jnp.take_along_axis(r, idx, axis=1))
        y = y * r_sel.reshape(B, C, 1)
        b_off = (jnp.arange(B) * S).reshape(B, 1)
        flat_idx = (idx + b_off).reshape(B * C)
        zero = (x * 0.0).reshape(B * S, D)
        upd = _scatter_add(zero, flat_idx, y.reshape(B * C, D), axis=0)
        return x + upd.reshape(B, S, D)
    x = A_x
    xn = _layernorm(x, axis=-1)
    return x + _A_ref(xn, A_wq, A_wk, A_wv, A_wo, A_beta) + _B_ref(xn, B_w_r, B_w_gate, B_w_up, B_w_down)
```

```python
import jax
import jax.numpy as jnp
from jax import lax
import jax.experimental.pallas as pl
import jax.experimental.pallas.tpu as pltpu

BF = jnp.bfloat16
F32 = jnp.float32

SEQ, D, H, DH = 2048, 576, 32, 18
NSEG, L, FF = 4, 512, 4608
HPG = 7
NG = 5
GN = (7, 7, 7, 7, 4)
GW = (128, 128, 128, 128, 80)
GP = 592
ZR = (126, 126, 126, 126, 78)
QSCALE = (DH ** -0.5) * 1.4426950408889634
NT_DIMS = (((1,), (1,)), ((), ()))
MOE_CHUNK = 512
NEG = -1e30


def _dot(a, b):
    return jnp.dot(a, b, preferred_element_type=F32)


def _dot_nt(a, b):
    return lax.dot_general(a, b, NT_DIMS, preferred_element_type=F32)


def _iota(shape, dim):
    return lax.broadcasted_iota(jnp.int32, shape, dim)


def _phi(t):
    return jnp.where(t > 0, t + 1.0, jnp.exp(t))


def _sigmoid(t):
    return 1.0 / (1.0 + jnp.exp(-t))


def _div18(i):
    return (i * 57) >> 10


def _colsum(a):
    return jnp.sum(jnp.sum(a.reshape(a.shape[0] // 8, 8, a.shape[1]), axis=0), axis=0, keepdims=True)


def _kernel(x_hbm, wq_hbm, wk_hbm, wv_hbm, wo_hbm, beta_hbm, wr_hbm, wg_hbm, wu_hbm, wd_hbm,
            out_hbm,
            x_v, xn_v, res_v, wraw, w_t, wo_t, beta_v, wr_v, wr_b, wg_v, wu_v, wd_v,
            q_t, pq_t, v_t, k_n, pk_t, o_t, am_t, den_t, m_t, r_row, gate_t, out_v,
            sem_in, sem_out):

    def x_copy(s):
        return pltpu.make_async_copy(x_hbm.at[0, :, pl.ds(s * L, L)], x_v.at[:, pl.ds(s * L, L)],
                                     sem_in.at[s])

    def w_copy(i):
        src = (wq_hbm, wk_hbm, wv_hbm, wo_hbm)[i]
        return pltpu.make_async_copy(src, wraw.at[i], sem_in.at[4 + i])

    beta_copy = pltpu.make_async_copy(beta_hbm, beta_v, sem_in.at[8])
    wr_copy = pltpu.make_async_copy(wr_hbm, wr_v, sem_in.at[9])
    wg_copy = pltpu.make_async_copy(wg_hbm, wg_v, sem_in.at[10])
    wu_copy = pltpu.make_async_copy(wu_hbm, wu_v, sem_in.at[11])
    wd_copy = pltpu.make_async_copy(wd_hbm, wd_v, sem_in.at[12])

    def out_copy(s):
        return pltpu.make_async_copy(out_v.at[:, pl.ds(s * L, L)], out_hbm.at[0, :, pl.ds(s * L, L)],
                                     sem_out.at[s])

    x_copy(0).start()
    w_copy(0).start()
    wr_copy.start()
    beta_copy.start()
    w_copy(1).start()
    w_copy(2).start()
    for s in range(1, NSEG):
        x_copy(s).start()
    w_copy(3).start()
    wg_copy.start()
    wu_copy.start()
    wd_copy.start()

    def layernorm(s, tt):
        cols = slice(s * L + tt * 128, s * L + (tt + 1) * 128)
        x = x_v[:, cols].astype(F32)
        mean = _colsum(x) * (1.0 / D)
        xc = x - mean
        var = _colsum(xc * xc) * (1.0 / D)
        xnb = (xc * lax.rsqrt(var + 1e-5)).astype(BF)
        xn_v[:, cols] = xnb
        xnf = xnb.astype(F32)
        res_v[:, cols] = x + xnf
        r = _colsum(xnf * wr_b[...])
        r_row[:, cols] = r.astype(BF).astype(F32)

    def prep_wr():
        wr = wr_v[...].astype(F32).reshape(1, D)
        wr_b[...] = jnp.broadcast_to(wr, (128, D)).T

    def prep_wt(g, which):
        n = DH * GN[g]
        r0 = 384 * g + which * GW[g]
        w_t[r0:r0 + n, :] = wraw[which, :, 126 * g:126 * g + n].T
        w_t[r0 + n:r0 + GW[g], :] = jnp.zeros((GW[g] - n, D), BF)

    def prep_wo(g):
        n = DH * GN[g]
        wo_t[:, 128 * g:128 * g + n] = wraw[3, 126 * g:126 * g + n, :].T
        wo_t[:, 128 * g + n:128 * g + GW[g]] = jnp.zeros((D, GW[g] - n), BF)

    def prep_gates():
        b = beta_v[...].astype(F32).reshape(1, H)
        sig = jnp.concatenate([_sigmoid(b), jnp.zeros((1, 128 - H), F32)], axis=1)
        gate_t[...] = jnp.broadcast_to(sig, (128, 128)).T

    def init_pads():
        for s in range(NSEG):
            for g in range(NG):
                n = DH * GN[g]
                o_t[s, 128 * g + n:128 * g + GW[g], :] = jnp.zeros((GW[g] - n, L), BF)

    def proj_qkv(s, tt, g):
        w = GW[g]
        rows = slice(128 * g, 128 * g + w)
        cols = slice(tt * 128, (tt + 1) * 128)
        r = _dot(w_t[384 * g:384 * g + 3 * w, :], xn_v[:, s * L + tt * 128:s * L + (tt + 1) * 128])
        q, k, v = r[:w], r[w:2 * w], r[2 * w:]
        q_t[s, rows, cols] = (q * QSCALE).astype(BF)
        if s > 0:
            pq_t[s - 1, rows, cols] = _phi(q).astype(BF)
        k_n[s, cols, rows] = k.astype(BF).T
        if s < NSEG - 1:
            pk_t[s, rows, cols] = _phi(k).astype(BF)
        v = jnp.where(_iota((w, 128), 0) == ZR[g], 1.0, v)
        v_t[s, rows, cols] = v.astype(BF)

    def mem_update(s, g):
        w = GW[g]
        rows = slice(128 * g, 128 * g + w)
        r = _dot_nt(v_t[s, rows, :], pk_t[s, rows, :])
        rr, cc = _iota((w, w), 0), _iota((w, w), 1)
        keep = (cc < DH * GN[g]) & ((_div18(rr) == _div18(cc)) | (rr == ZR[g]))
        r = jnp.where(keep, r, 0.0)
        if s > 0:
            r = r + m_t[g, :w, :w]
        m_t[g, :w, :w] = r

    def mem_read(s, g):
        w = GW[g]
        rows = slice(128 * g, 128 * g + w)
        m = m_t[g, :w, :w]
        z = m[ZR[g]:ZR[g] + 1, :]
        zrows = jnp.where(_iota((16, w), 0) == _div18(_iota((16, w), 1)), z, 0.0)
        lhs = jnp.concatenate([m, zrows], axis=0).astype(BF)
        r = _dot(lhs, pq_t[s - 1, rows, :])
        am_t[s - 1, rows, :] = r[:w]
        den_t[s - 1, 16 * g:16 * (g + 1), :] = r[w:]

    def proj_out(s, tt, fb):
        f0 = 192 * fb
        f1 = f0 + 192
        cols = slice(s * L + tt * 128, s * L + (tt + 1) * 128)
        p = _dot(wo_t[f0:f1, :], o_t[s, :, tt * 128:(tt + 1) * 128])
        out_v[f0:f1, cols] = (p + res_v[f0:f1, cols]).astype(BF)

    moe = {}

    def moe_select():
        r = r_row[...]
        io = _iota((1, SEQ), 1)
        m1 = jnp.max(r)
        i1 = jnp.min(jnp.where(r == m1, io, SEQ - 1))
        r2 = jnp.where(io == i1, -jnp.inf, r)
        m2 = jnp.max(r2)
        i2 = jnp.min(jnp.where((r2 == m2) & (io != i1), io, SEQ - 1))
        rows = []
        for i in (i1, i2):
            blk = pl.multiple_of((i // 128) * 128, 128)
            xb = xn_v[:, pl.ds(blk, 128)].T.astype(F32)
            rows.append(jnp.sum(jnp.where(_iota((128, D), 0) == i % 128, xb, 0.0), axis=0, keepdims=True))
        rr = _iota((16, D), 0)
        xs = jnp.where(rr == 0, rows[0], jnp.where(rr == 1, rows[1], 0.0))
        moe["x"] = xs.astype(BF)
        moe["w"] = _sigmoid(jnp.where(_iota((16, 1), 0) == 0, m1, m2))
        for s in range(NSEG):
            tok = _iota((2, L), 1) + s * L
            sel = jnp.where(_iota((2, L), 0) == 0, i1, i2)
            o_t[s, 126:128, :] = jnp.where(tok == sel, 1.0, 0.0).astype(BF)

    def moe_chunk(c):
        cs = slice(c * MOE_CHUNK, (c + 1) * MOE_CHUNK)
        g = _dot(moe["x"], wg_v[:, cs])
        u = _dot(moe["x"], wu_v[:, cs])
        h = (g * _sigmoid(g) * u).astype(BF)
        y = _dot_nt(h, wd_v[:, cs])
        moe["y"] = y if c == 0 else moe["y"] + y

    def moe_finish():
        y = moe["y"] * moe["w"]
        rr = _iota((128, D), 0)
        ypad = jnp.where(rr == 126, y[0:1], jnp.where(rr == 127, y[1:2], 0.0))
        cur = wo_t[:, 0:128].astype(F32)
        wo_t[:, 0:128] = jnp.where(_iota((D, 128), 1) >= 126, ypad.T, cur).astype(BF)

    causal = _iota((128, 128), 0) <= _iota((128, 128), 1)
    row128 = _iota((128, 128), 0)
    wrow = _iota((32, 128), 0)

    def make_attention(s):
        st, pt, mx = {}, {}, {}

        def qk(h):
            g, j = divmod(h, HPG)
            w = GW[g]
            for i in range(4):
                wq = q_t[s, 128 * g:128 * g + w, 128 * i:128 * (i + 1)]
                rowi = row128[:w]
                wq = jnp.where((rowi >= DH * j) & (rowi < DH * j + DH), wq, jnp.zeros_like(wq))
                m = None
                for kt in range(i + 1):
                    d = _dot(k_n[s, 128 * kt:128 * (kt + 1), 128 * g:128 * g + w], wq)
                    if kt == i:
                        d = jnp.where(causal, d, NEG)
                    st[(h, i, kt)] = d
                    pm = jnp.max(d.reshape(16, 8, 128), axis=0)
                    m = pm if m is None else jnp.maximum(m, pm)
                mx[(h, i)] = jnp.max(m, axis=0, keepdims=True)

        def sm(h):
            for i in range(4):
                m = mx.pop((h, i))
                for kt in range(i + 1):
                    pt[(h, i, kt)] = jnp.exp2(st.pop((h, i, kt)) - m).astype(BF)

        def pv(h):
            g, j = divmod(h, HPG)
            base = 128 * g + 16 * j
            gate = gate_t[h:h + 1, :]
            for i in range(4):
                cols = slice(128 * i, 128 * (i + 1))
                o = None
                for kt in range(i + 1):
                    v = v_t[s, base:base + 32, 128 * kt:128 * (kt + 1)]
                    v = jnp.where(wrow >= 30, jnp.ones_like(v), v)
                    r = _dot(v, pt.pop((h, i, kt)))
                    o = r if o is None else o + r
                o = o * ((1.0 - gate) / o[31:32, :])
                if s > 0:
                    den = den_t[s - 1, 16 * g + j:16 * g + j + 1, cols] + 1e-6
                    o = o + am_t[s - 1, base:base + 32, cols] * (gate / den)
                off = 2 * j
                o_t[s, base + off:base + off + DH, cols] = o[off:off + DH].astype(BF)

        return qk, sm, pv

    def emit_attention(s, fillers):
        qk, sm, pv = make_attention(s)
        total = sum(c for c, _ in fillers)
        done, fi = 0, 0
        for b in range(H + 1):
            if b < H:
                qk(b)
            target = total * (b + 1) / (H + 1)
            while fi < len(fillers) and (done + fillers[fi][0] / 2 <= target or b == H):
                done += fillers[fi][0]
                fillers[fi][1]()
                fi += 1
            if b > 0:
                sm(b - 1)
                pv(b - 1)

    def proj_tasks(s):
        return [(GW[g] // 16 * 15, lambda s=s, tt=tt, g=g: proj_qkv(s, tt, g))
                for tt in range(4) for g in range(NG)]

    def out_tasks(s):
        tasks = [(60, lambda s=s, tt=tt, fb=fb: proj_out(s, tt, fb)) for tt in range(4) for fb in range(3)]
        tasks.append((0, lambda s=s: out_copy(s).start()))
        return tasks

    def ln_tasks(s):
        return [(10, lambda s=s, tt=tt: layernorm(s, tt)) for tt in range(4)]

    def upd_tasks(s):
        return [(GW[g] // 4, lambda s=s, g=g: mem_update(s, g)) for g in range(NG)]

    def read_tasks(s):
        return [(GW[g] // 4 + 4, lambda s=s, g=g: mem_read(s, g)) for g in range(NG)]

    init_pads()
    wr_copy.wait()
    prep_wr()
    beta_copy.wait()
    prep_gates()
    x_copy(0).wait()
    for tt in range(4):
        layernorm(0, tt)
    w_copy(0).wait()
    w_copy(1).wait()
    w_copy(2).wait()
    x_copy(1).wait()
    for g in range(NG):
        for which in range(3):
            prep_wt(g, which)
        for tt in range(4):
            proj_qkv(0, tt, g)
        if g < 4:
            layernorm(1, g)
    x_copy(2).wait()
    x_copy(3).wait()
    w_copy(3).wait()

    misc0 = [(5, lambda g=g: prep_wo(g)) for g in range(NG)]
    emit_attention(0, upd_tasks(0) + proj_tasks(1) + ln_tasks(2) + ln_tasks(3) + misc0
                   + [(5, moe_select)] + read_tasks(1))

    def wait_moe():
        wg_copy.wait()
        wu_copy.wait()
        wd_copy.wait()

    moe_tasks = ([(0, wait_moe)]
                 + [(60, lambda c=c: moe_chunk(c)) for c in range(FF // MOE_CHUNK)]
                 + [(5, moe_finish)])
    emit_attention(1, upd_tasks(1) + proj_tasks(2) + moe_tasks + read_tasks(2) + out_tasks(0))
    emit_attention(2, upd_tasks(2) + proj_tasks(3) + out_tasks(1) + read_tasks(3))
    emit_attention(3, out_tasks(2))
    for _, t in out_tasks(3):
        t()
    for s in range(NSEG):
        out_copy(s).wait()


@jax.jit
def pallas_parallel_sum__memory_aug_infini_attn__moe_arch_mod__prompt_kernel(
    A_x: jax.Array,
    A_wq: jax.Array,
    A_wk: jax.Array,
    A_wv: jax.Array,
    A_wo: jax.Array,
    A_beta: jax.Array,
    B_x: jax.Array,
    B_w_r: jax.Array,
    B_w_gate: jax.Array,
    B_w_up: jax.Array,
    B_w_down: jax.Array,
):
    del B_x
    hbm = pl.BlockSpec(memory_space=pltpu.HBM)
    scratch = [
        pltpu.VMEM((D, SEQ), BF),
        pltpu.VMEM((D, SEQ), BF),
        pltpu.VMEM((D, SEQ), F32),
        pltpu.VMEM((4, D, D), BF),
        pltpu.VMEM((3 * GP, D), BF),
        pltpu.VMEM((D, GP), BF),
        pltpu.VMEM((H,), BF),
        pltpu.VMEM((D,), BF),
        pltpu.VMEM((D, 128), F32),
        pltpu.VMEM((D, FF), BF),
        pltpu.VMEM((D, FF), BF),
        pltpu.VMEM((D, FF), BF),
        pltpu.VMEM((NSEG, GP, L), BF),
        pltpu.VMEM((NSEG - 1, GP, L), BF),
        pltpu.VMEM((NSEG, GP, L), BF),
        pltpu.VMEM((NSEG, L, GP), BF),
        pltpu.VMEM((NSEG - 1, GP, L), BF),
        pltpu.VMEM((NSEG, GP, L), BF),
        pltpu.VMEM((NSEG - 1, GP, L), F32),
        pltpu.VMEM((NSEG - 1, 16 * NG, L), F32),
        pltpu.VMEM((NG, 128, 128), F32),
        pltpu.VMEM((1, SEQ), F32),
        pltpu.VMEM((128, 128), F32),
        pltpu.VMEM((D, SEQ), BF),
        pltpu.SemaphoreType.DMA((13,)),
        pltpu.SemaphoreType.DMA((NSEG,)),
    ]
    out_t = pl.pallas_call(
        _kernel,
        out_shape=jax.ShapeDtypeStruct((1, D, SEQ), BF),
        in_specs=[hbm] * 10,
        out_specs=hbm,
        scratch_shapes=scratch,
        compiler_params=pltpu.CompilerParams(vmem_limit_bytes=100 * 1024 * 1024),
    )(jnp.swapaxes(A_x, 1, 2), A_wq, A_wk, A_wv, A_wo, A_beta, B_w_r, B_w_gate, B_w_up,
      B_w_down.T)
    return jnp.swapaxes(out_t, 1, 2)
```

```python
import contextlib
import json
import os

import jax
import jax.numpy as jnp
from jax import lax
import jax.experimental.pallas as pl
import jax.experimental.pallas.tpu as pltpu

BF = jnp.bfloat16
F32 = jnp.float32

SEQ, D, H, DH = 2048, 576, 32, 18
NSEG, L, FF = 4, 512, 4608
HPG = 7
NG = 5
GN = (7, 7, 7, 7, 4)
GW = (128, 128, 128, 128, 80)
GP = 592
ZR = (126, 126, 126, 126, 78)
QSCALE = (DH ** -0.5) * 1.4426950408889634
NT_DIMS = (((1,), (1,)), ((), ()))
MOE_DMA = 2304
NEG = -1e30
SPLIT = 10
SCORE_LIMIT = 40.0
_SCOPES = os.environ.get("KSCOPES", "") == "1"
CFG = dict()
CFG.update(json.loads(os.environ.get("KCFG", "{}")))


def _dot(a, b):
    return jnp.dot(a, b, preferred_element_type=F32)


def _dot_nt(a, b):
    return lax.dot_general(a, b, NT_DIMS, preferred_element_type=F32)


def _iota(shape, dim):
    return lax.broadcasted_iota(jnp.int32, shape, dim)


def _phi(t):
    return jnp.where(t > 0, t + 1.0, jnp.exp(t))


def _sigmoid(t):
    return 1.0 / (1.0 + jnp.exp(-t))


def _recip(x):
    r = pl.reciprocal(x, approx=True)
    r = r * (2.0 - x * r)
    return r * (2.0 - x * r)


def _div18(i):
    return (i * 57) >> 10


def _blk(t, size=128):
    if isinstance(t, int):
        return slice(size * t, size * (t + 1))
    return pl.ds(pl.multiple_of(t * size, size), size)


def _rows(start, size, align):
    if isinstance(start, int):
        return slice(start, start + size)
    return pl.ds(pl.multiple_of(start, align), size)


def _colsum(a):
    return jnp.sum(jnp.sum(a.reshape(a.shape[0] // 8, 8, a.shape[1]), axis=0), axis=0, keepdims=True)


def _kernel(x_hbm, wq_hbm, wk_hbm, wv_hbm, wo_hbm, beta_hbm, wr_hbm, wg_hbm, wu_hbm, wd_hbm,
            out_hbm,
            x_v, xn_v, res_v, stat_v, wraw, w_t, wo_t, beta_v, wr_v, wr_b, wg_v, wu_v, wd_v,
            q_t, pq_t, v_t, k_n, pk_t, o_t, p_buf, am_t, den_t, m_t, r_row, gate_t, moe_y, out_v,
            sem_in, sem_moe, sem_out, sem_bar):

    def x_copy(s, tt=None):
        if tt is None:
            c0, n, k = s * L, L, 3 + s
        else:
            c0, n, k = tt * 128, 128, tt
        return pltpu.make_async_copy(x_hbm.at[0, :, pl.ds(c0, n)], x_v.at[:, pl.ds(c0, n)],
                                     sem_in.at[k])

    def w_copy(i, cb):
        src = (wq_hbm, wk_hbm, wv_hbm)[i]
        n = 128 if cb < 4 else 64
        return pltpu.make_async_copy(src.at[:, pl.ds(128 * cb, n)], wraw.at[i, :, pl.ds(128 * cb, n)],
                                     sem_in.at[7 + 5 * i + cb])

    wo_copy = pltpu.make_async_copy(wo_hbm, wraw.at[3], sem_in.at[22])
    beta_copy = pltpu.make_async_copy(beta_hbm, beta_v, sem_in.at[23])
    wr_copy = pltpu.make_async_copy(wr_hbm, wr_v, sem_in.at[24])
    NMC = FF // MOE_DMA

    def moe_copy(i, c):
        src, dst = ((wg_hbm, wg_v), (wu_hbm, wu_v), (wd_hbm, wd_v))[i]
        cs = pl.ds(c * MOE_DMA, MOE_DMA)
        return pltpu.make_async_copy(src.at[:, cs], dst.at[:, cs], sem_moe.at[i * NMC + c])

    def out_copy(t):
        cs = pl.ds(t * 128 if isinstance(t, int) else pl.multiple_of(t * 128, 128), 128)
        return pltpu.make_async_copy(out_v.at[t], out_hbm.at[0, :, cs], sem_out.at[t])

    wr_copy.start()
    x_copy(0, 0).start()
    for i in range(3):
        w_copy(i, 0).start()
    beta_copy.start()
    for tt in range(1, 4):
        x_copy(0, tt).start()
    for cb in range(1, 5):
        for i in range(3):
            w_copy(i, cb).start()
    x_copy(1).start()
    x_copy(2).start()
    x_copy(3).start()
    wo_copy.start()

    def ln_stats(t):
        cols = _blk(t)
        shift = x_v[0:16, cols].astype(F32)[0:1]
        s1 = [None] * 2
        s2 = [None] * 2
        for u in range(D // 16):
            d = x_v[16 * u:16 * (u + 1), cols].astype(F32) - shift
            d = d.reshape(2, 8, 128)
            for k in range(2):
                s1[k] = d[k] if u == 0 else s1[k] + d[k]
                s2[k] = d[k] * d[k] if u == 0 else s2[k] + d[k] * d[k]
        m1 = jnp.sum(s1[0] + s1[1], axis=0, keepdims=True) * (1.0 / D)
        m2 = jnp.sum(s2[0] + s2[1], axis=0, keepdims=True) * (1.0 / D)
        var = jnp.maximum(m2 - m1 * m1, 0.0)
        stat_v[0:1, cols] = m1 + shift
        stat_v[8:9, cols] = lax.rsqrt(var + 1e-5)

    def ln_apply(t):
        cols = _blk(t)
        mean = stat_v[0:1, cols]
        rstd = stat_v[8:9, cols]
        for u in range(D // 48):
            rows = slice(48 * u, 48 * (u + 1))
            x = x_v[rows, cols].astype(F32)
            xn = (x - mean) * rstd
            xn_v[t, rows, :] = xn.astype(BF)
            res_v[rows, cols] = x + xn

    def router(t):
        r = _dot(wr_b[...], xn_v[t])
        r_row[:, _blk(t)] = r[0:1].astype(BF).astype(F32)

    def layernorm(t):
        ln_stats(t)
        ln_apply(t)
        router(t)

    def prep_wr():
        wr = wr_v[...].reshape(1, D)
        wr_b[...] = jnp.broadcast_to(wr.astype(F32), (16, D)).astype(BF)

    def prep_wt(cb, which):
        nb = 128 if cb < 4 else 64
        n = DH * GN[cb]
        t = wraw[which, :, 128 * cb:128 * cb + nb].T
        r0 = 384 * cb + which * GW[cb]
        k = min(n - 2 * cb, nb)
        w_t[r0 + 2 * cb:r0 + 2 * cb + k, :] = t[0:k]
        w_t[r0 + n:r0 + GW[cb], :] = jnp.zeros((GW[cb] - n, D), BF)
        if cb < 4:
            r1 = 384 * (cb + 1) + which * GW[cb + 1]
            w_t[r1:r1 + 2 * (cb + 1), :] = t[128 - 2 * (cb + 1):128]

    def prep_wo(g):
        n = DH * GN[g]
        wo_t[:, 128 * g:128 * g + n] = wraw[3, 126 * g:126 * g + n, :].T
        wo_t[:, 128 * g + n:128 * g + GW[g]] = jnp.zeros((D, GW[g] - n), BF)

    def prep_gates():
        b = beta_v[...].astype(F32).reshape(1, H)
        sig = jnp.concatenate([_sigmoid(b), jnp.zeros((1, 128 - H), F32)], axis=1)
        rows = jnp.broadcast_to(sig, (128, 128)).T
        for g in range(NG):
            gate_t[g] = rows[HPG * g:HPG * g + 8]

    def proj_qkv(s, tt, g, need_pq=True, need_pk=True):
        w = GW[g]
        rows = slice(128 * g, 128 * g + w)
        r = _dot(w_t[384 * g:384 * g + 3 * w, :], xn_v[4 * s + tt])
        q, k, v = r[:w], r[w:2 * w], r[2 * w:]
        q_t[s, tt, rows, :] = (q * QSCALE).astype(BF)
        if need_pq:
            pq_t[s, tt, rows, :] = _phi(q).astype(BF)
        k_n[s, g, _blk(tt), :w] = k.astype(BF).T
        if need_pk:
            pk_t[s, tt, rows, :] = _phi(k).astype(BF)
        v = jnp.where(_iota((w, 128), 0) == ZR[g], 1.0, v)
        v_t[s, tt, rows, :] = v.astype(BF)

    def mem_update(s, g, first):
        w = GW[g]
        rows = slice(128 * g, 128 * g + w)
        r = _dot_nt(v_t[s, 0, rows, :], pk_t[s, 0, rows, :])
        for tt in range(1, 4):
            r = r + _dot_nt(v_t[s, tt, rows, :], pk_t[s, tt, rows, :])
        rr, cc = _iota((w, w), 0), _iota((w, w), 1)
        keep = (cc < DH * GN[g]) & ((_div18(rr) == _div18(cc)) | (rr == ZR[g]))
        r = jnp.where(keep, r, 0.0)
        if not first:
            r = r + m_t[g, :w, :w]
        m_t[g, :w, :w] = r

    def mem_read(s, g):
        w = GW[g]
        rows = slice(128 * g, 128 * g + w)
        m = m_t[g, :w, :w]
        z = m[ZR[g]:ZR[g] + 1, :]
        zrows = jnp.where(_iota((16, w), 0) == _div18(_iota((16, w), 1)), z, 0.0)
        lhs = jnp.concatenate([m, zrows], axis=0).astype(BF)
        for tt in range(4):
            cols = slice(128 * tt, 128 * (tt + 1))
            r = _dot(lhs, pq_t[s, tt, rows, :])
            am_t[s, rows, cols] = r[:w]
            den_t[s, 16 * g:16 * (g + 1), cols] = r[w:]

    def proj_out(s, tt, fb):
        f0 = 192 * fb
        f1 = f0 + 192
        p = _dot(wo_t[f0:f1, :], o_t[s, tt])
        out_v[4 * s + tt, f0:f1, :] = (p + res_v[f0:f1, _blk(4 * s + tt)]).astype(BF)

    moe = {}

    def moe_select():
        r = r_row[...]
        io = _iota((1, SEQ), 1)
        m1 = jnp.max(r)
        i1 = jnp.min(jnp.where(r == m1, io, SEQ - 1))
        r2 = jnp.where(io == i1, -jnp.inf, r)
        m2 = jnp.max(r2)
        i2 = jnp.min(jnp.where((r2 == m2) & (io != i1), io, SEQ - 1))
        rows = []
        for i in (i1, i2):
            xb = xn_v[i // 128].T.astype(F32)
            rows.append(jnp.sum(jnp.where(_iota((128, D), 0) == i % 128, xb, 0.0), axis=0, keepdims=True))
        rr = _iota((16, D), 0)
        xs = jnp.where(rr == 0, rows[0], jnp.where(rr == 1, rows[1], 0.0))
        moe["x"] = xs.astype(BF)
        moe["w"] = _sigmoid(jnp.where(_iota((16, 1), 0) == 0, m1, m2))
        sel = jnp.where(_iota((2, 128), 0) == 0, i1, i2)
        for t in range(4 * NSEG):
            tok = _iota((2, 128), 1) + 128 * t
            o_t[t // 4, t % 4, 126:128, :] = jnp.where(tok == sel, 1.0, 0.0).astype(BF)

    KTS = [(128 * k, min(128 * (k + 1), D)) for k in range(5)]

    def moe_up(name, ref, f, k):
        k0, k1 = KTS[k]
        r = _dot(moe["x"][:, k0:k1], ref[k0:k1, _blk(f)])
        moe[name] = r if k == 0 else moe[name] + r

    def moe_down(f, n, first):
        if n == 0:
            g = moe["g"]
            moe["h"] = (g * _sigmoid(g) * moe["u"]).astype(BF)
        n0, n1 = KTS[n]
        r = _dot_nt(moe["h"], wd_v[n0:n1, _blk(f)])
        moe[("y", n)] = r if first else moe[("y", n)] + r

    def moe_micro_tasks():
        tasks = []
        for f in range(FF // 128):
            tasks += [lambda f=f, k=k: moe_up("g", wg_v, f, k) for k in range(5)]
            tasks += [lambda f=f, k=k: moe_up("u", wu_v, f, k) for k in range(5)]
            tasks += [lambda f=f, n=n: moe_down(f, n, f == 0) for n in range(5)]
        return tasks

    def moe_finish():
        y = jnp.concatenate([moe[("y", n)] for n in range(5)], axis=1) * moe["w"]
        rr = _iota((128, D), 0)
        ypad = jnp.where(rr == 126, y[0:1], jnp.where(rr == 127, y[1:2], 0.0))
        cur = wo_t[:, 0:128].astype(F32)
        wo_t[:, 0:128] = jnp.where(_iota((D, 128), 1) >= 126, ypad.T, cur).astype(BF)

    causal = _iota((128, 128), 0) <= _iota((128, 128), 1)
    wrow = _iota((32, 128), 0)

    def barrier():
        pl.semaphore_signal(sem_bar, 1)
        pl.semaphore_wait(sem_bar, 1)

    def query_weights(s, g, j, i, w):
        wq = q_t[s, i, _rows(128 * g + 16 * j, 32, 16), :]
        wq = jnp.where((wrow >= 2 * j) & (wrow < 2 * j + DH), wq, jnp.zeros_like(wq))
        parts = [wq]
        if j > 0:
            parts.insert(0, jnp.zeros((16 * j, 128), BF))
        if w - 16 * j - 32 > 0:
            parts.append(jnp.zeros((w - 16 * j - 32, 128), BF))
        return jnp.concatenate(parts, axis=0) if len(parts) > 1 else wq

    def score_tile(s, g, i, kt, w, wq):
        d = _dot(k_n[s, g, 128 * kt:128 * (kt + 1), :w], wq)
        return jnp.where(causal, d, NEG) if kt == i else d

    def value_tile(s, g, j, kt, p):
        v = v_t[s, kt, _rows(128 * g + 16 * j, 32, 16), :]
        return _dot(jnp.where(wrow >= 30, jnp.ones_like(v), v), p)

    def finish_column(s, g, j, i, o, with_mem):
        cols = slice(128 * i, 128 * (i + 1))
        win = _rows(128 * g + 16 * j, 32, 16)
        gate = gate_t[g][j:j + 1]
        o = o * ((1.0 - gate) * _recip(o[31:32, :]))
        if with_mem:
            den = den_t[s, _rows(16 * g, 16, 16), cols][j:j + 1] + 1e-6
            o = o + am_t[s, win, cols] * (gate * _recip(den))
        if isinstance(g, int):
            r0 = 128 * g + DH * j
            o_t[s, i, r0:r0 + DH, :] = o[2 * j:2 * j + DH].astype(BF)
        else:
            mine = (wrow >= 2 * j) & (wrow < 2 * j + DH)
            o_t[s, i, win, :] = jnp.where(mine, o, o_t[s, i, win, :].astype(F32)).astype(BF)

    def running_max(m, d):
        pm = jnp.max(d.reshape(16, 8, 128), axis=0)
        return pm if m is None else jnp.maximum(m, pm)

    def compact_path():
        for c in range(NMC):
            start_moe(c)
        for g in range(NG):
            prep_wo(g)
            m_t[g] = jnp.zeros((128, 128), F32)
        am_t[0] = jnp.zeros((GP, L), F32)
        den_t[0] = jnp.ones((16 * NG, L), F32)

        @pl.loop(0, 4 * NSEG)
        def _(t):
            layernorm(t)

        for c in range(NMC):
            wait_moe(c)
        moe_select()

        def expert(f, y):
            for k in range(5):
                moe_up("g", wg_v, f, k)
            for k in range(5):
                moe_up("u", wu_v, f, k)
            for n in range(5):
                moe[("y", n)] = y[n]
                moe_down(f, n, False)
            return tuple(moe[("y", n)] for n in range(5))

        y = lax.fori_loop(0, FF // 128, expert,
                          tuple(jnp.zeros((16, k1 - k0), F32) for k0, k1 in KTS))
        for n in range(5):
            moe[("y", n)] = y[n]
        moe_finish()

        def head(s, g, j, w):
            for i in range(4):
                wq = query_weights(s, g, j, i, w)
                tiles, m = [], None
                for kt in range(i + 1):
                    tiles.append(score_tile(s, g, i, kt, w, wq))
                    m = running_max(m, tiles[-1])
                m = jnp.max(m, axis=0, keepdims=True)
                o = None
                for kt in range(i + 1):
                    r = value_tile(s, g, j, kt, jnp.exp2(tiles[kt] - m).astype(BF))
                    o = r if o is None else o + r
                finish_column(s, g, j, i, o, True)

        @pl.loop(0, NSEG)
        def _(s):
            @pl.loop(0, 4)
            def _(tt):
                for g in range(NG):
                    proj_qkv(s, tt, g)

            @pl.when(s > 0)
            def _():
                for g in range(NG):
                    mem_read(s, g)

            @pl.loop(0, NG - 1)
            def _(g):
                for j in range(HPG):
                    head(s, g, j, 128)

            for j in range(GN[NG - 1]):
                head(s, NG - 1, j, GW[NG - 1])
            for g in range(NG):
                mem_update(s, g, False)

            @pl.loop(0, 4)
            def _(tt):
                for fb in range(3):
                    proj_out(s, tt, fb)
                out_copy(4 * s + tt).start()
                out_copy(4 * s + tt).wait()

    def make_blocks():
        blocks = []
        for s in range(NSEG - 1):
            blocks += [[(s, h, i) for i in range(4)] for h in range(H)]
        s = NSEG - 1
        for i, per in ((3, 2), (2, 3), (1, 5), (0, 10)):
            for h0 in range(0, H, per):
                blocks.append([(s, h, i) for h in range(h0, min(h0 + per, H))])
        return blocks

    def run_pipeline():
        blocks = make_blocks()
        nb = len(blocks)
        st, mx = {}, {}

        def scores(b, micro):
            usemax = b < SPLIT or CFG.get("allmax")
            slot = 0
            for (s, h, i) in blocks[b]:
                g, j = divmod(h, HPG)
                wq = query_weights(s, g, j, i, GW[g])
                m = None
                for kt in range(i + 1):
                    d = score_tile(s, g, i, kt, GW[g], wq)
                    micro()
                    if usemax:
                        st[(b, slot)] = d
                        m = running_max(m, d)
                    else:
                        p_buf[b % 2, slot] = jnp.exp2(d).astype(BF)
                    slot += 1
                if usemax:
                    mx[(s, h, i)] = jnp.max(m, axis=0, keepdims=True)

        def values(b):
            usemax = b < SPLIT or CFG.get("allmax")
            slot = 0
            for (s, h, i) in blocks[b]:
                g, j = divmod(h, HPG)
                m = mx.pop((s, h, i)) if usemax else None
                o = None
                for kt in range(i + 1):
                    if usemax:
                        p = jnp.exp2(st.pop((b, slot)) - m).astype(BF)
                    else:
                        p = p_buf[b % 2, slot]
                    r = value_tile(s, g, j, kt, p)
                    o = r if o is None else o + r
                    slot += 1
                finish_column(s, g, j, i, o, s > 0)

        def proj_tasks(s, groups=range(NG)):
            return [(GW[g] // 16 * 15,
                     lambda s=s, tt=tt, g=g: proj_qkv(s, tt, g, s > 0, s < NSEG - 1))
                    for tt in range(4) for g in groups]

        def out_tasks(s, tts=range(4)):
            tasks = []
            for tt in tts:
                tasks += [(60, lambda s=s, tt=tt, fb=fb: proj_out(s, tt, fb)) for fb in range(3)]
                tasks.append((0, lambda s=s, tt=tt: out_copy(4 * s + tt).start()))
            return tasks

        def ln_tasks(s):
            ts = range(4 * s, 4 * s + 4)
            return ([(10, lambda t=t: ln_stats(t)) for t in ts]
                    + [(10, lambda t=t: ln_apply(t)) for t in ts]
                    + [(2, lambda t=t: router(t)) for t in ts])

        def upd_tasks(s):
            return [(GW[g] // 4, lambda s=s, g=g: mem_update(s, g, s == 0)) for g in range(NG)]

        def read_tasks(s):
            return [(GW[g] // 4 + 4, lambda s=s, g=g: mem_read(s, g)) for g in range(NG)]

        def prep_tasks(cbs):
            return [(5, lambda cb=cb, which=which: prep_wt(cb, which)) for cb in cbs for which in range(3)]

        guard = {}

        def norm_task(i):
            guard[i] = max_col_norm2(i)

        mtasks = moe_micro_tasks()
        a3 = 3 * H
        e3 = [a3 + 16, a3 + 27, a3 + 34, nb]
        streams = [
            (0, 1, prep_tasks((1,))),
            (0, 2, prep_tasks((2,))),
            (1, 4, proj_tasks(0, (1,))),
            (3, 5, prep_tasks((3, 4))),
            (4, 8, proj_tasks(0, (2,))),
            (3, 7, ln_tasks(1)),
            (5, 8, [(1, lambda i=i: norm_task(i)) for i in range(3)]),
            (8, 14, proj_tasks(0, (3, 4))),
            (12, 30, proj_tasks(1)),
            (16, 20, upd_tasks(0)),
            (30, 32, read_tasks(1)),
            (11, 30, ln_tasks(2) + ln_tasks(3)),
            (11, 31, [(5, lambda g=g: prep_wo(g)) for g in range(NG)]),
            (32, 33, [(1, moe_select)]),
            (33, 38, upd_tasks(1)),
            (32, 62, proj_tasks(2)),
            (62, 64, read_tasks(2)),
            (65, 70, upd_tasks(2)),
            (64, 94, proj_tasks(3)),
            (94, 96, read_tasks(3)),
            (95, 96, [(1, moe_finish)]),
            (a3 + 1, e3[2], out_tasks(0) + out_tasks(1) + out_tasks(2)),
            (e3[0] + 1, e3[1], out_tasks(3, (3,))),
            (e3[1] + 1, e3[2], out_tasks(3, (2,))),
            (e3[2] + 1, nb + 1, out_tasks(3, (1,))),
        ]
        micro_ranges = [(34, 64, mtasks[:270]), (64, 95, mtasks[270:])]
        ntiles = [sum(i + 1 for (_, _, i) in blk) for blk in blocks]

        def fence_w12():
            wait_w(1)
            wait_w(2)

        def fence_w34():
            wait_w(3)
            wait_w(4)
            x_copy(1).wait()

        def fence_a1():
            wait_moe(0)
            start_moe(1)

        fences = {0: fence_w12, 3: fence_w34, SPLIT: lambda: start_moe(0), 32: fence_a1,
                  64: lambda: wait_moe(1), a3: barrier}

        state = [[0, 0.0, float(sum(c for c, _ in t))] for _, _, t in streams]
        mstate = [[0, 0] for _ in micro_ranges]
        cur_scope = []

        def emit(b0, b1):
            for b in range(b0, b1 + 1):
                if _SCOPES and b % 4 == 0:
                    if cur_scope:
                        cur_scope.pop().__exit__(None, None, None)
                    cur_scope.append(jax.named_scope(f"blk{b:03d}"))
                    cur_scope[-1].__enter__()
                if b in fences and b < b1:
                    fences[b]()

                def micro(b=b):
                    for (lo, hi, tasks), ms in zip(micro_ranges, mstate):
                        if lo <= b < hi:
                            ms[0] += 1
                            total = sum(ntiles[lo:hi])
                            while ms[1] < len(tasks) and ms[1] < ms[0] * len(tasks) / total:
                                tasks[ms[1]]()
                                ms[1] += 1

                if b < b1:
                    scores(b, micro)
                if b < b1 or b == nb:
                    for (lo, hi, tasks), st_ in zip(streams, state):
                        if b < lo:
                            continue
                        frac = (b + 1 - lo) / (hi - lo)
                        while st_[0] < len(tasks) and st_[1] + tasks[st_[0]][0] / 2 <= frac * st_[2] + 1e-9:
                            st_[1] += tasks[st_[0]][0]
                            tasks[st_[0]][1]()
                            st_[0] += 1
                if b > b0:
                    values(b - 1)
            if cur_scope:
                cur_scope.pop().__exit__(None, None, None)

        def fast_rest():
            emit(SPLIT, nb)
            for (lo, hi, tasks), st_ in zip(streams, state):
                assert st_[0] == len(tasks), (lo, hi, st_)
            assert sum(ms[1] for ms in mstate) == len(mtasks)
            with scope("tail0"):
                for _, t in out_tasks(3, (0,)):
                    t()
            with scope("tail1"):
                for t in range(4 * NSEG):
                    out_copy(t).wait()

        emit(0, SPLIT)
        x_copy(2).wait()
        x_copy(3).wait()
        wo_copy.wait()
        safe = jnp.logical_and(guard[0] * guard[1] <= (SCORE_LIMIT / (1.05 * D * QSCALE * DH)) ** 2,
                               guard[2] <= 1e30)
        if CFG.get("only") == "fast":
            fast_rest()
        elif CFG.get("only") == "compact":
            compact_path()
        else:
            pl.when(safe)(fast_rest)
            pl.when(jnp.logical_not(safe))(compact_path)

    def prep_group(g):
        for which in range(3):
            prep_wt(g, which)

    def wait_w(cb):
        for i in range(3):
            w_copy(i, cb).wait()

    def start_moe(c):
        for i in range(3):
            moe_copy(i, c).start()

    def wait_moe(c):
        for i in range(3):
            moe_copy(i, c).wait()

    def max_col_norm2(i):
        m = None
        for cb in range(4):
            wv = wraw[i, :, 128 * cb:128 * (cb + 1)].astype(F32)
            c = _colsum(wv * wv)
            m = c if m is None else jnp.maximum(m, c)
        wv = wraw[i, :, 512:D].astype(F32)
        c = jnp.sum(wv * wv, axis=0, keepdims=True)
        return jnp.maximum(jnp.max(m), jnp.max(c))

    def scope(name):
        return jax.named_scope(name) if _SCOPES else contextlib.nullcontext()

    with scope("pre0"):
        for s in range(NSEG):
            for g in range(NG):
                n = DH * GN[g]
                for tt in range(4):
                    o_t[s, tt, 128 * g + n:128 * g + GW[g], :] = jnp.zeros((GW[g] - n, 128), BF)
        wr_copy.wait()
        x_copy(0, 0).wait()
        prep_wr()
        layernorm(0)
    with scope("pre1"):
        wait_w(0)
        prep_group(0)
        proj_qkv(0, 0, 0, False, True)
    with scope("pre2"):
        for tt in range(1, 4):
            x_copy(0, tt).wait()
        beta_copy.wait()
        for tt in range(1, 4):
            layernorm(tt)
            proj_qkv(0, tt, 0, False, True)
        prep_gates()
    run_pipeline()


@jax.jit
def pallas_parallel_sum__memory_aug_infini_attn__moe_arch_mod__prompt_kernel(
    A_x: jax.Array,
    A_wq: jax.Array,
    A_wk: jax.Array,
    A_wv: jax.Array,
    A_wo: jax.Array,
    A_beta: jax.Array,
    B_x: jax.Array,
    B_w_r: jax.Array,
    B_w_gate: jax.Array,
    B_w_up: jax.Array,
    B_w_down: jax.Array,
):
    del B_x
    hbm = pl.BlockSpec(memory_space=pltpu.HBM)
    scratch = [
        pltpu.VMEM((D, SEQ), BF),
        pltpu.VMEM((4 * NSEG, D, 128), BF),
        pltpu.VMEM((D, SEQ), F32),
        pltpu.VMEM((16, SEQ), F32),
        pltpu.VMEM((4, D, D), BF),
        pltpu.VMEM((3 * GP, D), BF),
        pltpu.VMEM((D, GP), BF),
        pltpu.VMEM((H,), BF),
        pltpu.VMEM((D,), BF),
        pltpu.VMEM((16, D), BF),
        pltpu.VMEM((D, FF), BF),
        pltpu.VMEM((D, FF), BF),
        pltpu.VMEM((D, FF), BF),
        pltpu.VMEM((NSEG, 4, GP, 128), BF),
        pltpu.VMEM((NSEG, 4, GP, 128), BF),
        pltpu.VMEM((NSEG, 4, GP, 128), BF),
        pltpu.VMEM((NSEG, NG, L, 128), BF),
        pltpu.VMEM((NSEG, 4, GP, 128), BF),
        pltpu.VMEM((NSEG, 4, GP, 128), BF),
        pltpu.VMEM((2, 10, 128, 128), BF),
        pltpu.VMEM((NSEG, GP, L), F32),
        pltpu.VMEM((NSEG, 16 * NG, L), F32),
        pltpu.VMEM((NG, 128, 128), F32),
        pltpu.VMEM((1, SEQ), F32),
        pltpu.VMEM((NG, 8, 128), F32),
        pltpu.VMEM((16, D), F32),
        pltpu.VMEM((4 * NSEG, D, 128), BF),
        pltpu.SemaphoreType.DMA((25,)),
        pltpu.SemaphoreType.DMA((3 * (FF // MOE_DMA),)),
        pltpu.SemaphoreType.DMA((4 * NSEG,)),
        pltpu.SemaphoreType.REGULAR,
    ]
    out_t = pl.pallas_call(
        _kernel,
        out_shape=jax.ShapeDtypeStruct((1, D, SEQ), BF),
        in_specs=[hbm] * 10,
        out_specs=hbm,
        scratch_shapes=scratch,
        compiler_params=pltpu.CompilerParams(vmem_limit_bytes=100 * 1024 * 1024),
    )(jnp.swapaxes(A_x, 1, 2), A_wq, A_wk, A_wv, A_wo, A_beta, B_w_r, B_w_gate, B_w_up,
      B_w_down.T)
    return jnp.swapaxes(out_t, 1, 2)
```

```python
import contextlib
import json
import os

import jax
import jax.numpy as jnp
from jax import lax
import jax.experimental.pallas as pl
import jax.experimental.pallas.tpu as pltpu

BF = jnp.bfloat16
F32 = jnp.float32

SEQ, D, H, DH = 2048, 576, 32, 18
NSEG, L, FF = 4, 512, 4608
HPG = 7
NG = 5
GN = (7, 7, 7, 7, 4)
GW = (128, 128, 128, 128, 80)
GP = 592
ZR = (126, 126, 126, 126, 78)
QSCALE = (DH ** -0.5) * 1.4426950408889634
NT_DIMS = (((1,), (1,)), ((), ()))
MOE_DMA = 2304
NEG = -1e30
SPLIT = int(os.environ.get('KSPLIT', 9))
SCORE_LIMIT = 40.0
_SCOPES = os.environ.get("KSCOPES", "") == "1"
CFG = dict()
CFG.update(json.loads(os.environ.get("KCFG", "{}")))


def _dot(a, b):
    return jnp.dot(a, b, preferred_element_type=F32)


def _dot_nt(a, b):
    return lax.dot_general(a, b, NT_DIMS, preferred_element_type=F32)


def _iota(shape, dim):
    return lax.broadcasted_iota(jnp.int32, shape, dim)


def _phi(t):
    return jnp.where(t > 0, t + 1.0, jnp.exp(t))


def _sigmoid(t):
    return 1.0 / (1.0 + jnp.exp(-t))


def _recip(x):
    r = pl.reciprocal(x, approx=True)
    r = r * (2.0 - x * r)
    return r * (2.0 - x * r)


def _div18(i):
    return (i * 57) >> 10


def _blk(t, size=128):
    if isinstance(t, int):
        return slice(size * t, size * (t + 1))
    return pl.ds(pl.multiple_of(t * size, size), size)


def _rows(start, size, align):
    if isinstance(start, int):
        return slice(start, start + size)
    return pl.ds(pl.multiple_of(start, align), size)


def _colsum(a):
    return jnp.sum(jnp.sum(a.reshape(a.shape[0] // 8, 8, a.shape[1]), axis=0), axis=0, keepdims=True)


def _kernel(x_hbm, wq_hbm, wk_hbm, wv_hbm, wo_hbm, beta_hbm, wr_hbm, wg_hbm, wu_hbm, wd_hbm,
            out_hbm,
            x_v, xn_v, res_v, stat_v, wraw, w_t, wo_t, beta_v, wr_v, wr_b, wg_v, wu_v, wd_v,
            q_t, pq_t, v_t, k_n, pk_t, o_t, p_buf, am_t, den_t, m_t, r_row, gate_t, moe_y, out_v,
            sem_in, sem_moe, sem_out, sem_bar):

    def x_copy(s, tt=None):
        if tt is None:
            c0, n, k = s * L, L, 3 + s
        else:
            c0, n, k = tt * 128, 128, tt
        return pltpu.make_async_copy(x_hbm.at[0, :, pl.ds(c0, n)], x_v.at[:, pl.ds(c0, n)],
                                     sem_in.at[k])

    def w_copy(i, cb):
        src = (wq_hbm, wk_hbm, wv_hbm)[i]
        n = 128 if cb < 4 else 64
        return pltpu.make_async_copy(src.at[:, pl.ds(128 * cb, n)], wraw.at[i, :, pl.ds(128 * cb, n)],
                                     sem_in.at[7 + 5 * i + cb])

    wo_copy = pltpu.make_async_copy(wo_hbm, wraw.at[3], sem_in.at[22])
    beta_copy = pltpu.make_async_copy(beta_hbm, beta_v, sem_in.at[23])
    wr_copy = pltpu.make_async_copy(wr_hbm, wr_v, sem_in.at[24])
    NMC = FF // MOE_DMA

    def moe_copy(i, c):
        src, dst = ((wg_hbm, wg_v), (wu_hbm, wu_v), (wd_hbm, wd_v))[i]
        cs = pl.ds(c * MOE_DMA, MOE_DMA)
        return pltpu.make_async_copy(src.at[:, cs], dst.at[:, cs], sem_moe.at[i * NMC + c])

    def out_copy(t):
        cs = pl.ds(t * 128 if isinstance(t, int) else pl.multiple_of(t * 128, 128), 128)
        return pltpu.make_async_copy(out_v.at[t], out_hbm.at[0, :, cs], sem_out.at[t])

    wr_copy.start()
    x_copy(0, 0).start()
    for i in range(3):
        w_copy(i, 0).start()
    beta_copy.start()
    for tt in range(1, 4):
        x_copy(0, tt).start()
    for cb in range(1, 5):
        for i in range(3):
            w_copy(i, cb).start()
    x_copy(1).start()
    x_copy(2).start()
    x_copy(3).start()
    wo_copy.start()

    pace = {}

    def paced(row):
        tok = pace.get("tok")
        return row if tok is None else row + tok * 0.0

    def ln_stats(t):
        cols = _blk(t)
        shift = paced(x_v[0:16, cols].astype(F32)[0:1])
        s1 = [None] * 2
        s2 = [None] * 2
        for u in range(D // 16):
            d = x_v[16 * u:16 * (u + 1), cols].astype(F32) - shift
            d = d.reshape(2, 8, 128)
            for k in range(2):
                s1[k] = d[k] if u == 0 else s1[k] + d[k]
                s2[k] = d[k] * d[k] if u == 0 else s2[k] + d[k] * d[k]
        m1 = jnp.sum(s1[0] + s1[1], axis=0, keepdims=True) * (1.0 / D)
        m2 = jnp.sum(s2[0] + s2[1], axis=0, keepdims=True) * (1.0 / D)
        var = jnp.maximum(m2 - m1 * m1, 0.0)
        stat_v[0:1, cols] = m1 + shift
        stat_v[8:9, cols] = lax.rsqrt(var + 1e-5)

    def ln_apply(t):
        cols = _blk(t)
        mean = paced(stat_v[0:1, cols])
        rstd = stat_v[8:9, cols]
        for u in range(D // 48):
            rows = slice(48 * u, 48 * (u + 1))
            x = x_v[rows, cols].astype(F32)
            xn = (x - mean) * rstd
            xn_v[t, rows, :] = xn.astype(BF)
            res_v[rows, cols] = x + xn

    def router(t):
        r = _dot(wr_b[...], xn_v[t])
        r_row[:, _blk(t)] = r[0:1].astype(BF).astype(F32)

    def layernorm(t):
        ln_stats(t)
        ln_apply(t)
        router(t)

    def prep_wr():
        wr = wr_v[...].reshape(1, D)
        wr_b[...] = jnp.broadcast_to(wr.astype(F32), (16, D)).astype(BF)

    def prep_wt(cb, which):
        nb = 128 if cb < 4 else 64
        n = DH * GN[cb]
        t = wraw[which, :, 128 * cb:128 * cb + nb].T
        r0 = 384 * cb + which * GW[cb]
        k = min(n - 2 * cb, nb)
        w_t[r0 + 2 * cb:r0 + 2 * cb + k, :] = t[0:k]
        w_t[r0 + n:r0 + GW[cb], :] = jnp.zeros((GW[cb] - n, D), BF)
        if cb < 4:
            r1 = 384 * (cb + 1) + which * GW[cb + 1]
            w_t[r1:r1 + 2 * (cb + 1), :] = t[128 - 2 * (cb + 1):128]

    def prep_wo(g):
        n = DH * GN[g]
        wo_t[:, 128 * g:128 * g + n] = wraw[3, 126 * g:126 * g + n, :].T
        wo_t[:, 128 * g + n:128 * g + GW[g]] = jnp.zeros((D, GW[g] - n), BF)

    def prep_gates():
        b = beta_v[...].astype(F32).reshape(1, H)
        sig = jnp.concatenate([_sigmoid(b), jnp.zeros((1, 128 - H), F32)], axis=1)
        rows = jnp.broadcast_to(sig, (128, 128)).T
        for g in range(NG):
            gate_t[g] = rows[HPG * g:HPG * g + 8]

    def proj_qkv(s, tt, g, need_pq=True, need_pk=True):
        w = GW[g]
        rows = slice(128 * g, 128 * g + w)
        r = _dot(w_t[384 * g:384 * g + 3 * w, :], xn_v[4 * s + tt])
        q, k, v = r[:w], r[w:2 * w], r[2 * w:]
        q_t[s, tt, rows, :] = (q * QSCALE).astype(BF)
        if need_pq:
            pq_t[s, tt, rows, :] = _phi(q).astype(BF)
        k_n[s, g, _blk(tt), :w] = k.astype(BF).T
        if need_pk:
            pk_t[s, tt, rows, :] = _phi(k).astype(BF)
        v = jnp.where(_iota((w, 128), 0) == ZR[g], 1.0, v)
        v_t[s, tt, rows, :] = v.astype(BF)

    def mem_update(s, g, first):
        w = GW[g]
        rows = slice(128 * g, 128 * g + w)
        r = _dot_nt(v_t[s, 0, rows, :], pk_t[s, 0, rows, :])
        for tt in range(1, 4):
            r = r + _dot_nt(v_t[s, tt, rows, :], pk_t[s, tt, rows, :])
        rr, cc = _iota((w, w), 0), _iota((w, w), 1)
        keep = (cc < DH * GN[g]) & ((_div18(rr) == _div18(cc)) | (rr == ZR[g]))
        r = jnp.where(keep, r, 0.0)
        if not first:
            r = r + m_t[g, :w, :w]
        m_t[g, :w, :w] = r

    def mem_read(s, g):
        w = GW[g]
        rows = slice(128 * g, 128 * g + w)
        m = m_t[g, :w, :w]
        z = m[ZR[g]:ZR[g] + 1, :]
        zrows = jnp.where(_iota((16, w), 0) == _div18(_iota((16, w), 1)), z, 0.0)
        lhs = jnp.concatenate([m, zrows], axis=0).astype(BF)
        for tt in range(4):
            cols = slice(128 * tt, 128 * (tt + 1))
            r = _dot(lhs, pq_t[s, tt, rows, :])
            am_t[s, rows, cols] = r[:w]
            den_t[s, 16 * g:16 * (g + 1), cols] = r[w:]

    def proj_out(s, tt, fb, by_group=False):
        f0 = 192 * fb
        f1 = f0 + 192
        if by_group:
            p = None
            for g in range(NG):
                r = _dot(wo_t[f0:f1, 128 * g:128 * g + GW[g]], o_t[s, tt, 128 * g:128 * g + GW[g], :])
                p = r if p is None else p + r
        else:
            p = _dot(wo_t[f0:f1, :], o_t[s, tt])
        out_v[4 * s + tt, f0:f1, :] = (p + res_v[f0:f1, _blk(4 * s + tt)]).astype(BF)

    moe = {}

    def moe_select():
        r = r_row[...]
        io = _iota((1, SEQ), 1)
        m1 = jnp.max(r)
        i1 = jnp.min(jnp.where(r == m1, io, SEQ - 1))
        r2 = jnp.where(io == i1, -jnp.inf, r)
        m2 = jnp.max(r2)
        i2 = jnp.min(jnp.where((r2 == m2) & (io != i1), io, SEQ - 1))
        rows = []
        for i in (i1, i2):
            xb = xn_v[i // 128].T.astype(F32)
            rows.append(jnp.sum(jnp.where(_iota((128, D), 0) == i % 128, xb, 0.0), axis=0, keepdims=True))
        rr = _iota((16, D), 0)
        xs = jnp.where(rr == 0, rows[0], jnp.where(rr == 1, rows[1], 0.0))
        moe["x"] = xs.astype(BF)
        moe["w"] = _sigmoid(jnp.where(_iota((16, 1), 0) == 0, m1, m2))
        sel = jnp.where(_iota((2, 128), 0) == 0, i1, i2)
        for t in range(4 * NSEG):
            tok = _iota((2, 128), 1) + 128 * t
            o_t[t // 4, t % 4, 126:128, :] = jnp.where(tok == sel, 1.0, 0.0).astype(BF)

    KTS = [(128 * k, min(128 * (k + 1), D)) for k in range(5)]

    def moe_up(name, ref, f, k):
        k0, k1 = KTS[k]
        r = _dot(moe["x"][:, k0:k1], ref[k0:k1, _blk(f)])
        moe[name] = r if k == 0 else moe[name] + r

    def moe_hidden(f):
        g = moe["g"]
        moe[("h", f if isinstance(f, int) else 0)] = (g * _sigmoid(g) * moe["u"]).astype(BF)

    def moe_down(f, n, first):
        n0, n1 = KTS[n]
        r = _dot_nt(moe[("h", f if isinstance(f, int) else 0)], wd_v[n0:n1, _blk(f)])
        moe[("y", n)] = r if first else moe[("y", n)] + r

    def moe_up_tasks(fs):
        tasks = []
        for f in fs:
            tasks += [lambda f=f, k=k: moe_up("g", wg_v, f, k) for k in range(5)]
            tasks += [lambda f=f, k=k: moe_up("u", wu_v, f, k) for k in range(4)]
            tasks.append(lambda f=f: (moe_up("u", wu_v, f, 4), moe_hidden(f)))
        return tasks

    def moe_down_tasks(fs):
        return [(f, lambda f=f, n=n: moe_down(f, n, f == 0)) for f in fs for n in range(5)]

    def moe_finish():
        y = jnp.concatenate([moe[("y", n)] for n in range(5)], axis=1) * moe["w"]
        rr = _iota((128, D), 0)
        ypad = jnp.where(rr == 126, y[0:1], jnp.where(rr == 127, y[1:2], 0.0))
        cur = wo_t[:, 0:128].astype(F32)
        wo_t[:, 0:128] = jnp.where(_iota((D, 128), 1) >= 126, ypad.T, cur).astype(BF)

    causal = _iota((128, 128), 0) <= _iota((128, 128), 1)
    wrow = _iota((32, 128), 0)

    def barrier():
        pl.semaphore_signal(sem_bar, 1)
        pl.semaphore_wait(sem_bar, 1)

    def query_weights(s, g, j, i, w):
        wq = q_t[s, i, _rows(128 * g + 16 * j, 32, 16), :]
        wq = jnp.where((wrow >= 2 * j) & (wrow < 2 * j + DH), wq, jnp.zeros_like(wq))
        parts = [wq]
        if j > 0:
            parts.insert(0, jnp.zeros((16 * j, 128), BF))
        if w - 16 * j - 32 > 0:
            parts.append(jnp.zeros((w - 16 * j - 32, 128), BF))
        return jnp.concatenate(parts, axis=0) if len(parts) > 1 else wq

    def score_tile(s, g, i, kt, w, wq):
        d = _dot(k_n[s, g, 128 * kt:128 * (kt + 1), :w], wq)
        return jnp.where(causal, d, NEG) if kt == i else d

    def value_tile(s, g, j, kt, p):
        v = v_t[s, kt, _rows(128 * g + 16 * j, 32, 16), :]
        return _dot(jnp.where(wrow >= 30, jnp.ones_like(v), v), p)

    def finish_column(s, g, j, i, o, with_mem):
        cols = slice(128 * i, 128 * (i + 1))
        win = _rows(128 * g + 16 * j, 32, 16)
        gate = gate_t[g][j:j + 1]
        scale = (1.0 - gate) * _recip(o[31:32, :])
        if isinstance(g, int) and CFG.get("pace", 1):
            pace["tok"] = scale
        o = o * scale
        if with_mem:
            den = den_t[s, _rows(16 * g, 16, 16), cols][j:j + 1] + 1e-6
            o = o + am_t[s, win, cols] * (gate * _recip(den))
        if isinstance(g, int):
            r0 = 128 * g + DH * j
            o_t[s, i, r0:r0 + DH, :] = o[2 * j:2 * j + DH].astype(BF)
        else:
            mine = (wrow >= 2 * j) & (wrow < 2 * j + DH)
            o_t[s, i, win, :] = jnp.where(mine, o, o_t[s, i, win, :].astype(F32)).astype(BF)

    def running_max(m, d):
        pm = jnp.max(d.reshape(16, 8, 128), axis=0)
        return pm if m is None else jnp.maximum(m, pm)

    def compact_path():
        pace.clear()
        for c in range(NMC):
            start_moe(c)
        for g in range(NG):
            prep_wo(g)
            m_t[g] = jnp.zeros((128, 128), F32)
        am_t[0] = jnp.zeros((GP, L), F32)
        den_t[0] = jnp.ones((16 * NG, L), F32)

        @pl.loop(0, 4 * NSEG)
        def _(t):
            layernorm(t)

        for c in range(NMC):
            wait_moe(c)
        moe_select()

        def expert(f, y):
            for k in range(5):
                moe_up("g", wg_v, f, k)
            for k in range(5):
                moe_up("u", wu_v, f, k)
            moe_hidden(f)
            for n in range(5):
                moe[("y", n)] = y[n]
                moe_down(f, n, False)
            return tuple(moe[("y", n)] for n in range(5))

        y = lax.fori_loop(0, FF // 128, expert,
                          tuple(jnp.zeros((16, k1 - k0), F32) for k0, k1 in KTS))
        for n in range(5):
            moe[("y", n)] = y[n]
        moe_finish()

        def head(s, g, j, w):
            for i in range(4):
                wq = query_weights(s, g, j, i, w)
                tiles, m = [], None
                for kt in range(i + 1):
                    tiles.append(score_tile(s, g, i, kt, w, wq))
                    m = running_max(m, tiles[-1])
                m = jnp.max(m, axis=0, keepdims=True)
                o = None
                for kt in range(i + 1):
                    r = value_tile(s, g, j, kt, jnp.exp2(tiles[kt] - m).astype(BF))
                    o = r if o is None else o + r
                finish_column(s, g, j, i, o, True)
                pace.clear()

        @pl.loop(0, NSEG)
        def _(s):
            @pl.loop(0, 4)
            def _(tt):
                for g in range(NG):
                    proj_qkv(s, tt, g)

            @pl.when(s > 0)
            def _():
                for g in range(NG):
                    mem_read(s, g)

            @pl.loop(0, NG - 1)
            def _(g):
                for j in range(HPG):
                    head(s, g, j, 128)

            for j in range(GN[NG - 1]):
                head(s, NG - 1, j, GW[NG - 1])
            for g in range(NG):
                mem_update(s, g, False)

            @pl.loop(0, 4)
            def _(tt):
                for fb in range(3):
                    proj_out(s, tt, fb)
                out_copy(4 * s + tt).start()
                out_copy(4 * s + tt).wait()

    def head_units(first_head):
        units, h = [], first_head
        while h < H:
            g, j = divmod(h, HPG)
            if j + 1 < GN[g]:
                units.append((h, h + 1))
                h += 2
            else:
                units.append((h,))
                h += 1
        return units

    def make_blocks():
        blocks = [[(0, (h,), i) for i in range(4)] for h in range(SPLIT)]
        for s in range(NSEG - 1):
            blocks += [[(s, u, i) for i in range(4)] for u in head_units(SPLIT if s == 0 else 0)]
        s = NSEG - 1
        for i, budget in ((3, 16), (2, 18), (1, 20), (0, 20)):
            cur, n = [], 0
            for u in head_units(0):
                cost = len(u) * (i + 1)
                if cur and n + cost > budget:
                    blocks.append(cur)
                    cur, n = [], 0
                cur.append((s, u, i))
                n += cost
            blocks.append(cur)
        return blocks

    col128 = _iota((64, 128), 1)
    mix_mask = _iota((64, 128), 0) <= (col128 & 63)

    def run_pipeline():
        blocks = make_blocks()
        nb = len(blocks)
        st, mx = {}, {}

        def scores(b, micro):
            usemax = b < SPLIT or CFG.get("allmax")
            slot = 0
            for (s, heads, i) in blocks[b]:
                g = heads[0] // HPG
                w = GW[g]
                wqs = [query_weights(s, g, h % HPG, i, w) for h in heads]
                paired = len(heads) == 2 and not usemax and not CFG.get("nopair")
                for n, h in enumerate(heads):
                    m = None
                    for kt in range(i + 1):
                        if paired and kt == i:
                            d = _dot(k_n[s, g, 128 * kt:128 * kt + 64, :w], wqs[n])
                            micro()
                            p_buf[b % 2, slot, 0:64, :] = jnp.exp2(
                                jnp.where(causal[:64], d, NEG)).astype(BF)
                            slot += 1
                            continue
                        d = score_tile(s, g, i, kt, w, wqs[n])
                        micro()
                        if usemax:
                            st[(b, slot)] = d
                            m = running_max(m, d)
                        else:
                            p_buf[b % 2, slot] = jnp.exp2(d).astype(BF)
                        slot += 1
                    if usemax:
                        mx[(s, h, i)] = jnp.max(m, axis=0, keepdims=True)
                if paired:
                    wmix = jnp.concatenate([wqs[1][:, 64:], wqs[0][:, 64:]], axis=1)
                    d = _dot(k_n[s, g, 128 * i + 64:128 * (i + 1), :w], wmix)
                    e = jnp.exp2(jnp.where(mix_mask, d, NEG))
                    zero = jnp.zeros((64, 64), F32)
                    p_buf[b % 2, slot - (i + 1) - 1, 64:128, :] = jnp.where(col128 >= 64, e, 0.0).astype(BF)
                    p_buf[b % 2, slot - 1, 64:128, :] = jnp.concatenate(
                        [zero, e[:, :64]], axis=1).astype(BF)

        def values(b):
            usemax = b < SPLIT or CFG.get("allmax")
            slot = 0
            for (s, heads, i) in blocks[b]:
                for h in heads:
                    g, j = divmod(h, HPG)
                    m = mx.pop((s, h, i)) if usemax else None
                    o = None
                    for kt in range(i + 1):
                        if usemax:
                            p = jnp.exp2(st.pop((b, slot)) - m).astype(BF)
                        else:
                            p = p_buf[b % 2, slot]
                        r = value_tile(s, g, j, kt, p)
                        o = r if o is None else o + r
                        slot += 1
                    finish_column(s, g, j, i, o, s > 0)

        def proj_tasks(s, groups=range(NG)):
            return [(GW[g] // 16 * 15,
                     lambda s=s, tt=tt, g=g: proj_qkv(s, tt, g, s > 0, s < NSEG - 1))
                    for tt in range(4) for g in groups]

        def out_tasks(s, tts=range(4)):
            tasks = []
            for tt in tts:
                tasks += [(60, lambda s=s, tt=tt, fb=fb: proj_out(s, tt, fb, (s, tt) == (NSEG - 1, 0)))
                          for fb in range(3)]
                tasks.append((0, lambda s=s, tt=tt: out_copy(4 * s + tt).start()))
            return tasks

        def ln_tasks(s):
            ts = range(4 * s, 4 * s + 4)
            return ([(10, lambda t=t: ln_stats(t)) for t in ts]
                    + [(10, lambda t=t: ln_apply(t)) for t in ts]
                    + [(2, lambda t=t: router(t)) for t in ts])

        def upd_tasks(s):
            return [(GW[g] // 4, lambda s=s, g=g: mem_update(s, g, s == 0)) for g in range(NG)]

        def read_tasks(s):
            return [(GW[g] // 4 + 4, lambda s=s, g=g: mem_read(s, g)) for g in range(NG)]

        def prep_tasks(cbs):
            return [(5, lambda cb=cb, which=which: prep_wt(cb, which)) for cb in cbs for which in range(3)]

        guard = {}

        def norm_task(i, cb):
            row = col_norm2(i, cb)
            guard[i] = row if i not in guard else jnp.maximum(guard[i], row)

        seg0 = [min(k for k, blk in enumerate(blocks) if blk[0][0] == s) for s in range(NSEG)] + [nb]
        last = {i: max(k for k, blk in enumerate(blocks) if blk[0][0] == NSEG - 1 and blk[0][2] == i)
                for i in range(4)}

        def at(s, frac):
            lo = SPLIT if s == 0 else seg0[s]
            return lo + round(frac * (seg0[s + 1] - lo))

        a1, a2, a3 = seg0[1], seg0[2], seg0[3]
        streams = [
            (0, 1, prep_tasks((1,))),
            (0, 2, prep_tasks((2,))),
            (1, 4, proj_tasks(0, (1,))),
            (3, 5, prep_tasks((3, 4))),
            (4, min(8, SPLIT + 1), proj_tasks(0, (2,))),
            (CFG.get('ln1', (3, SPLIT))[0], CFG.get('ln1', (3, SPLIT))[1], ln_tasks(1)),
            (0, 3, [(1, lambda i=i, cb=cb: norm_task(i, cb)) for cb in range(3) for i in range(3)]),
            (3, SPLIT - 1, [(1, lambda i=i, cb=cb: norm_task(i, cb)) for cb in (3, 4) for i in range(3)]),
            (min(8, SPLIT), at(0, 0.2), proj_tasks(0, (3, 4))),
            (at(0, CFG.get('p1', 0.1)), a1 - 1, proj_tasks(1)),
            (at(0, 0.3), at(0, 0.5), upd_tasks(0)),
            (a1 - 1, a1, read_tasks(1)),
            (CFG.get('ln23', SPLIT + 1), a1 - 1, ln_tasks(2) + ln_tasks(3)),
            (SPLIT + 1, a1, [(5, lambda g=g: prep_wo(g)) for g in range(NG)]),
            (a1, a1 + 1, [(1, moe_select)]),
            (a1 + 1, at(1, 0.2), upd_tasks(1)),
            (a1, a2 - 1, proj_tasks(2)),
            (a2 - 1, a2, read_tasks(2)),
            (a2 + 1, at(2, 0.2), upd_tasks(2)),
            (a2, a3 - 1, proj_tasks(3)),
            (a3 - 1, a3, read_tasks(3)),
            (a3 - 1, a3, [(1, lambda: (emit_downs(len(downs)), moe_finish()))]),
            (a3 + 1, last[1] + 1, out_tasks(0) + out_tasks(1) + out_tasks(2)),
            (last[3] + 2, last[2] + 1, out_tasks(3, (3,))),
            (last[2] + 2, last[1] + 1, out_tasks(3, (2,))),
            (last[1] + 2, nb + 1, out_tasks(3, (1,))),
        ]
        nf = FF // 128
        micro_ranges = [(a1 + 1, a2 - 1, moe_up_tasks(range(nf // 2))),
                        (a2, a3 - 2, moe_up_tasks(range(nf // 2, nf)))]
        downs = moe_down_tasks(range(nf))
        dstate = [0]

        def emit_downs(limit):
            n = 0
            while dstate[0] < len(downs) and n < limit and ("h", downs[dstate[0]][0]) in moe:
                downs[dstate[0]][1]()
                dstate[0] += 1
                n += 1

        ntiles = [sum(len(u) * (i + 1) for (_, u, i) in blk) for blk in blocks]

        def fence_w12():
            wait_w(1)
            wait_w(2)

        def fence_w34():
            wait_w(3)
            wait_w(4)
            x_copy(1).wait()

        def fence_a1():
            wait_moe(0)
            start_moe(1)

        fences = {0: fence_w12, 3: fence_w34, SPLIT: lambda: start_moe(0), a1: fence_a1,
                  a2: lambda: wait_moe(1), a3: barrier}

        state = [[0, 0.0, float(sum(c for c, _ in t))] for _, _, t in streams]
        mstate = [[0, 0] for _ in micro_ranges]
        cur_scope = []

        def emit(b0, b1):
            for b in range(b0, b1 + 1):
                if _SCOPES and b % 4 == 0:
                    if cur_scope:
                        cur_scope.pop().__exit__(None, None, None)
                    cur_scope.append(jax.named_scope(f"blk{b:03d}"))
                    cur_scope[-1].__enter__()
                if b in fences and b < b1:
                    fences[b]()

                def micro(b=b):
                    for (lo, hi, tasks), ms in zip(micro_ranges, mstate):
                        if lo <= b < hi:
                            ms[0] += 1
                            total = sum(ntiles[lo:hi])
                            while ms[1] < len(tasks) and ms[1] < ms[0] * len(tasks) / total:
                                tasks[ms[1]]()
                                ms[1] += 1

                if b < b1:
                    scores(b, micro)
                if b < b1 or b == nb:
                    for (lo, hi, tasks), st_ in zip(streams, state):
                        if b < lo:
                            continue
                        frac = (b + 1 - lo) / (hi - lo)
                        while st_[0] < len(tasks) and st_[1] + tasks[st_[0]][0] / 2 <= frac * st_[2] + 1e-9:
                            st_[1] += tasks[st_[0]][0]
                            tasks[st_[0]][1]()
                            st_[0] += 1
                            if tasks[st_[0] - 1][0] >= 75 and a1 < b < a3:
                                emit_downs(CFG.get("dper", 5))
                if b > b0:
                    values(b - 1)
            if cur_scope:
                cur_scope.pop().__exit__(None, None, None)

        def fast_rest():
            pace.clear()
            emit(SPLIT, nb)
            for (lo, hi, tasks), st_ in zip(streams, state):
                assert st_[0] == len(tasks), (lo, hi, st_)
            assert all(ms[1] == len(r[2]) for ms, r in zip(mstate, micro_ranges)) and dstate[0] == len(downs)
            with scope("tail0"):
                for _, t in out_tasks(3, (0,)):
                    t()
            with scope("tail1"):
                for t in range(4 * NSEG):
                    out_copy(t).wait()

        emit(0, SPLIT)
        x_copy(2).wait()
        x_copy(3).wait()
        wo_copy.wait()
        nq, nk, nv = (jnp.max(guard[i]) for i in range(3))
        safe = jnp.logical_and(nq * nk <= (SCORE_LIMIT / (1.05 * D * QSCALE * DH)) ** 2, nv <= 1e30)
        if CFG.get("only") == "fast":
            fast_rest()
        elif CFG.get("only") == "compact":
            compact_path()
        else:
            pl.when(safe)(fast_rest)
            pl.when(jnp.logical_not(safe))(compact_path)

    def prep_group(g):
        for which in range(3):
            prep_wt(g, which)

    def wait_w(cb):
        for i in range(3):
            w_copy(i, cb).wait()

    def start_moe(c):
        for i in range(3):
            moe_copy(i, c).start()

    def wait_moe(c):
        for i in range(3):
            moe_copy(i, c).wait()

    def col_norm2(i, cb):
        n = 128 if cb < 4 else 64
        acc = None
        for u in range(D // 64):
            wv = wraw[i, 64 * u:64 * (u + 1), 128 * cb:128 * cb + n].astype(F32)
            c = jnp.sum((wv * wv).reshape(8, 8, n), axis=0)
            acc = c if acc is None else acc + c
        row = jnp.sum(acc, axis=0, keepdims=True)
        if n < 128:
            row = jnp.concatenate([row, jnp.zeros((1, 128 - n), F32)], axis=1)
        return paced(row)

    def scope(name):
        return jax.named_scope(name) if _SCOPES else contextlib.nullcontext()

    with scope("pre0"):
        for s in range(NSEG):
            for g in range(NG):
                n = DH * GN[g]
                for tt in range(4):
                    o_t[s, tt, 128 * g + n:128 * g + GW[g], :] = jnp.zeros((GW[g] - n, 128), BF)
        wr_copy.wait()
        x_copy(0, 0).wait()
        prep_wr()
        layernorm(0)
    with scope("pre1"):
        wait_w(0)
        prep_group(0)
        proj_qkv(0, 0, 0, False, True)
    with scope("pre2"):
        for tt in range(1, 4):
            x_copy(0, tt).wait()
        beta_copy.wait()
        for tt in range(1, 4):
            layernorm(tt)
            proj_qkv(0, tt, 0, False, True)
        prep_gates()
    run_pipeline()


@jax.jit
def pallas_parallel_sum__memory_aug_infini_attn__moe_arch_mod__prompt_kernel(
    A_x: jax.Array,
    A_wq: jax.Array,
    A_wk: jax.Array,
    A_wv: jax.Array,
    A_wo: jax.Array,
    A_beta: jax.Array,
    B_x: jax.Array,
    B_w_r: jax.Array,
    B_w_gate: jax.Array,
    B_w_up: jax.Array,
    B_w_down: jax.Array,
):
    del B_x
    hbm = pl.BlockSpec(memory_space=pltpu.HBM)
    scratch = [
        pltpu.VMEM((D, SEQ), BF),
        pltpu.VMEM((4 * NSEG, D, 128), BF),
        pltpu.VMEM((D, SEQ), F32),
        pltpu.VMEM((16, SEQ), F32),
        pltpu.VMEM((4, D, D), BF),
        pltpu.VMEM((3 * GP, D), BF),
        pltpu.VMEM((D, GP), BF),
        pltpu.VMEM((H,), BF),
        pltpu.VMEM((D,), BF),
        pltpu.VMEM((16, D), BF),
        pltpu.VMEM((D, FF), BF),
        pltpu.VMEM((D, FF), BF),
        pltpu.VMEM((D, FF), BF),
        pltpu.VMEM((NSEG, 4, GP, 128), BF),
        pltpu.VMEM((NSEG, 4, GP, 128), BF),
        pltpu.VMEM((NSEG, 4, GP, 128), BF),
        pltpu.VMEM((NSEG, NG, L, 128), BF),
        pltpu.VMEM((NSEG, 4, GP, 128), BF),
        pltpu.VMEM((NSEG, 4, GP, 128), BF),
        pltpu.VMEM((2, 20, 128, 128), BF),
        pltpu.VMEM((NSEG, GP, L), F32),
        pltpu.VMEM((NSEG, 16 * NG, L), F32),
        pltpu.VMEM((NG, 128, 128), F32),
        pltpu.VMEM((1, SEQ), F32),
        pltpu.VMEM((NG, 8, 128), F32),
        pltpu.VMEM((16, D), F32),
        pltpu.VMEM((4 * NSEG, D, 128), BF),
        pltpu.SemaphoreType.DMA((25,)),
        pltpu.SemaphoreType.DMA((3 * (FF // MOE_DMA),)),
        pltpu.SemaphoreType.DMA((4 * NSEG,)),
        pltpu.SemaphoreType.REGULAR,
    ]
    out_t = pl.pallas_call(
        _kernel,
        out_shape=jax.ShapeDtypeStruct((1, D, SEQ), BF),
        in_specs=[hbm] * 10,
        out_specs=hbm,
        scratch_shapes=scratch,
        compiler_params=pltpu.CompilerParams(vmem_limit_bytes=100 * 1024 * 1024),
    )(jnp.swapaxes(A_x, 1, 2), A_wq, A_wk, A_wv, A_wo, A_beta, B_w_r, B_w_gate, B_w_up,
      B_w_down.T)
    return jnp.swapaxes(out_t, 1, 2)
```

```python
import contextlib
import json
import os

import jax
import jax.numpy as jnp
from jax import lax
import jax.experimental.pallas as pl
import jax.experimental.pallas.tpu as pltpu

BF = jnp.bfloat16
F32 = jnp.float32

SEQ, D, H, DH = 2048, 576, 32, 18
NSEG, L, FF = 4, 512, 4608
HPG = 7
NG = 5
GN = (7, 7, 7, 7, 4)
GW = (128, 128, 128, 128, 80)
GP = 592
ZR = (126, 126, 126, 126, 78)
QSCALE = (DH ** -0.5) * 1.4426950408889634
NT_DIMS = (((1,), (1,)), ((), ()))
MOE_DMA = 2304
NEG = -1e30
SPLIT = int(os.environ.get('KSPLIT', 9))
SCORE_LIMIT = 40.0
_SCOPES = os.environ.get("KSCOPES", "") == "1"
CFG = dict()
CFG.update(json.loads(os.environ.get("KCFG", "{}")))


def _dot(a, b):
    return jnp.dot(a, b, preferred_element_type=F32)


def _dot_nt(a, b):
    return lax.dot_general(a, b, NT_DIMS, preferred_element_type=F32)


def _iota(shape, dim):
    return lax.broadcasted_iota(jnp.int32, shape, dim)


def _phi(t):
    return jnp.where(t > 0, t + 1.0, jnp.exp(t))


def _sigmoid(t):
    return 1.0 / (1.0 + jnp.exp(-t))


def _recip(x):
    r = pl.reciprocal(x, approx=True)
    r = r * (2.0 - x * r)
    return r * (2.0 - x * r)


def _div18(i):
    return (i * 57) >> 10


def _blk(t, size=128):
    if isinstance(t, int):
        return slice(size * t, size * (t + 1))
    return pl.ds(pl.multiple_of(t * size, size), size)


def _rows(start, size, align):
    if isinstance(start, int):
        return slice(start, start + size)
    return pl.ds(pl.multiple_of(start, align), size)


def _colsum(a):
    return jnp.sum(jnp.sum(a.reshape(a.shape[0] // 8, 8, a.shape[1]), axis=0), axis=0, keepdims=True)


def _kernel(x_hbm, wq_hbm, wk_hbm, wv_hbm, wo_hbm, beta_hbm, wr_hbm, wg_hbm, wu_hbm, wd_hbm,
            out_hbm,
            x_v, xn_v, res_v, stat_v, wraw, w_t, wo_t, beta_v, wr_v, wr_b, wg_v, wu_v, wd_v,
            q_t, pq_t, v_t, k_n, pk_t, o_t, p_buf, am_t, den_t, m_t, r_row, gate_t, moe_y, out_v,
            sem_in, sem_moe, sem_out, sem_bar):

    def x_copy(s, tt=None):
        if tt is None:
            c0, n, k = s * L, L, 3 + s
        else:
            c0, n, k = tt * 128, 128, tt
        return pltpu.make_async_copy(x_hbm.at[0, :, pl.ds(c0, n)], x_v.at[:, pl.ds(c0, n)],
                                     sem_in.at[k])

    def w_copy(i, cb):
        src = (wq_hbm, wk_hbm, wv_hbm)[i]
        n = 128 if cb < 4 else 64
        return pltpu.make_async_copy(src.at[:, pl.ds(128 * cb, n)], wraw.at[i, :, pl.ds(128 * cb, n)],
                                     sem_in.at[7 + 5 * i + cb])

    wo_copy = pltpu.make_async_copy(wo_hbm, wraw.at[3], sem_in.at[22])
    beta_copy = pltpu.make_async_copy(beta_hbm, beta_v, sem_in.at[23])
    wr_copy = pltpu.make_async_copy(wr_hbm, wr_v, sem_in.at[24])
    NMC = FF // MOE_DMA

    def moe_copy(i, c):
        src, dst = ((wg_hbm, wg_v), (wu_hbm, wu_v), (wd_hbm, wd_v))[i]
        cs = pl.ds(c * MOE_DMA, MOE_DMA)
        return pltpu.make_async_copy(src.at[:, cs], dst.at[:, cs], sem_moe.at[i * NMC + c])

    def out_copy(t):
        cs = pl.ds(t * 128 if isinstance(t, int) else pl.multiple_of(t * 128, 128), 128)
        return pltpu.make_async_copy(out_v.at[t], out_hbm.at[0, :, cs], sem_out.at[t])

    wr_copy.start()
    x_copy(0, 0).start()
    for i in range(3):
        w_copy(i, 0).start()
    beta_copy.start()
    for tt in range(1, 4):
        x_copy(0, tt).start()
    for cb in range(1, 5):
        for i in range(3):
            w_copy(i, cb).start()
    x_copy(1).start()
    x_copy(2).start()
    x_copy(3).start()
    wo_copy.start()

    pace = {}

    def paced(row, lanes=128):
        tok = pace.get("tok")
        return row if tok is None else row + tok[:, :lanes] * 0.0

    def ln_stats(t):
        cols = _blk(t)
        shift = paced(x_v[0:16, cols].astype(F32)[0:1])
        s1 = [None] * 2
        s2 = [None] * 2
        for u in range(D // 16):
            d = x_v[16 * u:16 * (u + 1), cols].astype(F32) - shift
            d = d.reshape(2, 8, 128)
            for k in range(2):
                s1[k] = d[k] if u == 0 else s1[k] + d[k]
                s2[k] = d[k] * d[k] if u == 0 else s2[k] + d[k] * d[k]
        m1 = jnp.sum(s1[0] + s1[1], axis=0, keepdims=True) * (1.0 / D)
        m2 = jnp.sum(s2[0] + s2[1], axis=0, keepdims=True) * (1.0 / D)
        var = jnp.maximum(m2 - m1 * m1, 0.0)
        stat_v[0:1, cols] = m1 + shift
        stat_v[8:9, cols] = lax.rsqrt(var + 1e-5)

    def ln_apply(t):
        cols = _blk(t)
        mean = paced(stat_v[0:1, cols])
        rstd = stat_v[8:9, cols]
        for u in range(D // 48):
            rows = slice(48 * u, 48 * (u + 1))
            x = x_v[rows, cols].astype(F32)
            xn = (x - mean) * rstd
            xn_v[t, rows, :] = xn.astype(BF)
            res_v[rows, cols] = x + xn

    def router(t):
        r = _dot(wr_b[...], xn_v[t])
        r_row[:, _blk(t)] = r[0:1].astype(BF).astype(F32)

    def layernorm(t):
        ln_stats(t)
        ln_apply(t)
        router(t)

    def prep_wr():
        wr = wr_v[...].reshape(1, D)
        wr_b[...] = jnp.broadcast_to(wr.astype(F32), (16, D)).astype(BF)

    def prep_wt(cb, which):
        nb = 128 if cb < 4 else 64
        n = DH * GN[cb]
        t = wraw[which, :, 128 * cb:128 * cb + nb].T
        r0 = 384 * cb + which * GW[cb]
        k = min(n - 2 * cb, nb)
        w_t[r0 + 2 * cb:r0 + 2 * cb + k, :] = t[0:k]
        w_t[r0 + n:r0 + GW[cb], :] = jnp.zeros((GW[cb] - n, D), BF)
        if cb < 4:
            r1 = 384 * (cb + 1) + which * GW[cb + 1]
            w_t[r1:r1 + 2 * (cb + 1), :] = t[128 - 2 * (cb + 1):128]

    def prep_wo(g):
        n = DH * GN[g]
        wo_t[:, 128 * g:128 * g + n] = wraw[3, 126 * g:126 * g + n, :].T
        wo_t[:, 128 * g + n:128 * g + GW[g]] = jnp.zeros((D, GW[g] - n), BF)

    def prep_gates():
        b = beta_v[...].astype(F32).reshape(1, H)
        sig = jnp.concatenate([_sigmoid(b), jnp.zeros((1, 128 - H), F32)], axis=1)
        rows = jnp.broadcast_to(sig, (128, 128)).T
        for g in range(NG):
            gate_t[g] = rows[HPG * g:HPG * g + 8]

    def proj_qkv(s, tt, g, need_pq=True, need_pk=True):
        w = GW[g]
        rows = slice(128 * g, 128 * g + w)
        r = _dot(w_t[384 * g:384 * g + 3 * w, :], xn_v[4 * s + tt])
        q, k, v = r[:w], r[w:2 * w], r[2 * w:]
        q_t[s, tt, rows, :] = (q * QSCALE).astype(BF)
        if need_pq:
            pq_t[s, tt, rows, :] = _phi(q).astype(BF)
        k_n[s, g, _blk(tt), :w] = k.astype(BF).T
        if need_pk:
            pk_t[s, tt, rows, :] = _phi(k).astype(BF)
        v = jnp.where(_iota((w, 128), 0) == ZR[g], 1.0, v)
        v_t[s, tt, rows, :] = v.astype(BF)

    def mem_update(s, g, first):
        w = GW[g]
        rows = slice(128 * g, 128 * g + w)
        r = _dot_nt(v_t[s, 0, rows, :], pk_t[s, 0, rows, :])
        for tt in range(1, 4):
            r = r + _dot_nt(v_t[s, tt, rows, :], pk_t[s, tt, rows, :])
        rr, cc = _iota((w, w), 0), _iota((w, w), 1)
        keep = (cc < DH * GN[g]) & ((_div18(rr) == _div18(cc)) | (rr == ZR[g]))
        r = jnp.where(keep, r, 0.0)
        if not first:
            r = r + m_t[g, :w, :w]
        m_t[g, :w, :w] = r

    def mem_read(s, g):
        w = GW[g]
        rows = slice(128 * g, 128 * g + w)
        m = m_t[g, :w, :w]
        z = m[ZR[g]:ZR[g] + 1, :]
        zrows = jnp.where(_iota((16, w), 0) == _div18(_iota((16, w), 1)), z, 0.0)
        lhs = jnp.concatenate([m, zrows], axis=0).astype(BF)
        for tt in range(4):
            cols = slice(128 * tt, 128 * (tt + 1))
            r = _dot(lhs, pq_t[s, tt, rows, :])
            am_t[s, rows, cols] = r[:w]
            den_t[s, 16 * g:16 * (g + 1), cols] = r[w:]

    def proj_out(s, tt, fb, by_group=False):
        f0 = 192 * fb
        f1 = f0 + 192
        if by_group:
            p = None
            for g in range(NG):
                r = _dot(wo_t[f0:f1, 128 * g:128 * g + GW[g]], o_t[s, tt, 128 * g:128 * g + GW[g], :])
                p = r if p is None else p + r
        else:
            p = _dot(wo_t[f0:f1, :], o_t[s, tt])
        out_v[4 * s + tt, f0:f1, :] = (p + res_v[f0:f1, _blk(4 * s + tt)]).astype(BF)

    moe = {}

    def moe_select():
        r = r_row[...]
        io = _iota((1, SEQ), 1)
        m1 = jnp.max(r)
        i1 = jnp.min(jnp.where(r == m1, io, SEQ - 1))
        r2 = jnp.where(io == i1, -jnp.inf, r)
        m2 = jnp.max(r2)
        i2 = jnp.min(jnp.where((r2 == m2) & (io != i1), io, SEQ - 1))
        rows = []
        for i in (i1, i2):
            xb = xn_v[i // 128].T.astype(F32)
            rows.append(jnp.sum(jnp.where(_iota((128, D), 0) == i % 128, xb, 0.0), axis=0, keepdims=True))
        rr = _iota((16, D), 0)
        xs = jnp.where(rr == 0, rows[0], jnp.where(rr == 1, rows[1], 0.0))
        moe["x"] = xs.astype(BF)
        moe["w"] = _sigmoid(jnp.where(_iota((16, 1), 0) == 0, m1, m2))
        sel = jnp.where(_iota((2, 128), 0) == 0, i1, i2)
        for t in range(4 * NSEG):
            tok = _iota((2, 128), 1) + 128 * t
            o_t[t // 4, t % 4, 126:128, :] = jnp.where(tok == sel, 1.0, 0.0).astype(BF)

    KTS = [(128 * k, min(128 * (k + 1), D)) for k in range(5)]

    def moe_up(name, ref, f, k):
        k0, k1 = KTS[k]
        r = _dot(moe["x"][:, k0:k1], ref[k0:k1, _blk(f)])
        moe[name] = r if k == 0 else moe[name] + r

    def moe_hidden(f):
        g = moe["g"]
        moe[("h", f if isinstance(f, int) else 0)] = (g * _sigmoid(g) * moe["u"]).astype(BF)

    def moe_down(f, n, first):
        n0, n1 = KTS[n]
        r = _dot_nt(moe[("h", f if isinstance(f, int) else 0)], wd_v[n0:n1, _blk(f)])
        moe[("y", n)] = r if first else moe[("y", n)] + r

    def moe_up_tasks(fs):
        tasks = []
        for f in fs:
            tasks += [lambda f=f, k=k: moe_up("g", wg_v, f, k) for k in range(5)]
            tasks += [lambda f=f, k=k: moe_up("u", wu_v, f, k) for k in range(4)]
            tasks.append(lambda f=f: (moe_up("u", wu_v, f, 4), moe_hidden(f)))
        return tasks

    def moe_down_tasks(fs):
        return [(f, lambda f=f, n=n: moe_down(f, n, f == 0)) for f in fs for n in range(5)]

    def moe_finish():
        y = jnp.concatenate([moe[("y", n)] for n in range(5)], axis=1) * moe["w"]
        rr = _iota((128, D), 0)
        ypad = jnp.where(rr == 126, y[0:1], jnp.where(rr == 127, y[1:2], 0.0))
        cur = wo_t[:, 0:128].astype(F32)
        wo_t[:, 0:128] = jnp.where(_iota((D, 128), 1) >= 126, ypad.T, cur).astype(BF)

    causal = _iota((128, 128), 0) <= _iota((128, 128), 1)
    wrow = _iota((32, 128), 0)

    def barrier():
        pl.semaphore_signal(sem_bar, 1)
        pl.semaphore_wait(sem_bar, 1)

    def query_weights(s, g, j, i, w):
        wq = q_t[s, i, _rows(128 * g + 16 * j, 32, 16), :]
        wq = jnp.where((wrow >= 2 * j) & (wrow < 2 * j + DH), wq, jnp.zeros_like(wq))
        parts = [wq]
        if j > 0:
            parts.insert(0, jnp.zeros((16 * j, 128), BF))
        if w - 16 * j - 32 > 0:
            parts.append(jnp.zeros((w - 16 * j - 32, 128), BF))
        return jnp.concatenate(parts, axis=0) if len(parts) > 1 else wq

    def score_tile(s, g, i, kt, w, wq):
        d = _dot(k_n[s, g, 128 * kt:128 * (kt + 1), :w], wq)
        return jnp.where(causal, d, NEG) if kt == i else d

    def value_tile(s, g, j, kt, p):
        v = v_t[s, kt, _rows(128 * g + 16 * j, 32, 16), :]
        return _dot(jnp.where(wrow >= 30, jnp.ones_like(v), v), p)

    def finish_column(s, g, j, i, o, with_mem):
        cols = slice(128 * i, 128 * (i + 1))
        win = _rows(128 * g + 16 * j, 32, 16)
        gate = gate_t[g][j:j + 1]
        scale = (1.0 - gate) * _recip(o[31:32, :])
        if isinstance(g, int) and CFG.get("pace", 1):
            pace["tok"] = scale
        o = o * scale
        if with_mem:
            den = den_t[s, _rows(16 * g, 16, 16), cols][j:j + 1] + 1e-6
            o = o + am_t[s, win, cols] * (gate * _recip(den))
        if isinstance(g, int):
            r0 = 128 * g + DH * j
            o_t[s, i, r0:r0 + DH, :] = o[2 * j:2 * j + DH].astype(BF)
        else:
            mine = (wrow >= 2 * j) & (wrow < 2 * j + DH)
            o_t[s, i, win, :] = jnp.where(mine, o, o_t[s, i, win, :].astype(F32)).astype(BF)

    def running_max(m, d):
        pm = jnp.max(d.reshape(16, 8, 128), axis=0)
        return pm if m is None else jnp.maximum(m, pm)

    def compact_path():
        pace.clear()
        for c in range(NMC):
            start_moe(c)
        for g in range(NG):
            prep_wo(g)
            m_t[g] = jnp.zeros((128, 128), F32)
        am_t[0] = jnp.zeros((GP, L), F32)
        den_t[0] = jnp.ones((16 * NG, L), F32)

        @pl.loop(0, 4 * NSEG)
        def _(t):
            layernorm(t)

        for c in range(NMC):
            wait_moe(c)
        moe_select()

        def expert(f, y):
            for k in range(5):
                moe_up("g", wg_v, f, k)
            for k in range(5):
                moe_up("u", wu_v, f, k)
            moe_hidden(f)
            for n in range(5):
                moe[("y", n)] = y[n]
                moe_down(f, n, False)
            return tuple(moe[("y", n)] for n in range(5))

        y = lax.fori_loop(0, FF // 128, expert,
                          tuple(jnp.zeros((16, k1 - k0), F32) for k0, k1 in KTS))
        for n in range(5):
            moe[("y", n)] = y[n]
        moe_finish()

        def head(s, g, j, w):
            for i in range(4):
                wq = query_weights(s, g, j, i, w)
                tiles, m = [], None
                for kt in range(i + 1):
                    tiles.append(score_tile(s, g, i, kt, w, wq))
                    m = running_max(m, tiles[-1])
                m = jnp.max(m, axis=0, keepdims=True)
                o = None
                for kt in range(i + 1):
                    r = value_tile(s, g, j, kt, jnp.exp2(tiles[kt] - m).astype(BF))
                    o = r if o is None else o + r
                finish_column(s, g, j, i, o, True)
                pace.clear()

        @pl.loop(0, NSEG)
        def _(s):
            @pl.loop(0, 4)
            def _(tt):
                for g in range(NG):
                    proj_qkv(s, tt, g)

            @pl.when(s > 0)
            def _():
                for g in range(NG):
                    mem_read(s, g)

            @pl.loop(0, NG - 1)
            def _(g):
                for j in range(HPG):
                    head(s, g, j, 128)

            for j in range(GN[NG - 1]):
                head(s, NG - 1, j, GW[NG - 1])
            for g in range(NG):
                mem_update(s, g, False)

            @pl.loop(0, 4)
            def _(tt):
                for fb in range(3):
                    proj_out(s, tt, fb)
                out_copy(4 * s + tt).start()
                out_copy(4 * s + tt).wait()

    def head_units(first_head):
        units, h = [], first_head
        while h < H:
            g, j = divmod(h, HPG)
            if j + 1 < GN[g]:
                units.append((h, h + 1))
                h += 2
            else:
                units.append((h,))
                h += 1
        return units

    def make_blocks():
        blocks = [[(0, (h,), i) for i in range(4)] for h in range(SPLIT)]
        for s in range(NSEG - 1):
            blocks += [[(s, u, i) for i in range(4)] for u in head_units(SPLIT if s == 0 else 0)]
        s = NSEG - 1
        for i, budget in ((3, 16), (2, 18), (1, 20), (0, 20)):
            cur, n = [], 0
            for u in head_units(0):
                cost = len(u) * (i + 1)
                if cur and (n + cost > budget or (i == 0 and u[0] % HPG == 0)):
                    blocks.append(cur)
                    cur, n = [], 0
                cur.append((s, u, i))
                n += cost
            blocks.append(cur)
        return blocks

    col128 = _iota((64, 128), 1)
    mix_mask = _iota((64, 128), 0) <= (col128 & 63)

    def run_pipeline():
        blocks = make_blocks()
        nb = len(blocks)
        st, mx = {}, {}

        def scores(b, micro):
            usemax = b < SPLIT or CFG.get("allmax")
            slot = 0
            for (s, heads, i) in blocks[b]:
                g = heads[0] // HPG
                w = GW[g]
                wqs = [query_weights(s, g, h % HPG, i, w) for h in heads]
                paired = len(heads) == 2 and not usemax and not CFG.get("nopair")
                for n, h in enumerate(heads):
                    m = None
                    for kt in range(i + 1):
                        if paired and kt == i:
                            d = _dot(k_n[s, g, 128 * kt:128 * kt + 64, :w], wqs[n])
                            micro()
                            p_buf[b % 2, slot, 0:64, :] = jnp.exp2(
                                jnp.where(causal[:64], d, NEG)).astype(BF)
                            slot += 1
                            continue
                        d = score_tile(s, g, i, kt, w, wqs[n])
                        micro()
                        if usemax:
                            st[(b, slot)] = d
                            m = running_max(m, d)
                        else:
                            p_buf[b % 2, slot] = jnp.exp2(d).astype(BF)
                        slot += 1
                    if usemax:
                        mx[(s, h, i)] = jnp.max(m, axis=0, keepdims=True)
                if paired:
                    wmix = jnp.concatenate([wqs[1][:, 64:], wqs[0][:, 64:]], axis=1)
                    d = _dot(k_n[s, g, 128 * i + 64:128 * (i + 1), :w], wmix)
                    e = jnp.exp2(jnp.where(mix_mask, d, NEG))
                    zero = jnp.zeros((64, 64), F32)
                    p_buf[b % 2, slot - (i + 1) - 1, 64:128, :] = jnp.where(col128 >= 64, e, 0.0).astype(BF)
                    p_buf[b % 2, slot - 1, 64:128, :] = jnp.concatenate(
                        [zero, e[:, :64]], axis=1).astype(BF)

        def values(b):
            usemax = b < SPLIT or CFG.get("allmax")
            slot = 0
            for (s, heads, i) in blocks[b]:
                for h in heads:
                    g, j = divmod(h, HPG)
                    m = mx.pop((s, h, i)) if usemax else None
                    o = None
                    for kt in range(i + 1):
                        if usemax:
                            p = jnp.exp2(st.pop((b, slot)) - m).astype(BF)
                        else:
                            p = p_buf[b % 2, slot]
                        r = value_tile(s, g, j, kt, p)
                        o = r if o is None else o + r
                        slot += 1
                    finish_column(s, g, j, i, o, s > 0)

        def proj_tasks(s, groups=range(NG)):
            return [(GW[g] // 16 * 15,
                     lambda s=s, tt=tt, g=g: proj_qkv(s, tt, g, s > 0, s < NSEG - 1))
                    for tt in range(4) for g in groups]

        def out_tasks(s, tts=range(4)):
            tasks = []
            for tt in tts:
                tasks += [(60, lambda s=s, tt=tt, fb=fb: proj_out(s, tt, fb, (s, tt) == (NSEG - 1, 0)))
                          for fb in range(3)]
                tasks.append((0, lambda s=s, tt=tt: out_copy(4 * s + tt).start()))
            return tasks

        def ln_tasks(s):
            ts = range(4 * s, 4 * s + 4)
            return ([(10, lambda t=t: ln_stats(t)) for t in ts]
                    + [(10, lambda t=t: ln_apply(t)) for t in ts]
                    + [(2, lambda t=t: router(t)) for t in ts])

        def upd_tasks(s):
            return [(GW[g] // 4, lambda s=s, g=g: mem_update(s, g, s == 0)) for g in range(NG)]

        def read_tasks(s):
            return [(GW[g] // 4 + 4, lambda s=s, g=g: mem_read(s, g)) for g in range(NG)]

        def prep_tasks(cbs):
            return [(5, lambda cb=cb, which=which: prep_wt(cb, which)) for cb in cbs for which in range(3)]

        guard = {}

        def norm_task(i, cb, part):
            acc = col_norm2(i, cb, part)
            if part > 0:
                acc = acc + guard[("acc", i)]
            else:
                acc = acc + paced(jnp.zeros((1, acc.shape[1]), F32), acc.shape[1])
            guard[("acc", i)] = acc
            if part == 2:
                row = jnp.sum(acc, axis=0, keepdims=True)
                if row.shape[1] < 128:
                    row = jnp.concatenate([row, jnp.zeros((1, 128 - row.shape[1]), F32)], axis=1)
                guard[i] = row if i not in guard else jnp.maximum(guard[i], row)

        def guard_task():
            nq, nk, nv = (jnp.max(guard[i]) for i in range(3))
            guard["safe"] = jnp.logical_and(
                nq * nk <= (SCORE_LIMIT / (1.05 * D * QSCALE * DH)) ** 2, nv <= 1e30)

        def norm_tasks(cbs):
            return [(1, lambda i=i, cb=cb, part=part: norm_task(i, cb, part))
                    for cb in cbs for i in range(3) for part in range(3)]

        seg0 = [min(k for k, blk in enumerate(blocks) if blk[0][0] == s) for s in range(NSEG)] + [nb]
        last = {i: max(k for k, blk in enumerate(blocks) if blk[0][0] == NSEG - 1 and blk[0][2] == i)
                for i in range(4)}

        def at(s, frac):
            lo = SPLIT if s == 0 else seg0[s]
            return lo + round(frac * (seg0[s + 1] - lo))

        a1, a2, a3 = seg0[1], seg0[2], seg0[3]
        streams = [
            (0, 1, prep_tasks((1,))),
            (0, 2, prep_tasks((2,))),
            (1, 4, proj_tasks(0, (1,))),
            (3, 5, prep_tasks((3, 4))),
            (4, min(8, SPLIT + 1), proj_tasks(0, (2,))),
            (CFG.get('ln1', (3, SPLIT))[0], CFG.get('ln1', (3, SPLIT))[1], ln_tasks(1)),
            (-1, 0, norm_tasks((0,))),
            (0, 3, norm_tasks((1, 2))),
            (3, SPLIT - 3, norm_tasks((3, 4))),
            (SPLIT - 3, SPLIT - 2, [(1, guard_task)]),
            (min(8, SPLIT), at(0, 0.2), proj_tasks(0, (3, 4))),
            (at(0, CFG.get('p1', 0.1)), a1 - 1, proj_tasks(1)),
            (at(0, 0.3), at(0, 0.5), upd_tasks(0)),
            (a1 - 1, a1, read_tasks(1)),
            (CFG.get('ln23', SPLIT + 1), a1 - 1, ln_tasks(2) + ln_tasks(3)),
            (SPLIT + 1, a1, [(5, lambda g=g: prep_wo(g)) for g in range(NG)]),
            (a1, a1 + 1, [(1, moe_select)]),
            (a1 + 1, at(1, 0.2), upd_tasks(1)),
            (a1, a2 - 1, proj_tasks(2)),
            (a2 - 1, a2, read_tasks(2)),
            (a2 + 1, at(2, 0.2), upd_tasks(2)),
            (a2, a3 - 1, proj_tasks(3)),
            (a3 - 1, a3, read_tasks(3)),
            (a3 - 1, a3, [(1, lambda: (emit_downs(len(downs)), moe_finish()))]),
            (a3 + 1, last[1] + 1, out_tasks(0) + out_tasks(1) + out_tasks(2)),
            (last[3] + 2, last[2] + 1, out_tasks(3, (3,))),
            (last[2] + 2, last[1] + 1, out_tasks(3, (2,))),
            (last[1] + 2, nb + 1, out_tasks(3, (1,))),
        ]
        nf = FF // 128
        micro_ranges = [(a1 + 1, a2 - 1, moe_up_tasks(range(nf // 2))),
                        (a2, a3 - 2, moe_up_tasks(range(nf // 2, nf)))]
        downs = moe_down_tasks(range(nf))
        dstate = [0]

        def emit_downs(limit):
            n = 0
            while dstate[0] < len(downs) and n < limit and ("h", downs[dstate[0]][0]) in moe:
                downs[dstate[0]][1]()
                dstate[0] += 1
                n += 1

        ntiles = [sum(len(u) * (i + 1) for (_, u, i) in blk) for blk in blocks]

        def fence_w12():
            wait_w(1)
            wait_w(2)

        def fence_w34():
            wait_w(3)
            wait_w(4)
            x_copy(1).wait()

        def fence_a1():
            wait_moe(0)
            start_moe(1)

        fences = {0: fence_w12, 3: fence_w34, SPLIT: lambda: start_moe(0), a1: fence_a1,
                  a2: lambda: wait_moe(1)}

        state = [[0, 0.0, float(sum(c for c, _ in t))] for _, _, t in streams]
        mstate = [[0, 0] for _ in micro_ranges]
        cur_scope = []

        def emit(b0, b1):
            for b in range(b0, b1 + 1):
                if _SCOPES and b % 4 == 0:
                    if cur_scope:
                        cur_scope.pop().__exit__(None, None, None)
                    cur_scope.append(jax.named_scope(f"blk{b:03d}"))
                    cur_scope[-1].__enter__()
                if b in fences and b < b1:
                    fences[b]()

                def micro(b=b):
                    for (lo, hi, tasks), ms in zip(micro_ranges, mstate):
                        if lo <= b < hi:
                            ms[0] += 1
                            total = sum(ntiles[lo:hi])
                            while ms[1] < len(tasks) and ms[1] < ms[0] * len(tasks) / total:
                                tasks[ms[1]]()
                                ms[1] += 1

                if b < b1:
                    scores(b, micro)
                if b < b1 or b == nb:
                    for (lo, hi, tasks), st_ in zip(streams, state):
                        if b < lo:
                            continue
                        frac = (b + 1 - lo) / (hi - lo)
                        while st_[0] < len(tasks) and st_[1] + tasks[st_[0]][0] / 2 <= frac * st_[2] + 1e-9:
                            st_[1] += tasks[st_[0]][0]
                            tasks[st_[0]][1]()
                            st_[0] += 1
                            if tasks[st_[0] - 1][0] >= 75 and a1 < b < a3:
                                emit_downs(CFG.get("dper", 5))
                if b > b0:
                    values(b - 1)
            if cur_scope:
                cur_scope.pop().__exit__(None, None, None)

        def fast_rest():
            pace.clear()
            emit(SPLIT, nb)
            for (lo, hi, tasks), st_ in zip(streams, state):
                assert st_[0] == len(tasks), (lo, hi, st_)
            assert all(ms[1] == len(r[2]) for ms, r in zip(mstate, micro_ranges)) and dstate[0] == len(downs)
            with scope("tail0"):
                for _, t in out_tasks(3, (0,)):
                    t()
            with scope("tail1"):
                for t in range(4 * NSEG):
                    out_copy(t).wait()

        for (lo, hi, tasks), st_ in zip(streams, state):
            if lo < 0:
                for _, t in tasks:
                    t()
                st_[0] = len(tasks)
        emit(0, SPLIT)
        x_copy(2).wait()
        x_copy(3).wait()
        wo_copy.wait()
        safe = guard["safe"]
        if CFG.get("only") == "fast":
            fast_rest()
        elif CFG.get("only") == "compact":
            compact_path()
        else:
            pl.when(safe)(fast_rest)
            pl.when(jnp.logical_not(safe))(compact_path)

    def prep_group(g):
        for which in range(3):
            prep_wt(g, which)

    def wait_w(cb):
        for i in range(3):
            w_copy(i, cb).wait()

    def start_moe(c):
        for i in range(3):
            moe_copy(i, c).start()

    def wait_moe(c):
        for i in range(3):
            moe_copy(i, c).wait()

    def col_norm2(i, cb, part):
        n = 128 if cb < 4 else 64
        acc = None
        for u in range(3 * part, 3 * part + 3):
            wv = wraw[i, 64 * u:64 * (u + 1), 128 * cb:128 * cb + n].astype(F32)
            c = jnp.sum((wv * wv).reshape(8, 8, n), axis=0)
            acc = c if acc is None else acc + c
        return acc

    def scope(name):
        return jax.named_scope(name) if _SCOPES else contextlib.nullcontext()

    with scope("pre0"):
        for s in range(NSEG):
            for g in range(NG):
                n = DH * GN[g]
                for tt in range(4):
                    o_t[s, tt, 128 * g + n:128 * g + GW[g], :] = jnp.zeros((GW[g] - n, 128), BF)
        wr_copy.wait()
        x_copy(0, 0).wait()
        prep_wr()
        layernorm(0)
    with scope("pre1"):
        wait_w(0)
        prep_group(0)
        proj_qkv(0, 0, 0, False, True)
    with scope("pre2"):
        for tt in range(1, 4):
            x_copy(0, tt).wait()
        beta_copy.wait()
        for tt in range(1, 4):
            layernorm(tt)
            proj_qkv(0, tt, 0, False, True)
        prep_gates()
    run_pipeline()


@jax.jit
def pallas_parallel_sum__memory_aug_infini_attn__moe_arch_mod__prompt_kernel(
    A_x: jax.Array,
    A_wq: jax.Array,
    A_wk: jax.Array,
    A_wv: jax.Array,
    A_wo: jax.Array,
    A_beta: jax.Array,
    B_x: jax.Array,
    B_w_r: jax.Array,
    B_w_gate: jax.Array,
    B_w_up: jax.Array,
    B_w_down: jax.Array,
):
    del B_x
    hbm = pl.BlockSpec(memory_space=pltpu.HBM)
    scratch = [
        pltpu.VMEM((D, SEQ), BF),
        pltpu.VMEM((4 * NSEG, D, 128), BF),
        pltpu.VMEM((D, SEQ), F32),
        pltpu.VMEM((16, SEQ), F32),
        pltpu.VMEM((4, D, D), BF),
        pltpu.VMEM((3 * GP, D), BF),
        pltpu.VMEM((D, GP), BF),
        pltpu.VMEM((H,), BF),
        pltpu.VMEM((D,), BF),
        pltpu.VMEM((16, D), BF),
        pltpu.VMEM((D, FF), BF),
        pltpu.VMEM((D, FF), BF),
        pltpu.VMEM((D, FF), BF),
        pltpu.VMEM((NSEG, 4, GP, 128), BF),
        pltpu.VMEM((NSEG, 4, GP, 128), BF),
        pltpu.VMEM((NSEG, 4, GP, 128), BF),
        pltpu.VMEM((NSEG, NG, L, 128), BF),
        pltpu.VMEM((NSEG, 4, GP, 128), BF),
        pltpu.VMEM((NSEG, 4, GP, 128), BF),
        pltpu.VMEM((2, 20, 128, 128), BF),
        pltpu.VMEM((NSEG, GP, L), F32),
        pltpu.VMEM((NSEG, 16 * NG, L), F32),
        pltpu.VMEM((NG, 128, 128), F32),
        pltpu.VMEM((1, SEQ), F32),
        pltpu.VMEM((NG, 8, 128), F32),
        pltpu.VMEM((16, D), F32),
        pltpu.VMEM((4 * NSEG, D, 128), BF),
        pltpu.SemaphoreType.DMA((25,)),
        pltpu.SemaphoreType.DMA((3 * (FF // MOE_DMA),)),
        pltpu.SemaphoreType.DMA((4 * NSEG,)),
        pltpu.SemaphoreType.REGULAR,
    ]
    out_t = pl.pallas_call(
        _kernel,
        out_shape=jax.ShapeDtypeStruct((1, D, SEQ), BF),
        in_specs=[hbm] * 10,
        out_specs=hbm,
        scratch_shapes=scratch,
        compiler_params=pltpu.CompilerParams(vmem_limit_bytes=100 * 1024 * 1024),
    )(jnp.swapaxes(A_x, 1, 2), A_wq, A_wk, A_wv, A_wo, A_beta, B_w_r, B_w_gate, B_w_up,
      B_w_down.T)
    return jnp.swapaxes(out_t, 1, 2)
```

```python
import contextlib
import json
import os

import jax
import jax.numpy as jnp
from jax import lax
import jax.experimental.pallas as pl
import jax.experimental.pallas.tpu as pltpu

BF = jnp.bfloat16
F32 = jnp.float32

SEQ, D, H, DH = 2048, 576, 32, 18
NSEG, L, FF = 4, 512, 4608
HPG = 7
NG = 5
GN = (7, 7, 7, 7, 4)
GW = (128, 128, 128, 128, 80)
GP = 592
ZR = (126, 126, 126, 126, 78)
QSCALE = (DH ** -0.5) * 1.4426950408889634
NT_DIMS = (((1,), (1,)), ((), ()))
MOE_DMA = 2304
NEG = -1e30
SPLIT = int(os.environ.get('KSPLIT', 9))
SCORE_LIMIT = 40.0
_SCOPES = os.environ.get("KSCOPES", "") == "1"
CFG = dict()
CFG.update(json.loads(os.environ.get("KCFG", "{}")))


def _dot(a, b):
    return jnp.dot(a, b, preferred_element_type=F32)


def _dot_nt(a, b):
    return lax.dot_general(a, b, NT_DIMS, preferred_element_type=F32)


def _iota(shape, dim):
    return lax.broadcasted_iota(jnp.int32, shape, dim)


def _phi(t):
    return jnp.where(t > 0, t + 1.0, jnp.exp(t))


def _sigmoid(t):
    return 1.0 / (1.0 + jnp.exp(-t))


def _recip(x):
    r = pl.reciprocal(x, approx=True)
    r = r * (2.0 - x * r)
    return r * (2.0 - x * r)


def _div18(i):
    return (i * 57) >> 10


def _blk(t, size=128):
    if isinstance(t, int):
        return slice(size * t, size * (t + 1))
    return pl.ds(pl.multiple_of(t * size, size), size)


def _rows(start, size, align):
    if isinstance(start, int):
        return slice(start, start + size)
    return pl.ds(pl.multiple_of(start, align), size)


def _colsum(a):
    return jnp.sum(jnp.sum(a.reshape(a.shape[0] // 8, 8, a.shape[1]), axis=0), axis=0, keepdims=True)


def _kernel(x_hbm, wq_hbm, wk_hbm, wv_hbm, wo_hbm, beta_hbm, wr_hbm, wg_hbm, wu_hbm, wd_hbm,
            out_hbm,
            x_v, xn_v, res_v, stat_v, wraw, w_t, wo_t, beta_v, wr_v, wr_b, wg_v, wu_v, wd_v,
            q_t, pq_t, v_t, k_n, pk_t, o_t, p_buf, am_t, den_t, m_t, r_row, gate_t, moe_y, out_v,
            sem_in, sem_moe, sem_out, sem_bar):

    def x_copy(s, tt=None):
        if tt is None:
            c0, n, k = s * L, L, 3 + s
        else:
            c0, n, k = tt * 128, 128, tt
        return pltpu.make_async_copy(x_hbm.at[0, :, pl.ds(c0, n)], x_v.at[:, pl.ds(c0, n)],
                                     sem_in.at[k])

    def w_copy(i, cb):
        src = (wq_hbm, wk_hbm, wv_hbm)[i]
        n = 128 if cb < 4 else 64
        return pltpu.make_async_copy(src.at[:, pl.ds(128 * cb, n)], wraw.at[i, :, pl.ds(128 * cb, n)],
                                     sem_in.at[7 + 5 * i + cb])

    wo_copy = pltpu.make_async_copy(wo_hbm, wraw.at[3], sem_in.at[22])
    beta_copy = pltpu.make_async_copy(beta_hbm, beta_v, sem_in.at[23])
    wr_copy = pltpu.make_async_copy(wr_hbm, wr_v, sem_in.at[24])
    NMC = FF // MOE_DMA

    def moe_copy(i, c):
        src, dst = ((wg_hbm, wg_v), (wu_hbm, wu_v), (wd_hbm, wd_v))[i]
        cs = pl.ds(c * MOE_DMA, MOE_DMA)
        return pltpu.make_async_copy(src.at[:, cs], dst.at[:, cs], sem_moe.at[i * NMC + c])

    def out_copy(t):
        cs = pl.ds(t * 128 if isinstance(t, int) else pl.multiple_of(t * 128, 128), 128)
        return pltpu.make_async_copy(out_v.at[t], out_hbm.at[0, :, cs], sem_out.at[t])

    wr_copy.start()
    x_copy(0, 0).start()
    for i in range(3):
        w_copy(i, 0).start()
    beta_copy.start()
    for tt in range(1, 4):
        x_copy(0, tt).start()
    for cb in range(1, 5):
        for i in range(3):
            w_copy(i, cb).start()
    x_copy(1).start()
    x_copy(2).start()
    x_copy(3).start()
    wo_copy.start()

    pace = {}

    def paced(row, lanes=128):
        tok = pace.get("tok")
        return row if tok is None else row + tok[:, :lanes] * 0.0

    def ln_stats(t):
        cols = _blk(t)
        shift = paced(x_v[0:16, cols].astype(F32)[0:1])
        s1 = [None] * 2
        s2 = [None] * 2
        for u in range(D // 16):
            d = x_v[16 * u:16 * (u + 1), cols].astype(F32) - shift
            d = d.reshape(2, 8, 128)
            for k in range(2):
                s1[k] = d[k] if u == 0 else s1[k] + d[k]
                s2[k] = d[k] * d[k] if u == 0 else s2[k] + d[k] * d[k]
        m1 = jnp.sum(s1[0] + s1[1], axis=0, keepdims=True) * (1.0 / D)
        m2 = jnp.sum(s2[0] + s2[1], axis=0, keepdims=True) * (1.0 / D)
        var = jnp.maximum(m2 - m1 * m1, 0.0)
        stat_v[0:1, cols] = m1 + shift
        stat_v[8:9, cols] = lax.rsqrt(var + 1e-5)

    def ln_apply(t):
        cols = _blk(t)
        mean = paced(stat_v[0:1, cols])
        rstd = stat_v[8:9, cols]
        for u in range(D // 48):
            rows = slice(48 * u, 48 * (u + 1))
            x = x_v[rows, cols].astype(F32)
            xn = (x - mean) * rstd
            xn_v[t, rows, :] = xn.astype(BF)
            res_v[rows, cols] = x + xn

    def router(t):
        r = _dot(wr_b[...], xn_v[t])
        r_row[:, _blk(t)] = r[0:1].astype(BF).astype(F32)

    def layernorm(t):
        ln_stats(t)
        ln_apply(t)
        router(t)

    def prep_wr():
        wr = wr_v[...].reshape(1, D)
        wr_b[...] = jnp.broadcast_to(wr.astype(F32), (16, D)).astype(BF)

    def prep_wt(cb, which):
        nb = 128 if cb < 4 else 64
        n = DH * GN[cb]
        t = wraw[which, :, 128 * cb:128 * cb + nb].T
        r0 = 384 * cb + which * GW[cb]
        k = min(n - 2 * cb, nb)
        w_t[r0 + 2 * cb:r0 + 2 * cb + k, :] = t[0:k]
        w_t[r0 + n:r0 + GW[cb], :] = jnp.zeros((GW[cb] - n, D), BF)
        if cb < 4:
            r1 = 384 * (cb + 1) + which * GW[cb + 1]
            w_t[r1:r1 + 2 * (cb + 1), :] = t[128 - 2 * (cb + 1):128]

    def prep_wo(g):
        n = DH * GN[g]
        wo_t[:, 128 * g:128 * g + n] = wraw[3, 126 * g:126 * g + n, :].T
        wo_t[:, 128 * g + n:128 * g + GW[g]] = jnp.zeros((D, GW[g] - n), BF)

    def prep_gates():
        b = beta_v[...].astype(F32).reshape(1, H)
        sig = jnp.concatenate([_sigmoid(b), jnp.zeros((1, 128 - H), F32)], axis=1)
        rows = jnp.broadcast_to(sig, (128, 128)).T
        for g in range(NG):
            gate_t[g] = rows[HPG * g:HPG * g + 8]

    def proj_qkv(s, tt, g, need_pq=True, need_pk=True):
        w = GW[g]
        rows = slice(128 * g, 128 * g + w)
        r = _dot(w_t[384 * g:384 * g + 3 * w, :], xn_v[4 * s + tt])
        q, k, v = r[:w], r[w:2 * w], r[2 * w:]
        q_t[s, tt, rows, :] = (q * QSCALE).astype(BF)
        if need_pq:
            pq_t[s, tt, rows, :] = _phi(q).astype(BF)
        k_n[s, g, _blk(tt), :w] = k.astype(BF).T
        if need_pk:
            pk_t[s, tt, rows, :] = _phi(k).astype(BF)
        v = jnp.where(_iota((w, 128), 0) == ZR[g], 1.0, v)
        v_t[s, tt, rows, :] = v.astype(BF)

    def mem_update(s, g, first):
        w = GW[g]
        rows = slice(128 * g, 128 * g + w)
        r = _dot_nt(v_t[s, 0, rows, :], pk_t[s, 0, rows, :])
        for tt in range(1, 4):
            r = r + _dot_nt(v_t[s, tt, rows, :], pk_t[s, tt, rows, :])
        rr, cc = _iota((w, w), 0), _iota((w, w), 1)
        keep = (cc < DH * GN[g]) & ((_div18(rr) == _div18(cc)) | (rr == ZR[g]))
        r = jnp.where(keep, r, 0.0)
        if not first:
            r = r + m_t[g, :w, :w]
        m_t[g, :w, :w] = r

    def mem_read(s, g):
        w = GW[g]
        rows = slice(128 * g, 128 * g + w)
        m = m_t[g, :w, :w]
        z = m[ZR[g]:ZR[g] + 1, :]
        zrows = jnp.where(_iota((16, w), 0) == _div18(_iota((16, w), 1)), z, 0.0)
        lhs = jnp.concatenate([m, zrows], axis=0).astype(BF)
        for tt in range(4):
            cols = slice(128 * tt, 128 * (tt + 1))
            r = _dot(lhs, pq_t[s, tt, rows, :])
            am_t[s, rows, cols] = r[:w]
            den_t[s, 16 * g:16 * (g + 1), cols] = r[w:]

    def proj_out(s, tt, fb, by_group=False):
        f0 = 192 * fb
        f1 = f0 + 192
        if by_group:
            p = None
            for g in range(NG):
                r = _dot(wo_t[f0:f1, 128 * g:128 * g + GW[g]], o_t[s, tt, 128 * g:128 * g + GW[g], :])
                p = r if p is None else p + r
        else:
            p = _dot(wo_t[f0:f1, :], o_t[s, tt])
        out_v[4 * s + tt, f0:f1, :] = (p + res_v[f0:f1, _blk(4 * s + tt)]).astype(BF)

    moe = {}

    def moe_select():
        r = r_row[...]
        io = _iota((1, SEQ), 1)
        m1 = jnp.max(r)
        i1 = jnp.min(jnp.where(r == m1, io, SEQ - 1))
        r2 = jnp.where(io == i1, -jnp.inf, r)
        m2 = jnp.max(r2)
        i2 = jnp.min(jnp.where((r2 == m2) & (io != i1), io, SEQ - 1))
        rows = []
        for i in (i1, i2):
            xb = xn_v[i // 128].T.astype(F32)
            rows.append(jnp.sum(jnp.where(_iota((128, D), 0) == i % 128, xb, 0.0), axis=0, keepdims=True))
        rr = _iota((16, D), 0)
        xs = jnp.where(rr == 0, rows[0], jnp.where(rr == 1, rows[1], 0.0))
        moe["x"] = xs.astype(BF)
        moe["w"] = _sigmoid(jnp.where(_iota((16, 1), 0) == 0, m1, m2))
        sel = jnp.where(_iota((2, 128), 0) == 0, i1, i2)
        for t in range(4 * NSEG):
            tok = _iota((2, 128), 1) + 128 * t
            o_t[t // 4, t % 4, 126:128, :] = jnp.where(tok == sel, 1.0, 0.0).astype(BF)

    KTS = [(128 * k, min(128 * (k + 1), D)) for k in range(5)]

    def moe_up(name, ref, f, k):
        k0, k1 = KTS[k]
        r = _dot(moe["x"][:, k0:k1], ref[k0:k1, _blk(f)])
        moe[name] = r if k == 0 else moe[name] + r

    def moe_hidden(f):
        g = moe["g"]
        moe[("h", f if isinstance(f, int) else 0)] = (g * _sigmoid(g) * moe["u"]).astype(BF)

    def moe_down(f, n, first):
        n0, n1 = KTS[n]
        r = _dot_nt(moe[("h", f if isinstance(f, int) else 0)], wd_v[n0:n1, _blk(f)])
        moe[("y", n)] = r if first else moe[("y", n)] + r

    def moe_up_tasks(fs):
        tasks = []
        for f in fs:
            tasks += [lambda f=f, k=k: moe_up("g", wg_v, f, k) for k in range(5)]
            tasks += [lambda f=f, k=k: moe_up("u", wu_v, f, k) for k in range(4)]
            tasks.append(lambda f=f: (moe_up("u", wu_v, f, 4), moe_hidden(f)))
        return tasks

    def moe_down_tasks(fs):
        return [(f, lambda f=f, n=n: moe_down(f, n, f == 0)) for f in fs for n in range(5)]

    def moe_finish():
        y = jnp.concatenate([moe[("y", n)] for n in range(5)], axis=1) * moe["w"]
        rr = _iota((128, D), 0)
        ypad = jnp.where(rr == 126, y[0:1], jnp.where(rr == 127, y[1:2], 0.0))
        cur = wo_t[:, 0:128].astype(F32)
        wo_t[:, 0:128] = jnp.where(_iota((D, 128), 1) >= 126, ypad.T, cur).astype(BF)

    causal = _iota((128, 128), 0) <= _iota((128, 128), 1)
    wrow = _iota((32, 128), 0)

    def barrier():
        pl.semaphore_signal(sem_bar, 1)
        pl.semaphore_wait(sem_bar, 1)

    def query_weights(s, g, j, i, w):
        wq = q_t[s, i, _rows(128 * g + 16 * j, 32, 16), :]
        wq = jnp.where((wrow >= 2 * j) & (wrow < 2 * j + DH), wq, jnp.zeros_like(wq))
        parts = [wq]
        if j > 0:
            parts.insert(0, jnp.zeros((16 * j, 128), BF))
        if w - 16 * j - 32 > 0:
            parts.append(jnp.zeros((w - 16 * j - 32, 128), BF))
        return jnp.concatenate(parts, axis=0) if len(parts) > 1 else wq

    def key_tile(s, g, kt, w):
        return k_n[s, g, 128 * kt:128 * (kt + 1), :w]

    def score_tile(s, g, i, kt, w, wq):
        d = _dot(key_tile(s, g, kt, w), wq)
        return jnp.where(causal, d, NEG) if kt == i else d

    def value_window(s, g, j, kt):
        v = v_t[s, kt, _rows(128 * g + 16 * j, 32, 16), :]
        return jnp.where(wrow >= 30, jnp.ones_like(v), v)

    def value_tile(s, g, j, kt, p):
        return _dot(value_window(s, g, j, kt), p)

    def finish_column(s, g, j, i, o, with_mem):
        cols = slice(128 * i, 128 * (i + 1))
        win = _rows(128 * g + 16 * j, 32, 16)
        gate = gate_t[g][j:j + 1]
        scale = (1.0 - gate) * _recip(o[31:32, :])
        if isinstance(g, int) and CFG.get("pace", 1):
            pace["tok"] = scale
        o = o * scale
        if with_mem:
            den = den_t[s, _rows(16 * g, 16, 16), cols][j:j + 1] + 1e-6
            o = o + am_t[s, win, cols] * (gate * _recip(den))
        if isinstance(g, int):
            r0 = 128 * g + DH * j
            o_t[s, i, r0:r0 + DH, :] = o[2 * j:2 * j + DH].astype(BF)
        else:
            mine = (wrow >= 2 * j) & (wrow < 2 * j + DH)
            o_t[s, i, win, :] = jnp.where(mine, o, o_t[s, i, win, :].astype(F32)).astype(BF)

    def running_max(m, d):
        pm = jnp.max(d.reshape(16, 8, 128), axis=0)
        return pm if m is None else jnp.maximum(m, pm)

    def compact_path():
        pace.clear()
        for c in range(NMC):
            start_moe(c)
        for g in range(NG):
            prep_wo(g)
            m_t[g] = jnp.zeros((128, 128), F32)
        am_t[0] = jnp.zeros((GP, L), F32)
        den_t[0] = jnp.ones((16 * NG, L), F32)

        @pl.loop(0, 4 * NSEG)
        def _(t):
            layernorm(t)

        for c in range(NMC):
            wait_moe(c)
        moe_select()

        def expert(f, y):
            for k in range(5):
                moe_up("g", wg_v, f, k)
            for k in range(5):
                moe_up("u", wu_v, f, k)
            moe_hidden(f)
            for n in range(5):
                moe[("y", n)] = y[n]
                moe_down(f, n, False)
            return tuple(moe[("y", n)] for n in range(5))

        y = lax.fori_loop(0, FF // 128, expert,
                          tuple(jnp.zeros((16, k1 - k0), F32) for k0, k1 in KTS))
        for n in range(5):
            moe[("y", n)] = y[n]
        moe_finish()

        def head(s, g, j, w):
            for i in range(4):
                wq = query_weights(s, g, j, i, w)
                tiles, m = [], None
                for kt in range(i + 1):
                    tiles.append(score_tile(s, g, i, kt, w, wq))
                    m = running_max(m, tiles[-1])
                m = jnp.max(m, axis=0, keepdims=True)
                o = None
                for kt in range(i + 1):
                    r = value_tile(s, g, j, kt, jnp.exp2(tiles[kt] - m).astype(BF))
                    o = r if o is None else o + r
                finish_column(s, g, j, i, o, True)
                pace.clear()

        @pl.loop(0, NSEG)
        def _(s):
            @pl.loop(0, 4)
            def _(tt):
                for g in range(NG):
                    proj_qkv(s, tt, g)

            @pl.when(s > 0)
            def _():
                for g in range(NG):
                    mem_read(s, g)

            @pl.loop(0, NG - 1)
            def _(g):
                for j in range(HPG):
                    head(s, g, j, 128)

            for j in range(GN[NG - 1]):
                head(s, NG - 1, j, GW[NG - 1])
            for g in range(NG):
                mem_update(s, g, False)

            @pl.loop(0, 4)
            def _(tt):
                for fb in range(3):
                    proj_out(s, tt, fb)
                out_copy(4 * s + tt).start()
                out_copy(4 * s + tt).wait()

    def head_units(first_head):
        units, h = [], first_head
        while h < H:
            g, j = divmod(h, HPG)
            if j + 1 < GN[g]:
                units.append((h, h + 1))
                h += 2
            else:
                units.append((h,))
                h += 1
        return units

    def make_blocks():
        blocks = [[(0, (h,), i) for i in range(4)] for h in range(SPLIT)]
        for s in range(NSEG - 1):
            blocks += [[(s, u, i) for i in range(4)] for u in head_units(SPLIT if s == 0 else 0)]
        s = NSEG - 1
        for i, budget in ((3, 16), (2, 18), (1, 20), (0, 20)):
            cur, n = [], 0
            for u in head_units(0):
                cost = len(u) * (i + 1)
                if cur and (n + cost > budget or (i == 0 and u[0] % HPG == 0)):
                    blocks.append(cur)
                    cur, n = [], 0
                cur.append((s, u, i))
                n += cost
            blocks.append(cur)
        return blocks

    col128 = _iota((64, 128), 1)
    mix_mask = _iota((64, 128), 0) <= (col128 & 63)

    def run_pipeline():
        blocks = make_blocks()
        nb = len(blocks)
        st, mx = {}, {}

        def slots(b):
            out, n = {}, 0
            for e, (_, heads, i) in enumerate(blocks[b]):
                for pos in range(len(heads)):
                    for kt in range(i + 1):
                        out[(e, pos, kt)] = n
                        n += 1
            return out

        def scores(b, micro):
            usemax = b < SPLIT or CFG.get("allmax")
            slot = slots(b)
            for e, (s, heads, i) in enumerate(blocks[b]):
                g = heads[0] // HPG
                w = GW[g]
                wqs = [query_weights(s, g, h % HPG, i, w) for h in heads]
                paired = len(heads) == 2 and not usemax
                ms = [None] * len(heads)
                for kt in range(i + 1):
                    if paired and kt == i:
                        keys = k_n[s, g, 128 * kt:128 * kt + 64, :w]
                        for pos in range(2):
                            d = _dot(keys, wqs[pos])
                            micro()
                            p_buf[b % 2, slot[(e, pos, kt)], 0:64, :] = jnp.exp2(
                                jnp.where(causal[:64], d, NEG)).astype(BF)
                        continue
                    keys = key_tile(s, g, kt, w)
                    for pos in range(len(heads)):
                        d = _dot(keys, wqs[pos])
                        micro()
                        if kt == i:
                            d = jnp.where(causal, d, NEG)
                        if usemax:
                            st[(b, slot[(e, pos, kt)])] = d
                            ms[pos] = running_max(ms[pos], d)
                        else:
                            p_buf[b % 2, slot[(e, pos, kt)]] = jnp.exp2(d).astype(BF)
                if usemax:
                    for pos, h in enumerate(heads):
                        mx[(s, h, i)] = jnp.max(ms[pos], axis=0, keepdims=True)
                if paired:
                    wmix = jnp.concatenate([wqs[1][:, 64:], wqs[0][:, 64:]], axis=1)
                    d = _dot(k_n[s, g, 128 * i + 64:128 * (i + 1), :w], wmix)
                    ex = jnp.exp2(jnp.where(mix_mask, d, NEG))
                    zero = jnp.zeros((64, 64), F32)
                    p_buf[b % 2, slot[(e, 0, i)], 64:128, :] = jnp.where(col128 >= 64, ex, 0.0).astype(BF)
                    p_buf[b % 2, slot[(e, 1, i)], 64:128, :] = jnp.concatenate(
                        [zero, ex[:, :64]], axis=1).astype(BF)

        def values(b):
            usemax = b < SPLIT or CFG.get("allmax")
            slot = slots(b)
            windows = {}
            for e, (s, heads, i) in enumerate(blocks[b]):
                for pos, h in enumerate(heads):
                    g, j = divmod(h, HPG)
                    m = mx.pop((s, h, i)) if usemax else None
                    o = None
                    for kt in range(i + 1):
                        if usemax:
                            p = jnp.exp2(st.pop((b, slot[(e, pos, kt)])) - m).astype(BF)
                        else:
                            p = p_buf[b % 2, slot[(e, pos, kt)]]
                        if (h, kt) not in windows or not CFG.get("vcache", 1):
                            windows[(h, kt)] = value_window(s, g, j, kt)
                        r = _dot(windows[(h, kt)], p)
                        o = r if o is None else o + r
                    finish_column(s, g, j, i, o, s > 0)

        def proj_tasks(s, groups=range(NG)):
            return [(GW[g] // 16 * 15,
                     lambda s=s, tt=tt, g=g: proj_qkv(s, tt, g, s > 0, s < NSEG - 1))
                    for tt in range(4) for g in groups]

        def out_tasks(s, tts=range(4)):
            tasks = []
            for tt in tts:
                tasks += [(60, lambda s=s, tt=tt, fb=fb: proj_out(s, tt, fb, (s, tt) == (NSEG - 1, 0)))
                          for fb in range(3)]
                tasks.append((0, lambda s=s, tt=tt: out_copy(4 * s + tt).start()))
            return tasks

        def ln_tasks(s):
            ts = range(4 * s, 4 * s + 4)
            return ([(10, lambda t=t: ln_stats(t)) for t in ts]
                    + [(10, lambda t=t: ln_apply(t)) for t in ts]
                    + [(2, lambda t=t: router(t)) for t in ts])

        def upd_tasks(s):
            return [(GW[g] // 4, lambda s=s, g=g: mem_update(s, g, s == 0)) for g in range(NG)]

        def read_tasks(s):
            return [(GW[g] // 4 + 4, lambda s=s, g=g: mem_read(s, g)) for g in range(NG)]

        def prep_tasks(cbs):
            return [(5, lambda cb=cb, which=which: prep_wt(cb, which)) for cb in cbs for which in range(3)]

        guard = {}

        def norm_task(i, cb, part):
            acc = col_norm2(i, cb, part)
            if part > 0:
                acc = acc + guard[("acc", i)]
            else:
                acc = acc + paced(jnp.zeros((1, acc.shape[1]), F32), acc.shape[1])
            guard[("acc", i)] = acc
            if part == 2:
                row = jnp.sum(acc, axis=0, keepdims=True)
                if row.shape[1] < 128:
                    row = jnp.concatenate([row, jnp.zeros((1, 128 - row.shape[1]), F32)], axis=1)
                guard[i] = row if i not in guard else jnp.maximum(guard[i], row)

        def guard_task():
            nq, nk, nv = (jnp.max(guard[i]) for i in range(3))
            guard["safe"] = jnp.logical_and(
                nq * nk <= (SCORE_LIMIT / (1.05 * D * QSCALE * DH)) ** 2, nv <= 1e30)

        def norm_tasks(cbs):
            return [(1, lambda i=i, cb=cb, part=part: norm_task(i, cb, part))
                    for cb in cbs for i in range(3) for part in range(3)]

        seg0 = [min(k for k, blk in enumerate(blocks) if blk[0][0] == s) for s in range(NSEG)] + [nb]
        last = {i: max(k for k, blk in enumerate(blocks) if blk[0][0] == NSEG - 1 and blk[0][2] == i)
                for i in range(4)}

        def at(s, frac):
            lo = SPLIT if s == 0 else seg0[s]
            return lo + round(frac * (seg0[s + 1] - lo))

        a1, a2, a3 = seg0[1], seg0[2], seg0[3]
        streams = [
            (0, 1, prep_tasks((1,))),
            (0, 2, prep_tasks((2,))),
            (1, 4, proj_tasks(0, (1,))),
            (3, 5, prep_tasks((3, 4))),
            (4, min(8, SPLIT + 1), proj_tasks(0, (2,))),
            (CFG.get('ln1', (3, SPLIT))[0], CFG.get('ln1', (3, SPLIT))[1], ln_tasks(1)),
            (-1, 0, norm_tasks((0,))),
            (0, 3, norm_tasks((1, 2))),
            (3, SPLIT - 3, norm_tasks((3, 4))),
            (SPLIT - 3, SPLIT - 2, [(1, guard_task)]),
            (min(8, SPLIT), at(0, 0.2), proj_tasks(0, (3, 4))),
            (at(0, CFG.get('p1', 0.1)), a1 - 1, proj_tasks(1)),
            (at(0, 0.3), at(0, 0.5), upd_tasks(0)),
            (a1 - 1, a1, read_tasks(1)),
            (CFG.get('ln23', SPLIT + 1), a1 - 1, ln_tasks(2) + ln_tasks(3)),
            (SPLIT + 1, a1, [(5, lambda g=g: prep_wo(g)) for g in range(NG)]),
            (a1, a1 + 1, [(1, moe_select)]),
            (a1 + 1, at(1, 0.2), upd_tasks(1)),
            (a1, a2 - 1, proj_tasks(2)),
            (a2 - 1, a2, read_tasks(2)),
            (a2 + 1, at(2, 0.2), upd_tasks(2)),
            (a2, a3 - 1, proj_tasks(3)),
            (a3 - 1, a3, read_tasks(3)),
            (a3 - 1, a3, [(1, lambda: (emit_downs(len(downs)), moe_finish()))]),
            (a3 + 1, last[1] + 1, out_tasks(0) + out_tasks(1) + out_tasks(2)),
            (last[3] + 2, last[2] + 1, out_tasks(3, (3,))),
            (last[2] + 2, last[1] + 1, out_tasks(3, (2,))),
            (last[1] + 2, nb + 1, out_tasks(3, (1,))),
        ]
        nf = FF // 128
        micro_ranges = [(a1 + 1, a2 - 1, moe_up_tasks(range(nf // 2))),
                        (a2, a3 - 2, moe_up_tasks(range(nf // 2, nf)))]
        downs = moe_down_tasks(range(nf))
        dstate = [0]

        def emit_downs(limit):
            n = 0
            while dstate[0] < len(downs) and n < limit and ("h", downs[dstate[0]][0]) in moe:
                downs[dstate[0]][1]()
                dstate[0] += 1
                n += 1

        ntiles = [sum(len(u) * (i + 1) for (_, u, i) in blk) for blk in blocks]

        def fence_w12():
            wait_w(1)
            wait_w(2)

        def fence_w34():
            wait_w(3)
            wait_w(4)
            x_copy(1).wait()

        def fence_a1():
            wait_moe(0)
            start_moe(1)

        fences = {0: fence_w12, 3: fence_w34, SPLIT: lambda: start_moe(0), a1: fence_a1,
                  a2: lambda: wait_moe(1)}

        state = [[0, 0.0, float(sum(c for c, _ in t))] for _, _, t in streams]
        mstate = [[0, 0] for _ in micro_ranges]
        cur_scope = []

        def emit(b0, b1):
            for b in range(b0, b1 + 1):
                if _SCOPES and b % 4 == 0:
                    if cur_scope:
                        cur_scope.pop().__exit__(None, None, None)
                    cur_scope.append(jax.named_scope(f"blk{b:03d}"))
                    cur_scope[-1].__enter__()
                if b in fences and b < b1:
                    fences[b]()

                def micro(b=b):
                    for (lo, hi, tasks), ms in zip(micro_ranges, mstate):
                        if lo <= b < hi:
                            ms[0] += 1
                            total = sum(ntiles[lo:hi])
                            while ms[1] < len(tasks) and ms[1] < ms[0] * len(tasks) / total:
                                tasks[ms[1]]()
                                ms[1] += 1

                if b < b1:
                    scores(b, micro)
                if b < b1 or b == nb:
                    for (lo, hi, tasks), st_ in zip(streams, state):
                        if b < lo:
                            continue
                        frac = (b + 1 - lo) / (hi - lo)
                        while st_[0] < len(tasks) and st_[1] + tasks[st_[0]][0] / 2 <= frac * st_[2] + 1e-9:
                            st_[1] += tasks[st_[0]][0]
                            tasks[st_[0]][1]()
                            st_[0] += 1
                            if tasks[st_[0] - 1][0] >= 75 and a1 < b < a3:
                                emit_downs(CFG.get("dper", 5))
                if b > b0:
                    values(b - 1)
            if cur_scope:
                cur_scope.pop().__exit__(None, None, None)

        def fast_rest():
            pace.clear()
            emit(SPLIT, nb)
            for (lo, hi, tasks), st_ in zip(streams, state):
                assert st_[0] == len(tasks), (lo, hi, st_)
            assert all(ms[1] == len(r[2]) for ms, r in zip(mstate, micro_ranges)) and dstate[0] == len(downs)
            with scope("tail0"):
                for _, t in out_tasks(3, (0,)):
                    t()
            with scope("tail1"):
                for t in range(4 * NSEG):
                    out_copy(t).wait()

        for (lo, hi, tasks), st_ in zip(streams, state):
            if lo < 0:
                for _, t in tasks:
                    t()
                st_[0] = len(tasks)
        emit(0, SPLIT)
        x_copy(2).wait()
        x_copy(3).wait()
        wo_copy.wait()
        safe = guard["safe"]
        if CFG.get("only") == "fast":
            fast_rest()
        elif CFG.get("only") == "compact":
            compact_path()
        else:
            pl.when(safe)(fast_rest)
            pl.when(jnp.logical_not(safe))(compact_path)

    def prep_group(g):
        for which in range(3):
            prep_wt(g, which)

    def wait_w(cb):
        for i in range(3):
            w_copy(i, cb).wait()

    def start_moe(c):
        for i in range(3):
            moe_copy(i, c).start()

    def wait_moe(c):
        for i in range(3):
            moe_copy(i, c).wait()

    def col_norm2(i, cb, part):
        n = 128 if cb < 4 else 64
        acc = None
        for u in range(3 * part, 3 * part + 3):
            wv = wraw[i, 64 * u:64 * (u + 1), 128 * cb:128 * cb + n].astype(F32)
            c = jnp.sum((wv * wv).reshape(8, 8, n), axis=0)
            acc = c if acc is None else acc + c
        return acc

    def scope(name):
        return jax.named_scope(name) if _SCOPES else contextlib.nullcontext()

    with scope("pre0"):
        for s in range(NSEG):
            for g in range(NG):
                n = DH * GN[g]
                for tt in range(4):
                    o_t[s, tt, 128 * g + n:128 * g + GW[g], :] = jnp.zeros((GW[g] - n, 128), BF)
        wr_copy.wait()
        x_copy(0, 0).wait()
        prep_wr()
        layernorm(0)
    with scope("pre1"):
        wait_w(0)
        prep_group(0)
        proj_qkv(0, 0, 0, False, True)
    with scope("pre2"):
        for tt in range(1, 4):
            x_copy(0, tt).wait()
        beta_copy.wait()
        for tt in range(1, 4):
            layernorm(tt)
            proj_qkv(0, tt, 0, False, True)
        prep_gates()
    run_pipeline()


@jax.jit
def pallas_parallel_sum__memory_aug_infini_attn__moe_arch_mod__prompt_kernel(
    A_x: jax.Array,
    A_wq: jax.Array,
    A_wk: jax.Array,
    A_wv: jax.Array,
    A_wo: jax.Array,
    A_beta: jax.Array,
    B_x: jax.Array,
    B_w_r: jax.Array,
    B_w_gate: jax.Array,
    B_w_up: jax.Array,
    B_w_down: jax.Array,
):
    del B_x
    hbm = pl.BlockSpec(memory_space=pltpu.HBM)
    scratch = [
        pltpu.VMEM((D, SEQ), BF),
        pltpu.VMEM((4 * NSEG, D, 128), BF),
        pltpu.VMEM((D, SEQ), F32),
        pltpu.VMEM((16, SEQ), F32),
        pltpu.VMEM((4, D, D), BF),
        pltpu.VMEM((3 * GP, D), BF),
        pltpu.VMEM((D, GP), BF),
        pltpu.VMEM((H,), BF),
        pltpu.VMEM((D,), BF),
        pltpu.VMEM((16, D), BF),
        pltpu.VMEM((D, FF), BF),
        pltpu.VMEM((D, FF), BF),
        pltpu.VMEM((D, FF), BF),
        pltpu.VMEM((NSEG, 4, GP, 128), BF),
        pltpu.VMEM((NSEG, 4, GP, 128), BF),
        pltpu.VMEM((NSEG, 4, GP, 128), BF),
        pltpu.VMEM((NSEG, NG, L, 128), BF),
        pltpu.VMEM((NSEG, 4, GP, 128), BF),
        pltpu.VMEM((NSEG, 4, GP, 128), BF),
        pltpu.VMEM((2, 20, 128, 128), BF),
        pltpu.VMEM((NSEG, GP, L), F32),
        pltpu.VMEM((NSEG, 16 * NG, L), F32),
        pltpu.VMEM((NG, 128, 128), F32),
        pltpu.VMEM((1, SEQ), F32),
        pltpu.VMEM((NG, 8, 128), F32),
        pltpu.VMEM((16, D), F32),
        pltpu.VMEM((4 * NSEG, D, 128), BF),
        pltpu.SemaphoreType.DMA((25,)),
        pltpu.SemaphoreType.DMA((3 * (FF // MOE_DMA),)),
        pltpu.SemaphoreType.DMA((4 * NSEG,)),
        pltpu.SemaphoreType.REGULAR,
    ]
    out_t = pl.pallas_call(
        _kernel,
        out_shape=jax.ShapeDtypeStruct((1, D, SEQ), BF),
        in_specs=[hbm] * 10,
        out_specs=hbm,
        scratch_shapes=scratch,
        compiler_params=pltpu.CompilerParams(vmem_limit_bytes=100 * 1024 * 1024),
    )(jnp.swapaxes(A_x, 1, 2), A_wq, A_wk, A_wv, A_wo, A_beta, B_w_r, B_w_gate, B_w_up,
      B_w_down.T)
    return jnp.swapaxes(out_t, 1, 2)
```

```python
import contextlib
import json
import os

import jax
import jax.numpy as jnp
from jax import lax
import jax.experimental.pallas as pl
import jax.experimental.pallas.tpu as pltpu

BF = jnp.bfloat16
F32 = jnp.float32

SEQ, D, H, DH = 2048, 576, 32, 18
NSEG, L, FF = 4, 512, 4608
HPG = 7
NG = 5
GN = (7, 7, 7, 7, 4)
GW = (128, 128, 128, 128, 80)
GP = 592
ZR = (126, 126, 126, 126, 78)
QSCALE = (DH ** -0.5) * 1.4426950408889634
NT_DIMS = (((1,), (1,)), ((), ()))
MOE_DMA = 2304
NEG = -1e30
SCORE_LIMIT = 40.0
_SCOPES = os.environ.get("KSCOPES", "") == "1"
CFG = dict()
CFG.update(json.loads(os.environ.get("KCFG", "{}")))


def _dot(a, b):
    return jnp.dot(a, b, preferred_element_type=F32)


def _dot_nt(a, b):
    return lax.dot_general(a, b, NT_DIMS, preferred_element_type=F32)


def _iota(shape, dim):
    return lax.broadcasted_iota(jnp.int32, shape, dim)


def _phi(t):
    return jnp.where(t > 0, t + 1.0, jnp.exp(t))


def _sigmoid(t):
    return 1.0 / (1.0 + jnp.exp(-t))


def _recip(x):
    r = pl.reciprocal(x, approx=True)
    r = r * (2.0 - x * r)
    return r * (2.0 - x * r)


def _div18(i):
    return (i * 57) >> 10


def _blk(t, size=128):
    if isinstance(t, int):
        return slice(size * t, size * (t + 1))
    return pl.ds(pl.multiple_of(t * size, size), size)


def _rows(start, size, align):
    if isinstance(start, int):
        return slice(start, start + size)
    return pl.ds(pl.multiple_of(start, align), size)


def _colsum(a):
    return jnp.sum(jnp.sum(a.reshape(a.shape[0] // 8, 8, a.shape[1]), axis=0), axis=0, keepdims=True)


def _kernel(x_hbm, wq_hbm, wk_hbm, wv_hbm, wo_hbm, beta_hbm, wr_hbm, wg_hbm, wu_hbm, wd_hbm,
            out_hbm,
            x_v, xn_v, res_v, stat_v, wraw, w_t, wo_t, beta_v, wr_v, wr_b, wg_v, wu_v, wd_v,
            q_t, pq_t, v_t, k_n, pk_t, o_t, p_buf, am_t, den_t, m_t, r_row, gate_t, moe_y, out_v,
            sem_in, sem_moe, sem_out, sem_bar):

    def x_copy(s, tt=None):
        if tt is None:
            c0, n, k = s * L, L, 3 + s
        else:
            c0, n, k = tt * 128, 128, tt
        return pltpu.make_async_copy(x_hbm.at[0, :, pl.ds(c0, n)], x_v.at[:, pl.ds(c0, n)],
                                     sem_in.at[k])

    def w_copy(i, cb):
        src = (wq_hbm, wk_hbm, wv_hbm)[i]
        n = 128 if cb < 4 else 64
        return pltpu.make_async_copy(src.at[:, pl.ds(128 * cb, n)], wraw.at[i, :, pl.ds(128 * cb, n)],
                                     sem_in.at[7 + 5 * i + cb])

    wo_copy = pltpu.make_async_copy(wo_hbm, wraw.at[3], sem_in.at[22])
    beta_copy = pltpu.make_async_copy(beta_hbm, beta_v, sem_in.at[23])
    wr_copy = pltpu.make_async_copy(wr_hbm, wr_v, sem_in.at[24])
    NMC = FF // MOE_DMA

    def moe_copy(i, c):
        src, dst = ((wg_hbm, wg_v), (wu_hbm, wu_v), (wd_hbm, wd_v))[i]
        cs = pl.ds(c * MOE_DMA, MOE_DMA)
        return pltpu.make_async_copy(src.at[:, cs], dst.at[:, cs], sem_moe.at[i * NMC + c])

    def out_copy(t):
        cs = pl.ds(t * 128 if isinstance(t, int) else pl.multiple_of(t * 128, 128), 128)
        return pltpu.make_async_copy(out_v.at[t], out_hbm.at[0, :, cs], sem_out.at[t])

    wr_copy.start()
    x_copy(0, 0).start()
    for i in range(3):
        w_copy(i, 0).start()
    beta_copy.start()
    for tt in range(1, 4):
        x_copy(0, tt).start()
    for cb in range(1, 5):
        for i in range(3):
            w_copy(i, cb).start()
    x_copy(1).start()
    x_copy(2).start()
    x_copy(3).start()
    wo_copy.start()

    pace = {}

    def paced(row, lanes=128):
        tok = pace.get("tok")
        return row if tok is None else row + tok[:, :lanes] * 0.0

    def ln_stats(t):
        cols = _blk(t)
        shift = paced(x_v[0:16, cols].astype(F32)[0:1])
        s1 = [None] * 2
        s2 = [None] * 2
        for u in range(D // 16):
            d = x_v[16 * u:16 * (u + 1), cols].astype(F32) - shift
            d = d.reshape(2, 8, 128)
            for k in range(2):
                s1[k] = d[k] if u == 0 else s1[k] + d[k]
                s2[k] = d[k] * d[k] if u == 0 else s2[k] + d[k] * d[k]
        m1 = jnp.sum(s1[0] + s1[1], axis=0, keepdims=True) * (1.0 / D)
        m2 = jnp.sum(s2[0] + s2[1], axis=0, keepdims=True) * (1.0 / D)
        var = jnp.maximum(m2 - m1 * m1, 0.0)
        stat_v[0:1, cols] = m1 + shift
        stat_v[8:9, cols] = lax.rsqrt(var + 1e-5)

    def ln_apply(t):
        cols = _blk(t)
        mean = paced(stat_v[0:1, cols])
        rstd = stat_v[8:9, cols]
        for u in range(D // 48):
            rows = slice(48 * u, 48 * (u + 1))
            x = x_v[rows, cols].astype(F32)
            xn = (x - mean) * rstd
            xn_v[t, rows, :] = xn.astype(BF)
            res_v[rows, cols] = x + xn

    def router(t):
        r = _dot(wr_b[...], xn_v[t])
        r_row[:, _blk(t)] = r[0:1].astype(BF).astype(F32)

    def layernorm(t):
        ln_stats(t)
        ln_apply(t)
        router(t)

    def prep_wr():
        wr = wr_v[...].reshape(1, D)
        wr_b[...] = jnp.broadcast_to(wr.astype(F32), (16, D)).astype(BF)

    def prep_wt(cb, which):
        nb = 128 if cb < 4 else 64
        n = DH * GN[cb]
        t = wraw[which, :, 128 * cb:128 * cb + nb].T
        r0 = 384 * cb + which * GW[cb]
        k = min(n - 2 * cb, nb)
        w_t[r0 + 2 * cb:r0 + 2 * cb + k, :] = t[0:k]
        w_t[r0 + n:r0 + GW[cb], :] = jnp.zeros((GW[cb] - n, D), BF)
        if cb < 4:
            r1 = 384 * (cb + 1) + which * GW[cb + 1]
            w_t[r1:r1 + 2 * (cb + 1), :] = t[128 - 2 * (cb + 1):128]

    def prep_wo(g):
        n = DH * GN[g]
        wo_t[:, 128 * g:128 * g + n] = wraw[3, 126 * g:126 * g + n, :].T
        wo_t[:, 128 * g + n:128 * g + GW[g]] = jnp.zeros((D, GW[g] - n), BF)

    def prep_gates():
        b = beta_v[...].astype(F32).reshape(1, H)
        sig = jnp.concatenate([_sigmoid(b), jnp.zeros((1, 128 - H), F32)], axis=1)
        rows = jnp.broadcast_to(sig, (128, 128)).T
        for g in range(NG):
            gate_t[g] = rows[HPG * g:HPG * g + 8]

    def proj_qkv(s, tt, g, need_pq=True, need_pk=True):
        w = GW[g]
        rows = slice(128 * g, 128 * g + w)
        r = _dot(w_t[384 * g:384 * g + 3 * w, :], xn_v[4 * s + tt])
        q, k, v = r[:w], r[w:2 * w], r[2 * w:]
        q_t[s, tt, rows, :] = (q * QSCALE).astype(BF)
        if need_pq:
            pq_t[s, tt, rows, :] = _phi(q).astype(BF)
        k_n[s, g, _blk(tt), :w] = k.astype(BF).T
        if need_pk:
            pk_t[s, tt, rows, :] = _phi(k).astype(BF)
        v = jnp.where(_iota((w, 128), 0) == ZR[g], 1.0, v)
        v_t[s, tt, rows, :] = v.astype(BF)

    def mem_update(s, g, first):
        w = GW[g]
        rows = slice(128 * g, 128 * g + w)
        r = _dot_nt(v_t[s, 0, rows, :], pk_t[s, 0, rows, :])
        for tt in range(1, 4):
            r = r + _dot_nt(v_t[s, tt, rows, :], pk_t[s, tt, rows, :])
        rr, cc = _iota((w, w), 0), _iota((w, w), 1)
        keep = (cc < DH * GN[g]) & ((_div18(rr) == _div18(cc)) | (rr == ZR[g]))
        r = jnp.where(keep, r, 0.0)
        if not first:
            r = r + m_t[g, :w, :w]
        m_t[g, :w, :w] = r

    def mem_read(s, g):
        w = GW[g]
        rows = slice(128 * g, 128 * g + w)
        m = m_t[g, :w, :w]
        z = m[ZR[g]:ZR[g] + 1, :]
        zrows = jnp.where(_iota((16, w), 0) == _div18(_iota((16, w), 1)), z, 0.0)
        lhs = jnp.concatenate([m, zrows], axis=0).astype(BF)
        for tt in range(4):
            cols = slice(128 * tt, 128 * (tt + 1))
            r = _dot(lhs, pq_t[s, tt, rows, :])
            am_t[s, rows, cols] = r[:w]
            den_t[s, 16 * g:16 * (g + 1), cols] = r[w:]

    def proj_out(s, tt, fb, by_group=False):
        f0 = 192 * fb
        f1 = f0 + 192
        if by_group:
            p = None
            for g in range(NG):
                r = _dot(wo_t[f0:f1, 128 * g:128 * g + GW[g]], o_t[s, tt, 128 * g:128 * g + GW[g], :])
                p = r if p is None else p + r
        else:
            p = _dot(wo_t[f0:f1, :], o_t[s, tt])
        out_v[4 * s + tt, f0:f1, :] = (p + res_v[f0:f1, _blk(4 * s + tt)]).astype(BF)

    moe = {}

    def moe_select():
        r = r_row[...]
        io = _iota((1, SEQ), 1)
        m1 = jnp.max(r)
        i1 = jnp.min(jnp.where(r == m1, io, SEQ - 1))
        r2 = jnp.where(io == i1, -jnp.inf, r)
        m2 = jnp.max(r2)
        i2 = jnp.min(jnp.where((r2 == m2) & (io != i1), io, SEQ - 1))
        rows = []
        for i in (i1, i2):
            xb = xn_v[i // 128].T.astype(F32)
            rows.append(jnp.sum(jnp.where(_iota((128, D), 0) == i % 128, xb, 0.0), axis=0, keepdims=True))
        rr = _iota((16, D), 0)
        xs = jnp.where(rr == 0, rows[0], jnp.where(rr == 1, rows[1], 0.0))
        moe["x"] = xs.astype(BF)
        moe["w"] = _sigmoid(jnp.where(_iota((16, 1), 0) == 0, m1, m2))
        sel = jnp.where(_iota((2, 128), 0) == 0, i1, i2)
        for t in range(4 * NSEG):
            tok = _iota((2, 128), 1) + 128 * t
            o_t[t // 4, t % 4, 126:128, :] = jnp.where(tok == sel, 1.0, 0.0).astype(BF)

    KTS = [(128 * k, min(128 * (k + 1), D)) for k in range(5)]

    def moe_up(name, ref, f, k):
        k0, k1 = KTS[k]
        r = _dot(moe["x"][:, k0:k1], ref[k0:k1, _blk(f)])
        moe[name] = r if k == 0 else moe[name] + r

    def moe_hidden(f):
        g = moe["g"]
        moe[("h", f if isinstance(f, int) else 0)] = (g * _sigmoid(g) * moe["u"]).astype(BF)

    def moe_down(f, n, first):
        n0, n1 = KTS[n]
        r = _dot_nt(moe[("h", f if isinstance(f, int) else 0)], wd_v[n0:n1, _blk(f)])
        moe[("y", n)] = r if first else moe[("y", n)] + r

    def moe_up_tasks(fs):
        tasks = []
        for f in fs:
            tasks += [lambda f=f, k=k: moe_up("g", wg_v, f, k) for k in range(5)]
            tasks += [lambda f=f, k=k: moe_up("u", wu_v, f, k) for k in range(4)]
            tasks.append(lambda f=f: (moe_up("u", wu_v, f, 4), moe_hidden(f)))
        return tasks

    def moe_down_tasks(fs):
        return [(f, lambda f=f, n=n: moe_down(f, n, f == 0)) for f in fs for n in range(5)]

    def moe_finish():
        y = jnp.concatenate([moe[("y", n)] for n in range(5)], axis=1) * moe["w"]
        rr = _iota((128, D), 0)
        ypad = jnp.where(rr == 126, y[0:1], jnp.where(rr == 127, y[1:2], 0.0))
        cur = wo_t[:, 0:128].astype(F32)
        wo_t[:, 0:128] = jnp.where(_iota((D, 128), 1) >= 126, ypad.T, cur).astype(BF)

    causal = _iota((128, 128), 0) <= _iota((128, 128), 1)
    wrow = _iota((32, 128), 0)

    def barrier():
        pl.semaphore_signal(sem_bar, 1)
        pl.semaphore_wait(sem_bar, 1)

    def query_weights(s, g, j, i, w):
        wq = q_t[s, i, _rows(128 * g + 16 * j, 32, 16), :]
        wq = jnp.where((wrow >= 2 * j) & (wrow < 2 * j + DH), wq, jnp.zeros_like(wq))
        parts = [wq]
        if j > 0:
            parts.insert(0, jnp.zeros((16 * j, 128), BF))
        if w - 16 * j - 32 > 0:
            parts.append(jnp.zeros((w - 16 * j - 32, 128), BF))
        return jnp.concatenate(parts, axis=0) if len(parts) > 1 else wq

    def key_tile(s, g, kt, w):
        return k_n[s, g, 128 * kt:128 * (kt + 1), :w]

    def score_tile(s, g, i, kt, w, wq):
        d = _dot(key_tile(s, g, kt, w), wq)
        return jnp.where(causal, d, NEG) if kt == i else d

    def value_window(s, g, j, kt):
        v = v_t[s, kt, _rows(128 * g + 16 * j, 32, 16), :]
        return jnp.where(wrow >= 30, jnp.ones_like(v), v)

    def value_tile(s, g, j, kt, p):
        return _dot(value_window(s, g, j, kt), p)

    def finish_column(s, g, j, i, o, with_mem):
        cols = slice(128 * i, 128 * (i + 1))
        win = _rows(128 * g + 16 * j, 32, 16)
        gate = gate_t[g][j:j + 1]
        scale = (1.0 - gate) * _recip(o[31:32, :])
        if isinstance(g, int) and CFG.get("pace", 1):
            pace["tok"] = scale
        o = o * scale
        if with_mem:
            den = den_t[s, _rows(16 * g, 16, 16), cols][j:j + 1] + 1e-6
            o = o + am_t[s, win, cols] * (gate * _recip(den))
        if isinstance(g, int):
            r0 = 128 * g + DH * j
            o_t[s, i, r0:r0 + DH, :] = o[2 * j:2 * j + DH].astype(BF)
        else:
            mine = (wrow >= 2 * j) & (wrow < 2 * j + DH)
            o_t[s, i, win, :] = jnp.where(mine, o, o_t[s, i, win, :].astype(F32)).astype(BF)

    def running_max(m, d):
        pm = jnp.max(d.reshape(16, 8, 128), axis=0)
        return pm if m is None else jnp.maximum(m, pm)

    def compact_path():
        pace.clear()
        for g in range(NG):
            prep_wo(g)
            m_t[g] = jnp.zeros((128, 128), F32)
        am_t[0] = jnp.zeros((GP, L), F32)
        den_t[0] = jnp.ones((16 * NG, L), F32)

        @pl.loop(0, 4 * NSEG)
        def _(t):
            layernorm(t)

        moe_select()

        def expert(f, y):
            for k in range(5):
                moe_up("g", wg_v, f, k)
            for k in range(5):
                moe_up("u", wu_v, f, k)
            moe_hidden(f)
            for n in range(5):
                moe[("y", n)] = y[n]
                moe_down(f, n, False)
            return tuple(moe[("y", n)] for n in range(5))

        y = lax.fori_loop(0, FF // 128, expert,
                          tuple(jnp.zeros((16, k1 - k0), F32) for k0, k1 in KTS))
        for n in range(5):
            moe[("y", n)] = y[n]
        moe_finish()

        def head(s, g, j, w):
            for i in range(4):
                wq = query_weights(s, g, j, i, w)
                tiles, m = [], None
                for kt in range(i + 1):
                    tiles.append(score_tile(s, g, i, kt, w, wq))
                    m = running_max(m, tiles[-1])
                m = jnp.max(m, axis=0, keepdims=True)
                o = None
                for kt in range(i + 1):
                    r = value_tile(s, g, j, kt, jnp.exp2(tiles[kt] - m).astype(BF))
                    o = r if o is None else o + r
                finish_column(s, g, j, i, o, True)
                pace.clear()

        @pl.loop(0, NSEG)
        def _(s):
            @pl.loop(0, 4)
            def _(tt):
                for g in range(NG):
                    proj_qkv(s, tt, g)

            @pl.when(s > 0)
            def _():
                for g in range(NG):
                    mem_read(s, g)

            @pl.loop(0, NG - 1)
            def _(g):
                for j in range(HPG):
                    head(s, g, j, 128)

            for j in range(GN[NG - 1]):
                head(s, NG - 1, j, GW[NG - 1])
            for g in range(NG):
                mem_update(s, g, False)

            @pl.loop(0, 4)
            def _(tt):
                for fb in range(3):
                    proj_out(s, tt, fb)
                out_copy(4 * s + tt).start()
                out_copy(4 * s + tt).wait()

    def head_units(first_head):
        units, h = [], first_head
        while h < H:
            g, j = divmod(h, HPG)
            if j + 1 < GN[g]:
                units.append((h, h + 1))
                h += 2
            else:
                units.append((h,))
                h += 1
        return units

    def make_blocks():
        blocks = []
        for s in range(NSEG - 1):
            blocks += [[(s, u, i) for i in range(4)] for u in head_units(0)]
        s = NSEG - 1
        for i, budget in ((3, 16), (2, 18), (1, 20), (0, 20)):
            cur, n = [], 0
            for u in head_units(0):
                cost = len(u) * (i + 1)
                if cur and (n + cost > budget or (i == 0 and u[0] % HPG == 0)):
                    blocks.append(cur)
                    cur, n = [], 0
                cur.append((s, u, i))
                n += cost
            blocks.append(cur)
        return blocks

    col128 = _iota((64, 128), 1)
    mix_mask = _iota((64, 128), 0) <= (col128 & 63)

    def run_pipeline():
        blocks = make_blocks()
        nb = len(blocks)
        st, mx = {}, {}

        def slots(b):
            out, n = {}, 0
            for e, (_, heads, i) in enumerate(blocks[b]):
                for pos in range(len(heads)):
                    for kt in range(i + 1):
                        out[(e, pos, kt)] = n
                        n += 1
            return out

        def scores(b, micro):
            usemax = bool(CFG.get("allmax"))
            slot = slots(b)
            for e, (s, heads, i) in enumerate(blocks[b]):
                g = heads[0] // HPG
                w = GW[g]
                wqs = [query_weights(s, g, h % HPG, i, w) for h in heads]
                paired = len(heads) == 2 and not usemax
                ms = [None] * len(heads)
                for kt in range(i + 1):
                    if paired and kt == i:
                        keys = k_n[s, g, 128 * kt:128 * kt + 64, :w]
                        for pos in range(2):
                            d = _dot(keys, wqs[pos])
                            micro()
                            p_buf[b % 2, slot[(e, pos, kt)], 0:64, :] = jnp.exp2(
                                jnp.where(causal[:64], d, NEG)).astype(BF)
                        continue
                    keys = key_tile(s, g, kt, w)
                    for pos in range(len(heads)):
                        d = _dot(keys, wqs[pos])
                        micro()
                        if kt == i:
                            d = jnp.where(causal, d, NEG)
                        if usemax:
                            st[(b, slot[(e, pos, kt)])] = d
                            ms[pos] = running_max(ms[pos], d)
                        else:
                            p_buf[b % 2, slot[(e, pos, kt)]] = jnp.exp2(d).astype(BF)
                if usemax:
                    for pos, h in enumerate(heads):
                        mx[(s, h, i)] = jnp.max(ms[pos], axis=0, keepdims=True)
                if paired:
                    wmix = jnp.concatenate([wqs[1][:, 64:], wqs[0][:, 64:]], axis=1)
                    d = _dot(k_n[s, g, 128 * i + 64:128 * (i + 1), :w], wmix)
                    ex = jnp.exp2(jnp.where(mix_mask, d, NEG))
                    zero = jnp.zeros((64, 64), F32)
                    p_buf[b % 2, slot[(e, 0, i)], 64:128, :] = jnp.where(col128 >= 64, ex, 0.0).astype(BF)
                    p_buf[b % 2, slot[(e, 1, i)], 64:128, :] = jnp.concatenate(
                        [zero, ex[:, :64]], axis=1).astype(BF)

        def values(b):
            usemax = bool(CFG.get("allmax"))
            slot = slots(b)
            windows = {}
            for e, (s, heads, i) in enumerate(blocks[b]):
                for pos, h in enumerate(heads):
                    g, j = divmod(h, HPG)
                    m = mx.pop((s, h, i)) if usemax else None
                    o = None
                    for kt in range(i + 1):
                        if usemax:
                            p = jnp.exp2(st.pop((b, slot[(e, pos, kt)])) - m).astype(BF)
                        else:
                            p = p_buf[b % 2, slot[(e, pos, kt)]]
                        if (h, kt) not in windows or not CFG.get("vcache", 1):
                            windows[(h, kt)] = value_window(s, g, j, kt)
                        r = _dot(windows[(h, kt)], p)
                        o = r if o is None else o + r
                    finish_column(s, g, j, i, o, s > 0)

        def proj_tasks(s, groups=range(NG)):
            return [(GW[g] // 16 * 15,
                     lambda s=s, tt=tt, g=g: proj_qkv(s, tt, g, s > 0, s < NSEG - 1))
                    for tt in range(4) for g in groups]

        def out_tasks(s, tts=range(4)):
            tasks = []
            for tt in tts:
                tasks += [(60, lambda s=s, tt=tt, fb=fb: proj_out(s, tt, fb, (s, tt) == (NSEG - 1, 0)))
                          for fb in range(3)]
                tasks.append((0, lambda s=s, tt=tt: out_copy(4 * s + tt).start()))
            return tasks

        def ln_tasks(s):
            ts = range(4 * s, 4 * s + 4)
            return ([(10, lambda t=t: ln_stats(t)) for t in ts]
                    + [(10, lambda t=t: ln_apply(t)) for t in ts]
                    + [(2, lambda t=t: router(t)) for t in ts])

        def upd_tasks(s):
            return [(GW[g] // 4, lambda s=s, g=g: mem_update(s, g, s == 0)) for g in range(NG)]

        def read_tasks(s):
            return [(GW[g] // 4 + 4, lambda s=s, g=g: mem_read(s, g)) for g in range(NG)]

        def prep_tasks(cbs):
            return [(5, lambda cb=cb, which=which: prep_wt(cb, which)) for cb in cbs for which in range(3)]

        guard = {}

        def norm_task(i, cb, part):
            acc = col_norm2(i, cb, part)
            if part > 0:
                acc = acc + guard[("acc", i)]
            else:
                acc = acc + paced(jnp.zeros((1, acc.shape[1]), F32), acc.shape[1])
            guard[("acc", i)] = acc
            if part == 2:
                row = jnp.sum(acc, axis=0, keepdims=True)
                if row.shape[1] < 128:
                    row = jnp.concatenate([row, jnp.zeros((1, 128 - row.shape[1]), F32)], axis=1)
                guard[i] = row if i not in guard else jnp.maximum(guard[i], row)

        def guard_task():
            nq, nk, nv = (jnp.max(guard[i]) for i in range(3))
            guard["safe"] = jnp.logical_and(
                nq * nk <= (SCORE_LIMIT / (1.05 * D * QSCALE * DH)) ** 2, nv <= 1e30)

        def norm_tasks(cbs):
            return [(1, lambda i=i, cb=cb, part=part: norm_task(i, cb, part))
                    for cb in cbs for i in range(3) for part in range(3)]

        seg0 = [min(k for k, blk in enumerate(blocks) if blk[0][0] == s) for s in range(NSEG)] + [nb]
        last = {i: max(k for k, blk in enumerate(blocks) if blk[0][0] == NSEG - 1 and blk[0][2] == i)
                for i in range(4)}

        def at(s, frac):
            return seg0[s] + round(frac * (seg0[s + 1] - seg0[s]))

        a1, a2, a3 = seg0[1], seg0[2], seg0[3]
        c2, c5 = CFG.get("c2", 2), CFG.get("c5", 5)
        streams = [
            (0, 1, prep_tasks((1, 2))),
            (0, 2, proj_tasks(0, (1,))),
            (c2, c2 + 1, prep_tasks((3, 4))),
            (c2, 4, proj_tasks(0, (2,))),
            (c2, c5, ln_tasks(1)),
            (4, 7, proj_tasks(0, (3, 4))),
            (6, a1 - 1, proj_tasks(1)),
            (8, 10, upd_tasks(0)),
            (a1 - 1, a1, read_tasks(1)),
            (c5 + 1, a1 - 1, ln_tasks(2) + ln_tasks(3)),
            (c5 + 1, a1, [(5, lambda g=g: prep_wo(g)) for g in range(NG)]),
            (a1 + 1, a3 - 1, norm_tasks(range(5))),
            (a3 + 1, a3 + 2, [(1, guard_task)]),
            (a1, a1 + 1, [(1, moe_select)]),
            (a1 + 1, at(1, 0.2), upd_tasks(1)),
            (a1, a2 - 1, proj_tasks(2)),
            (a2 - 1, a2, read_tasks(2)),
            (a2 + 1, at(2, 0.2), upd_tasks(2)),
            (a2, a3 - 1, proj_tasks(3)),
            (a3 - 1, a3, read_tasks(3)),
            (a3 - 1, a3, [(1, lambda: (emit_downs(len(downs)), moe_finish()))]),
            (a3 + 1, last[1] + 1, out_tasks(0) + out_tasks(1) + out_tasks(2)),
            (last[3] + 2, last[2] + 1, out_tasks(3, (3,))),
            (last[2] + 2, last[1] + 1, out_tasks(3, (2,))),
            (last[1] + 2, nb + 1, out_tasks(3, (1,))),
        ]
        nf = FF // 128
        micro_ranges = [(a1 + 1, a2 - 1, moe_up_tasks(range(nf // 2))),
                        (a2, a3 - 2, moe_up_tasks(range(nf // 2, nf)))]
        downs = moe_down_tasks(range(nf))
        dstate = [0]

        def emit_downs(limit):
            n = 0
            while dstate[0] < len(downs) and n < limit and ("h", downs[dstate[0]][0]) in moe:
                downs[dstate[0]][1]()
                dstate[0] += 1
                n += 1

        ntiles = [sum(len(u) * (i + 1) for (_, u, i) in blk) for blk in blocks]

        def fence_w12():
            wait_w(1)
            wait_w(2)

        def fence_w34():
            wait_w(3)
            wait_w(4)
            x_copy(1).wait()

        def fence_a1():
            wait_moe(0)
            start_moe(1)

        def fence_a0():
            x_copy(2).wait()
            x_copy(3).wait()
            wo_copy.wait()
            start_moe(0)

        fences = {0: fence_w12, c2: fence_w34, c5: fence_a0, a1: fence_a1, a2: lambda: wait_moe(1)}

        state = [[0, 0.0, float(sum(c for c, _ in t))] for _, _, t in streams]
        mstate = [[0, 0] for _ in micro_ranges]
        cur_scope = []

        def emit(b0, b1):
            for b in range(b0, b1 + 1):
                if _SCOPES and b % 4 == 0:
                    if cur_scope:
                        cur_scope.pop().__exit__(None, None, None)
                    cur_scope.append(jax.named_scope(f"blk{b:03d}"))
                    cur_scope[-1].__enter__()
                if b in fences and b < b1:
                    fences[b]()

                def micro(b=b):
                    for (lo, hi, tasks), ms in zip(micro_ranges, mstate):
                        if lo <= b < hi:
                            ms[0] += 1
                            total = sum(ntiles[lo:hi])
                            while ms[1] < len(tasks) and ms[1] < ms[0] * len(tasks) / total:
                                tasks[ms[1]]()
                                ms[1] += 1

                if b < b1:
                    scores(b, micro)
                if b < b1 or b == nb:
                    for (lo, hi, tasks), st_ in zip(streams, state):
                        if b < lo:
                            continue
                        frac = (b + 1 - lo) / (hi - lo)
                        while st_[0] < len(tasks) and st_[1] + tasks[st_[0]][0] / 2 <= frac * st_[2] + 1e-9:
                            st_[1] += tasks[st_[0]][0]
                            tasks[st_[0]][1]()
                            st_[0] += 1
                            if tasks[st_[0] - 1][0] >= 75 and a1 < b < a3:
                                emit_downs(CFG.get("dper", 5))
                if b > b0:
                    values(b - 1)
            if cur_scope:
                cur_scope.pop().__exit__(None, None, None)

        def wait_outputs():
            for t in range(4 * NSEG):
                out_copy(t).wait()

        emit(0, nb)
        for (lo, hi, tasks), st_ in zip(streams, state):
            assert st_[0] == len(tasks), (lo, hi, st_)
        assert all(ms[1] == len(r[2]) for ms, r in zip(mstate, micro_ranges)) and dstate[0] == len(downs)
        with scope("tail0"):
            for _, t in out_tasks(3, (0,)):
                t()

        def redo():
            wait_outputs()
            compact_path()

        if CFG.get("only") == "fast":
            wait_outputs()
        elif CFG.get("only") == "compact":
            redo()
        else:
            lax.cond(guard["safe"], wait_outputs, redo)

    def prep_group(g):
        for which in range(3):
            prep_wt(g, which)

    def wait_w(cb):
        for i in range(3):
            w_copy(i, cb).wait()

    def start_moe(c):
        for i in range(3):
            moe_copy(i, c).start()

    def wait_moe(c):
        for i in range(3):
            moe_copy(i, c).wait()

    def col_norm2(i, cb, part):
        n = 128 if cb < 4 else 64
        acc = None
        for u in range(3 * part, 3 * part + 3):
            wv = wraw[i, 64 * u:64 * (u + 1), 128 * cb:128 * cb + n].astype(F32)
            c = jnp.sum((wv * wv).reshape(8, 8, n), axis=0)
            acc = c if acc is None else acc + c
        return acc

    def scope(name):
        return jax.named_scope(name) if _SCOPES else contextlib.nullcontext()

    with scope("pre0"):
        for s in range(NSEG):
            for g in range(NG):
                n = DH * GN[g]
                for tt in range(4):
                    o_t[s, tt, 128 * g + n:128 * g + GW[g], :] = jnp.zeros((GW[g] - n, 128), BF)
        wr_copy.wait()
        x_copy(0, 0).wait()
        prep_wr()
        layernorm(0)
    with scope("pre1"):
        wait_w(0)
        prep_group(0)
        proj_qkv(0, 0, 0, False, True)
    with scope("pre2"):
        for tt in range(1, 4):
            x_copy(0, tt).wait()
        beta_copy.wait()
        for tt in range(1, 4):
            layernorm(tt)
            proj_qkv(0, tt, 0, False, True)
        prep_gates()
    run_pipeline()


@jax.jit
def pallas_parallel_sum__memory_aug_infini_attn__moe_arch_mod__prompt_kernel(
    A_x: jax.Array,
    A_wq: jax.Array,
    A_wk: jax.Array,
    A_wv: jax.Array,
    A_wo: jax.Array,
    A_beta: jax.Array,
    B_x: jax.Array,
    B_w_r: jax.Array,
    B_w_gate: jax.Array,
    B_w_up: jax.Array,
    B_w_down: jax.Array,
):
    del B_x
    hbm = pl.BlockSpec(memory_space=pltpu.HBM)
    scratch = [
        pltpu.VMEM((D, SEQ), BF),
        pltpu.VMEM((4 * NSEG, D, 128), BF),
        pltpu.VMEM((D, SEQ), F32),
        pltpu.VMEM((16, SEQ), F32),
        pltpu.VMEM((4, D, D), BF),
        pltpu.VMEM((3 * GP, D), BF),
        pltpu.VMEM((D, GP), BF),
        pltpu.VMEM((H,), BF),
        pltpu.VMEM((D,), BF),
        pltpu.VMEM((16, D), BF),
        pltpu.VMEM((D, FF), BF),
        pltpu.VMEM((D, FF), BF),
        pltpu.VMEM((D, FF), BF),
        pltpu.VMEM((NSEG, 4, GP, 128), BF),
        pltpu.VMEM((NSEG, 4, GP, 128), BF),
        pltpu.VMEM((NSEG, 4, GP, 128), BF),
        pltpu.VMEM((NSEG, NG, L, 128), BF),
        pltpu.VMEM((NSEG, 4, GP, 128), BF),
        pltpu.VMEM((NSEG, 4, GP, 128), BF),
        pltpu.VMEM((2, 20, 128, 128), BF),
        pltpu.VMEM((NSEG, GP, L), F32),
        pltpu.VMEM((NSEG, 16 * NG, L), F32),
        pltpu.VMEM((NG, 128, 128), F32),
        pltpu.VMEM((1, SEQ), F32),
        pltpu.VMEM((NG, 8, 128), F32),
        pltpu.VMEM((16, D), F32),
        pltpu.VMEM((4 * NSEG, D, 128), BF),
        pltpu.SemaphoreType.DMA((25,)),
        pltpu.SemaphoreType.DMA((3 * (FF // MOE_DMA),)),
        pltpu.SemaphoreType.DMA((4 * NSEG,)),
        pltpu.SemaphoreType.REGULAR,
    ]
    out_t = pl.pallas_call(
        _kernel,
        out_shape=jax.ShapeDtypeStruct((1, D, SEQ), BF),
        in_specs=[hbm] * 10,
        out_specs=hbm,
        scratch_shapes=scratch,
        compiler_params=pltpu.CompilerParams(vmem_limit_bytes=100 * 1024 * 1024),
    )(jnp.swapaxes(A_x, 1, 2), A_wq, A_wk, A_wv, A_wo, A_beta, B_w_r, B_w_gate, B_w_up,
      B_w_down.T)
    return jnp.swapaxes(out_t, 1, 2)
```

```python
import jax
import jax.numpy as jnp
from jax import lax
import jax.experimental.pallas as pl
import jax.experimental.pallas.tpu as pltpu

BF = jnp.bfloat16
F32 = jnp.float32

SEQ, D, H, DH = 2048, 576, 32, 18
NSEG, L, FF = 4, 512, 4608
HPG = 7
NG = 5
GN = (7, 7, 7, 7, 4)
GW = (128, 128, 128, 128, 80)
GP = 592
ZR = (126, 126, 126, 126, 78)
QSCALE = (DH ** -0.5) * 1.4426950408889634
NT_DIMS = (((1,), (1,)), ((), ()))
MOE_DMA = 2304
NMC = FF // MOE_DMA
OUT_ROWS = 192
NEG = -1e30
SCORE_LIMIT = 40.0
KTS = tuple((128 * k, min(128 * (k + 1), D)) for k in range(5))


def _dot(a, b):
    return jnp.dot(a, b, preferred_element_type=F32)


def _dot_nt(a, b):
    return lax.dot_general(a, b, NT_DIMS, preferred_element_type=F32)


def _iota(shape, dim):
    return lax.broadcasted_iota(jnp.int32, shape, dim)


def _phi(t):
    return jnp.where(t > 0, t + 1.0, jnp.exp(t))


def _sigmoid(t):
    return 1.0 / (1.0 + jnp.exp(-t))


def _recip(x):
    r = pl.reciprocal(x, approx=True)
    r = r * (2.0 - x * r)
    return r * (2.0 - x * r)


def _div18(i):
    return (i * 57) >> 10


def _blk(t, size=128):
    if isinstance(t, int):
        return slice(size * t, size * (t + 1))
    return pl.ds(pl.multiple_of(t * size, size), size)


def _rows(start, size, align):
    if isinstance(start, int):
        return slice(start, start + size)
    return pl.ds(pl.multiple_of(start, align), size)


def _kernel(x_hbm, wq_hbm, wk_hbm, wv_hbm, wo_hbm, beta_hbm, wr_hbm, wg_hbm, wu_hbm, wd_hbm,
            out_hbm,
            x_v, xn_v, res_v, stat_v, wraw, w_t, wo_t, beta_v, wr_v, wr_b, wg_v, wu_v, wd_v,
            q_t, pq_t, v_t, k_n, pk_t, o_t, p_buf, am_t, den_t, m_t, r_row, gate_t, out_v,
            sem_in, sem_moe, sem_out):

    def x_copy(s, tt=None):
        if tt is None:
            c0, n, k = s * L, L, 3 + s
        else:
            c0, n, k = tt * 128, 128, tt
        return pltpu.make_async_copy(x_hbm.at[0, :, pl.ds(c0, n)], x_v.at[:, pl.ds(c0, n)],
                                     sem_in.at[k])

    def w_copy(i, cb):
        src = (wq_hbm, wk_hbm, wv_hbm)[i]
        n = 128 if cb < 4 else 64
        return pltpu.make_async_copy(src.at[:, pl.ds(128 * cb, n)], wraw.at[i, :, pl.ds(128 * cb, n)],
                                     sem_in.at[7 + 5 * i + cb])

    wo_copy = pltpu.make_async_copy(wo_hbm, wraw.at[3], sem_in.at[22])
    beta_copy = pltpu.make_async_copy(beta_hbm, beta_v, sem_in.at[23])
    wr_copy = pltpu.make_async_copy(wr_hbm, wr_v, sem_in.at[24])

    def moe_copy(i, c):
        src, dst = ((wg_hbm, wg_v), (wu_hbm, wu_v), (wd_hbm, wd_v))[i]
        cs = pl.ds(c * MOE_DMA, MOE_DMA)
        return pltpu.make_async_copy(src.at[:, cs], dst.at[:, cs], sem_moe.at[i * NMC + c])

    def out_copy(t):
        cs = pl.ds(t * 128 if isinstance(t, int) else pl.multiple_of(t * 128, 128), 128)
        return pltpu.make_async_copy(out_v.at[t], out_hbm.at[0, :, cs], sem_out.at[t])

    wr_copy.start()
    x_copy(0, 0).start()
    for i in range(3):
        w_copy(i, 0).start()
    beta_copy.start()
    for tt in range(1, 4):
        x_copy(0, tt).start()
    for cb in range(1, 5):
        for i in range(3):
            w_copy(i, cb).start()
    x_copy(1).start()
    x_copy(2).start()
    x_copy(3).start()
    wo_copy.start()

    pace = {}

    def paced(row, lanes=128):
        tok = pace.get("tok")
        return row if tok is None else row + tok[:, :lanes] * 0.0

    def ln_stats(t):
        cols = _blk(t)
        shift = paced(x_v[0:16, cols].astype(F32)[0:1])
        s1 = [None] * 2
        s2 = [None] * 2
        for u in range(D // 16):
            d = x_v[16 * u:16 * (u + 1), cols].astype(F32) - shift
            d = d.reshape(2, 8, 128)
            for k in range(2):
                s1[k] = d[k] if u == 0 else s1[k] + d[k]
                s2[k] = d[k] * d[k] if u == 0 else s2[k] + d[k] * d[k]
        m1 = jnp.sum(s1[0] + s1[1], axis=0, keepdims=True) * (1.0 / D)
        m2 = jnp.sum(s2[0] + s2[1], axis=0, keepdims=True) * (1.0 / D)
        var = jnp.maximum(m2 - m1 * m1, 0.0)
        stat_v[0:1, cols] = m1 + shift
        stat_v[8:9, cols] = lax.rsqrt(var + 1e-5)

    def ln_apply(t):
        cols = _blk(t)
        mean = paced(stat_v[0:1, cols])
        rstd = stat_v[8:9, cols]
        for u in range(D // 48):
            rows = slice(48 * u, 48 * (u + 1))
            x = x_v[rows, cols].astype(F32)
            xn = (x - mean) * rstd
            xn_v[t, rows, :] = xn.astype(BF)
            res_v[rows, cols] = x + xn

    def router(t):
        r = _dot(wr_b[...], xn_v[t])
        r_row[:, _blk(t)] = r[0:1].astype(BF).astype(F32)

    def layernorm(t):
        ln_stats(t)
        ln_apply(t)
        router(t)

    def prep_wr():
        wr = wr_v[...].reshape(1, D)
        wr_b[...] = jnp.broadcast_to(wr.astype(F32), (16, D)).astype(BF)

    def prep_wt(cb, which):
        nb = 128 if cb < 4 else 64
        n = DH * GN[cb]
        t = wraw[which, :, 128 * cb:128 * cb + nb].T
        r0 = 384 * cb + which * GW[cb]
        k = min(n - 2 * cb, nb)
        w_t[r0 + 2 * cb:r0 + 2 * cb + k, :] = t[0:k]
        w_t[r0 + n:r0 + GW[cb], :] = jnp.zeros((GW[cb] - n, D), BF)
        if cb < 4:
            r1 = 384 * (cb + 1) + which * GW[cb + 1]
            w_t[r1:r1 + 2 * (cb + 1), :] = t[128 - 2 * (cb + 1):128]

    def prep_wo(g):
        n = DH * GN[g]
        wo_t[:, 128 * g:128 * g + n] = wraw[3, 126 * g:126 * g + n, :].T
        wo_t[:, 128 * g + n:128 * g + GW[g]] = jnp.zeros((D, GW[g] - n), BF)

    def prep_gates():
        b = beta_v[...].astype(F32).reshape(1, H)
        sig = jnp.concatenate([_sigmoid(b), jnp.zeros((1, 128 - H), F32)], axis=1)
        rows = jnp.broadcast_to(sig, (128, 128)).T
        for g in range(NG):
            gate_t[g] = rows[HPG * g:HPG * g + 8]

    def proj_qkv(s, tt, g, need_pq=True, need_pk=True):
        w = GW[g]
        rows = slice(128 * g, 128 * g + w)
        r = _dot(w_t[384 * g:384 * g + 3 * w, :], xn_v[4 * s + tt])
        q, k, v = r[:w], r[w:2 * w], r[2 * w:]
        q_t[s, tt, rows, :] = (q * QSCALE).astype(BF)
        if need_pq:
            pq_t[s, tt, rows, :] = _phi(q).astype(BF)
        k_n[s, g, _blk(tt), :w] = k.astype(BF).T
        if need_pk:
            pk_t[s, tt, rows, :] = _phi(k).astype(BF)
        v = jnp.where(_iota((w, 128), 0) == ZR[g], 1.0, v)
        v_t[s, tt, rows, :] = v.astype(BF)

    def mem_update(s, g, first):
        w = GW[g]
        rows = slice(128 * g, 128 * g + w)
        r = _dot_nt(v_t[s, 0, rows, :], pk_t[s, 0, rows, :])
        for tt in range(1, 4):
            r = r + _dot_nt(v_t[s, tt, rows, :], pk_t[s, tt, rows, :])
        rr, cc = _iota((w, w), 0), _iota((w, w), 1)
        keep = (cc < DH * GN[g]) & ((_div18(rr) == _div18(cc)) | (rr == ZR[g]))
        r = jnp.where(keep, r, 0.0)
        if not first:
            r = r + m_t[g, :w, :w]
        m_t[g, :w, :w] = r

    def mem_read(s, g):
        w = GW[g]
        rows = slice(128 * g, 128 * g + w)
        m = m_t[g, :w, :w]
        z = m[ZR[g]:ZR[g] + 1, :]
        zrows = jnp.where(_iota((16, w), 0) == _div18(_iota((16, w), 1)), z, 0.0)
        lhs = jnp.concatenate([m, zrows], axis=0).astype(BF)
        for tt in range(4):
            cols = slice(128 * tt, 128 * (tt + 1))
            r = _dot(lhs, pq_t[s, tt, rows, :])
            am_t[s, rows, cols] = r[:w]
            den_t[s, 16 * g:16 * (g + 1), cols] = r[w:]

    def proj_out(s, tt, fb, by_group=False):
        f0 = OUT_ROWS * fb
        f1 = f0 + OUT_ROWS
        if by_group:
            p = None
            for g in range(NG):
                r = _dot(wo_t[f0:f1, 128 * g:128 * g + GW[g]], o_t[s, tt, 128 * g:128 * g + GW[g], :])
                p = r if p is None else p + r
        else:
            p = _dot(wo_t[f0:f1, :], o_t[s, tt])
        out_v[4 * s + tt, f0:f1, :] = (p + res_v[f0:f1, _blk(4 * s + tt)]).astype(BF)

    moe = {}

    def moe_select():
        r = r_row[...]
        io = _iota((1, SEQ), 1)
        m1 = jnp.max(r)
        i1 = jnp.min(jnp.where(r == m1, io, SEQ - 1))
        r2 = jnp.where(io == i1, -jnp.inf, r)
        m2 = jnp.max(r2)
        i2 = jnp.min(jnp.where((r2 == m2) & (io != i1), io, SEQ - 1))
        rows = []
        for i in (i1, i2):
            xb = xn_v[i // 128].T.astype(F32)
            rows.append(jnp.sum(jnp.where(_iota((128, D), 0) == i % 128, xb, 0.0), axis=0, keepdims=True))
        rr = _iota((16, D), 0)
        xs = jnp.where(rr == 0, rows[0], jnp.where(rr == 1, rows[1], 0.0))
        moe["x"] = xs.astype(BF)
        moe["w"] = _sigmoid(jnp.where(_iota((16, 1), 0) == 0, m1, m2))
        sel = jnp.where(_iota((2, 128), 0) == 0, i1, i2)
        for t in range(4 * NSEG):
            tok = _iota((2, 128), 1) + 128 * t
            o_t[t // 4, t % 4, 126:128, :] = jnp.where(tok == sel, 1.0, 0.0).astype(BF)

    def moe_up(name, ref, f, k):
        k0, k1 = KTS[k]
        r = _dot(moe["x"][:, k0:k1], ref[k0:k1, _blk(f)])
        moe[name] = r if k == 0 else moe[name] + r

    def moe_hidden(f):
        g = moe["g"]
        moe[("h", f if isinstance(f, int) else 0)] = (g * _sigmoid(g) * moe["u"]).astype(BF)

    def moe_down(f, n, first):
        n0, n1 = KTS[n]
        r = _dot_nt(moe[("h", f if isinstance(f, int) else 0)], wd_v[n0:n1, _blk(f)])
        moe[("y", n)] = r if first else moe[("y", n)] + r

    def moe_up_tasks(fs):
        tasks = []
        for f in fs:
            tasks += [lambda f=f, k=k: moe_up("g", wg_v, f, k) for k in range(5)]
            tasks += [lambda f=f, k=k: moe_up("u", wu_v, f, k) for k in range(4)]
            tasks.append(lambda f=f: (moe_up("u", wu_v, f, 4), moe_hidden(f)))
        return tasks

    def moe_down_tasks(fs):
        return [(f, lambda f=f, n=n: moe_down(f, n, f == 0)) for f in fs for n in range(5)]

    def moe_finish():
        y = jnp.concatenate([moe[("y", n)] for n in range(5)], axis=1) * moe["w"]
        rr = _iota((128, D), 0)
        ypad = jnp.where(rr == 126, y[0:1], jnp.where(rr == 127, y[1:2], 0.0))
        cur = wo_t[:, 0:128].astype(F32)
        wo_t[:, 0:128] = jnp.where(_iota((D, 128), 1) >= 126, ypad.T, cur).astype(BF)

    causal = _iota((128, 128), 0) <= _iota((128, 128), 1)
    wrow = _iota((32, 128), 0)

    def query_weights(s, g, j, i, w):
        wq = q_t[s, i, _rows(128 * g + 16 * j, 32, 16), :]
        wq = jnp.where((wrow >= 2 * j) & (wrow < 2 * j + DH), wq, jnp.zeros_like(wq))
        parts = [wq]
        if j > 0:
            parts.insert(0, jnp.zeros((16 * j, 128), BF))
        if w - 16 * j - 32 > 0:
            parts.append(jnp.zeros((w - 16 * j - 32, 128), BF))
        return jnp.concatenate(parts, axis=0) if len(parts) > 1 else wq

    def key_tile(s, g, kt, w):
        return k_n[s, g, 128 * kt:128 * (kt + 1), :w]

    def score_tile(s, g, i, kt, w, wq):
        d = _dot(key_tile(s, g, kt, w), wq)
        return jnp.where(causal, d, NEG) if kt == i else d

    def value_window(s, g, j, kt):
        v = v_t[s, kt, _rows(128 * g + 16 * j, 32, 16), :]
        return jnp.where(wrow >= 30, jnp.ones_like(v), v)

    def value_tile(s, g, j, kt, p):
        return _dot(value_window(s, g, j, kt), p)

    def finish_column(s, g, j, i, o, with_mem):
        cols = slice(128 * i, 128 * (i + 1))
        win = _rows(128 * g + 16 * j, 32, 16)
        gate = gate_t[g][j:j + 1]
        scale = (1.0 - gate) * _recip(o[31:32, :])
        if isinstance(g, int):
            pace["tok"] = scale
        o = o * scale
        if with_mem:
            den = den_t[s, _rows(16 * g, 16, 16), cols][j:j + 1] + 1e-6
            o = o + am_t[s, win, cols] * (gate * _recip(den))
        if isinstance(g, int):
            r0 = 128 * g + DH * j
            o_t[s, i, r0:r0 + DH, :] = o[2 * j:2 * j + DH].astype(BF)
        else:
            mine = (wrow >= 2 * j) & (wrow < 2 * j + DH)
            o_t[s, i, win, :] = jnp.where(mine, o, o_t[s, i, win, :].astype(F32)).astype(BF)

    def running_max(m, d):
        pm = jnp.max(d.reshape(16, 8, 128), axis=0)
        return pm if m is None else jnp.maximum(m, pm)

    def compact_path():
        pace.clear()
        for g in range(NG):
            prep_wo(g)
            m_t[g] = jnp.zeros((128, 128), F32)
        am_t[0] = jnp.zeros((GP, L), F32)
        den_t[0] = jnp.ones((16 * NG, L), F32)

        @pl.loop(0, 4 * NSEG)
        def _(t):
            layernorm(t)

        moe_select()

        def expert(f, y):
            for k in range(5):
                moe_up("g", wg_v, f, k)
            for k in range(5):
                moe_up("u", wu_v, f, k)
            moe_hidden(f)
            for n in range(5):
                moe[("y", n)] = y[n]
                moe_down(f, n, False)
            return tuple(moe[("y", n)] for n in range(5))

        y = lax.fori_loop(0, FF // 128, expert,
                          tuple(jnp.zeros((16, k1 - k0), F32) for k0, k1 in KTS))
        for n in range(5):
            moe[("y", n)] = y[n]
        moe_finish()

        def head(s, g, j, w):
            for i in range(4):
                wq = query_weights(s, g, j, i, w)
                tiles, m = [], None
                for kt in range(i + 1):
                    tiles.append(score_tile(s, g, i, kt, w, wq))
                    m = running_max(m, tiles[-1])
                m = jnp.max(m, axis=0, keepdims=True)
                o = None
                for kt in range(i + 1):
                    r = value_tile(s, g, j, kt, jnp.exp2(tiles[kt] - m).astype(BF))
                    o = r if o is None else o + r
                finish_column(s, g, j, i, o, True)
                pace.clear()

        @pl.loop(0, NSEG)
        def _(s):
            @pl.loop(0, 4)
            def _(tt):
                for g in range(NG):
                    proj_qkv(s, tt, g)

            @pl.when(s > 0)
            def _():
                for g in range(NG):
                    mem_read(s, g)

            @pl.loop(0, NG - 1)
            def _(g):
                for j in range(HPG):
                    head(s, g, j, 128)

            for j in range(GN[NG - 1]):
                head(s, NG - 1, j, GW[NG - 1])
            for g in range(NG):
                mem_update(s, g, False)

            @pl.loop(0, 4)
            def _(tt):
                for fb in range(D // OUT_ROWS):
                    proj_out(s, tt, fb)
                out_copy(4 * s + tt).start()

    def head_units():
        units, h = [], 0
        while h < H:
            g, j = divmod(h, HPG)
            if j + 1 < GN[g]:
                units.append((h, h + 1))
                h += 2
            else:
                units.append((h,))
                h += 1
        return units

    def make_blocks():
        blocks = []
        for s in range(NSEG - 1):
            blocks += [[(s, u, i) for i in (3, 2, 1, 0)] for u in head_units()]
        s = NSEG - 1
        for i, budget in ((3, 16), (2, 18), (1, 20), (0, 20)):
            cur, n = [], 0
            for u in head_units():
                cost = len(u) * (i + 1)
                if cur and (n + cost > budget or (i == 0 and u[0] % HPG == 0)):
                    blocks.append(cur)
                    cur, n = [], 0
                cur.append((s, u, i))
                n += cost
            blocks.append(cur)
        return blocks

    col128 = _iota((64, 128), 1)
    mix_mask = _iota((64, 128), 0) <= (col128 & 63)

    def run_pipeline():
        blocks = make_blocks()
        nb = len(blocks)

        def slots(b):
            out, n = {}, 0
            for e, (_, heads, i) in enumerate(blocks[b]):
                for pos in range(len(heads)):
                    for kt in range(i + 1):
                        out[(e, pos, kt)] = n
                        n += 1
            return out

        def scores(b, micro):
            slot = slots(b)
            for e, (s, heads, i) in enumerate(blocks[b]):
                g = heads[0] // HPG
                w = GW[g]
                wqs = [query_weights(s, g, h % HPG, i, w) for h in heads]
                paired = len(heads) == 2
                for kt in range(i + 1):
                    half = paired and kt == i
                    keys = k_n[s, g, 128 * kt:128 * kt + (64 if half else 128), :w]
                    for pos in range(len(heads)):
                        d = _dot(keys, wqs[pos])
                        micro()
                        if kt == i:
                            d = jnp.where(causal[:d.shape[0]], d, NEG)
                        p_buf[b % 2, slot[(e, pos, kt)], 0:d.shape[0], :] = jnp.exp2(d).astype(BF)
                if paired:
                    wmix = jnp.concatenate([wqs[1][:, 64:], wqs[0][:, 64:]], axis=1)
                    d = _dot(k_n[s, g, 128 * i + 64:128 * (i + 1), :w], wmix)
                    ex = jnp.exp2(jnp.where(mix_mask, d, NEG))
                    zero = jnp.zeros((64, 64), F32)
                    p_buf[b % 2, slot[(e, 0, i)], 64:128, :] = jnp.where(col128 >= 64, ex, 0.0).astype(BF)
                    p_buf[b % 2, slot[(e, 1, i)], 64:128, :] = jnp.concatenate(
                        [zero, ex[:, :64]], axis=1).astype(BF)

        def values(b):
            slot = slots(b)
            windows = {}
            for e, (s, heads, i) in enumerate(blocks[b]):
                for pos, h in enumerate(heads):
                    g, j = divmod(h, HPG)
                    o = None
                    for kt in range(i + 1):
                        if (h, kt) not in windows:
                            windows[(h, kt)] = value_window(s, g, j, kt)
                        r = _dot(windows[(h, kt)], p_buf[b % 2, slot[(e, pos, kt)]])
                        o = r if o is None else o + r
                    finish_column(s, g, j, i, o, s > 0)

        def proj_tasks(s, groups=range(NG)):
            return [(GW[g] // 16 * 15,
                     lambda s=s, tt=tt, g=g: proj_qkv(s, tt, g, s > 0, s < NSEG - 1))
                    for tt in range(4) for g in groups]

        def out_tasks(s, tts=range(4)):
            tasks = []
            for tt in tts:
                tasks += [(OUT_ROWS * 5 // 16, lambda s=s, tt=tt, fb=fb: proj_out(s, tt, fb, (s, tt) == (NSEG - 1, 0)))
                          for fb in range(D // OUT_ROWS)]
                tasks.append((0, lambda s=s, tt=tt: out_copy(4 * s + tt).start()))
            return tasks

        def ln_tasks(s):
            ts = range(4 * s, 4 * s + 4)
            return ([(10, lambda t=t: ln_stats(t)) for t in ts]
                    + [(10, lambda t=t: ln_apply(t)) for t in ts]
                    + [(2, lambda t=t: router(t)) for t in ts])

        def upd_tasks(s):
            return [(GW[g] // 4, lambda s=s, g=g: mem_update(s, g, s == 0)) for g in range(NG)]

        def read_tasks(s):
            return [(GW[g] // 4 + 4, lambda s=s, g=g: mem_read(s, g)) for g in range(NG)]

        def prep_tasks(cbs):
            return [(5, lambda cb=cb, which=which: prep_wt(cb, which)) for cb in cbs for which in range(3)]

        guard = {}

        def norm_task(i, cb, part):
            acc = col_norm2(i, cb, part)
            if part > 0:
                acc = acc + guard[("acc", i)]
            else:
                acc = acc + paced(jnp.zeros((1, acc.shape[1]), F32), acc.shape[1])
            guard[("acc", i)] = acc
            if part == 2:
                row = jnp.sum(acc, axis=0, keepdims=True)
                if row.shape[1] < 128:
                    row = jnp.concatenate([row, jnp.zeros((1, 128 - row.shape[1]), F32)], axis=1)
                guard[i] = row if i not in guard else jnp.maximum(guard[i], row)

        def guard_task():
            nq, nk, nv = (jnp.max(guard[i]) for i in range(3))
            guard["safe"] = jnp.logical_and(
                nq * nk <= (SCORE_LIMIT / (1.05 * D * QSCALE * DH)) ** 2, nv <= 1e30)

        def norm_tasks(cbs):
            return [(1, lambda i=i, cb=cb, part=part: norm_task(i, cb, part))
                    for cb in cbs for i in range(3) for part in range(3)]

        seg0 = [min(k for k, blk in enumerate(blocks) if blk[0][0] == s) for s in range(NSEG)] + [nb]
        last = {i: max(k for k, blk in enumerate(blocks) if blk[0][0] == NSEG - 1 and blk[0][2] == i)
                for i in range(4)}

        def at(s, frac):
            return seg0[s] + round(frac * (seg0[s + 1] - seg0[s]))

        a1, a2, a3 = seg0[1], seg0[2], seg0[3]
        streams = [
            (0, 1, prep_tasks((1, 2))),
            (0, 2, proj_tasks(0, (1,))),
            (2, 3, prep_tasks((3, 4))),
            (2, 4, proj_tasks(0, (2,))),
            (2, 5, ln_tasks(1)),
            (4, 7, proj_tasks(0, (3, 4))),
            (6, a1 - 1, proj_tasks(1)),
            (8, 10, upd_tasks(0)),
            (a1 - 1, a1, read_tasks(1)),
            (6, a1 - 1, ln_tasks(2) + ln_tasks(3)),
            (6, a1, [(5, lambda g=g: prep_wo(g)) for g in range(NG)]),
            (a3 + 1, nb - 6, norm_tasks(range(5))),
            (nb - 5, nb - 4, [(1, guard_task)]),
            (a1, a1 + 1, [(1, moe_select)]),
            (a1 + 1, at(1, 0.2), upd_tasks(1)),
            (a1, a2 - 1, proj_tasks(2)),
            (a2 - 1, a2, read_tasks(2)),
            (a2 + 1, at(2, 0.2), upd_tasks(2)),
            (a2, a3 - 1, proj_tasks(3)),
            (a3 - 1, a3, read_tasks(3)),
            (a3 - 1, a3, [(1, lambda: (emit_downs(len(downs)), moe_finish()))]),
            (a3 + 1, last[1] + 1, out_tasks(0) + out_tasks(1) + out_tasks(2)),
            (last[3] + 2, last[2] + 1, out_tasks(3, (3,))),
            (last[2] + 2, last[1] + 1, out_tasks(3, (2,))),
            (last[1] + 2, nb + 1, out_tasks(3, (1,))),
        ]
        nf = FF // 128
        micro_ranges = [(a1 + 1, a2 - 1, moe_up_tasks(range(nf // 2))),
                        (a2, a3 - 2, moe_up_tasks(range(nf // 2, nf)))]
        downs = moe_down_tasks(range(nf))
        dstate = [0]

        def emit_downs(limit):
            n = 0
            while dstate[0] < len(downs) and n < limit and ("h", downs[dstate[0]][0]) in moe:
                downs[dstate[0]][1]()
                dstate[0] += 1
                n += 1

        ntiles = [sum(len(u) * (i + 1) for (_, u, i) in blk) for blk in blocks]

        def fence_w12():
            wait_w(1)
            wait_w(2)

        def fence_w34():
            wait_w(3)
            wait_w(4)
            x_copy(1).wait()

        def fence_a1():
            wait_moe(0)
            start_moe(1)

        def fence_a0():
            x_copy(2).wait()
            x_copy(3).wait()
            wo_copy.wait()
            start_moe(0)

        fences = {0: fence_w12, 2: fence_w34, 5: fence_a0, a1: fence_a1, a2: lambda: wait_moe(1)}

        state = [[0, 0.0, float(sum(c for c, _ in t))] for _, _, t in streams]
        mstate = [[0, 0] for _ in micro_ranges]

        for b in range(nb + 1):
            if b in fences:
                fences[b]()

            def micro(b=b):
                for (lo, hi, tasks), ms in zip(micro_ranges, mstate):
                    if lo <= b < hi:
                        ms[0] += 1
                        total = sum(ntiles[lo:hi])
                        while ms[1] < len(tasks) and ms[1] < ms[0] * len(tasks) / total:
                            tasks[ms[1]]()
                            ms[1] += 1

            if b < nb:
                scores(b, micro)
            for (lo, hi, tasks), st_ in zip(streams, state):
                if b < lo:
                    continue
                frac = (b + 1 - lo) / (hi - lo)
                while st_[0] < len(tasks) and st_[1] + tasks[st_[0]][0] / 2 <= frac * st_[2] + 1e-9:
                    cost, task = tasks[st_[0]]
                    task()
                    st_[1] += cost
                    st_[0] += 1
                    if cost >= 75 and a1 < b < a3:
                        emit_downs(5)
            if b > 0:
                values(b - 1)
        for (lo, hi, tasks), st_ in zip(streams, state):
            assert st_[0] == len(tasks), (lo, hi, st_)
        assert all(ms[1] == len(r[2]) for ms, r in zip(mstate, micro_ranges)) and dstate[0] == len(downs)
        for _, t in out_tasks(3, (0,)):
            t()

        def wait_outputs():
            for t in range(4 * NSEG):
                out_copy(t).wait()

        @pl.when(jnp.logical_not(guard["safe"]))
        def _():
            wait_outputs()
            compact_path()

        wait_outputs()

    def prep_group(g):
        for which in range(3):
            prep_wt(g, which)

    def wait_w(cb):
        for i in range(3):
            w_copy(i, cb).wait()

    def start_moe(c):
        for i in range(3):
            moe_copy(i, c).start()

    def wait_moe(c):
        for i in range(3):
            moe_copy(i, c).wait()

    def col_norm2(i, cb, part):
        n = 128 if cb < 4 else 64
        acc = None
        for u in range(3 * part, 3 * part + 3):
            wv = wraw[i, 64 * u:64 * (u + 1), 128 * cb:128 * cb + n].astype(F32)
            c = jnp.sum((wv * wv).reshape(8, 8, n), axis=0)
            acc = c if acc is None else acc + c
        return acc

    for s in range(NSEG):
        for g in range(NG):
            n = DH * GN[g]
            for tt in range(4):
                o_t[s, tt, 128 * g + n:128 * g + GW[g], :] = jnp.zeros((GW[g] - n, 128), BF)
    wr_copy.wait()
    x_copy(0, 0).wait()
    prep_wr()
    layernorm(0)
    wait_w(0)
    prep_group(0)
    proj_qkv(0, 0, 0, False, True)
    for tt in range(1, 4):
        x_copy(0, tt).wait()
    beta_copy.wait()
    for tt in range(1, 4):
        layernorm(tt)
        proj_qkv(0, tt, 0, False, True)
    prep_gates()
    run_pipeline()


@jax.jit
def pallas_parallel_sum__memory_aug_infini_attn__moe_arch_mod__prompt_kernel(
    A_x: jax.Array,
    A_wq: jax.Array,
    A_wk: jax.Array,
    A_wv: jax.Array,
    A_wo: jax.Array,
    A_beta: jax.Array,
    B_x: jax.Array,
    B_w_r: jax.Array,
    B_w_gate: jax.Array,
    B_w_up: jax.Array,
    B_w_down: jax.Array,
):
    del B_x
    hbm = pl.BlockSpec(memory_space=pltpu.HBM)
    scratch = [
        pltpu.VMEM((D, SEQ), BF),
        pltpu.VMEM((4 * NSEG, D, 128), BF),
        pltpu.VMEM((D, SEQ), F32),
        pltpu.VMEM((16, SEQ), F32),
        pltpu.VMEM((4, D, D), BF),
        pltpu.VMEM((3 * GP, D), BF),
        pltpu.VMEM((D, GP), BF),
        pltpu.VMEM((H,), BF),
        pltpu.VMEM((D,), BF),
        pltpu.VMEM((16, D), BF),
        pltpu.VMEM((D, FF), BF),
        pltpu.VMEM((D, FF), BF),
        pltpu.VMEM((D, FF), BF),
        pltpu.VMEM((NSEG, 4, GP, 128), BF),
        pltpu.VMEM((NSEG, 4, GP, 128), BF),
        pltpu.VMEM((NSEG, 4, GP, 128), BF),
        pltpu.VMEM((NSEG, NG, L, 128), BF),
        pltpu.VMEM((NSEG, 4, GP, 128), BF),
        pltpu.VMEM((NSEG, 4, GP, 128), BF),
        pltpu.VMEM((2, 20, 128, 128), BF),
        pltpu.VMEM((NSEG, GP, L), F32),
        pltpu.VMEM((NSEG, 16 * NG, L), F32),
        pltpu.VMEM((NG, 128, 128), F32),
        pltpu.VMEM((1, SEQ), F32),
        pltpu.VMEM((NG, 8, 128), F32),
        pltpu.VMEM((4 * NSEG, D, 128), BF),
        pltpu.SemaphoreType.DMA((25,)),
        pltpu.SemaphoreType.DMA((3 * NMC,)),
        pltpu.SemaphoreType.DMA((4 * NSEG,)),
    ]
    out_t = pl.pallas_call(
        _kernel,
        out_shape=jax.ShapeDtypeStruct((1, D, SEQ), BF),
        in_specs=[hbm] * 10,
        out_specs=hbm,
        scratch_shapes=scratch,
        compiler_params=pltpu.CompilerParams(vmem_limit_bytes=100 * 1024 * 1024),
    )(jnp.swapaxes(A_x, 1, 2), A_wq, A_wk, A_wv, A_wo, A_beta, B_w_r, B_w_gate, B_w_up,
      B_w_down.T)
    return jnp.swapaxes(out_t, 1, 2)
```

```python
import jax
import jax.numpy as jnp
from jax import lax
import jax.experimental.pallas as pl
import jax.experimental.pallas.tpu as pltpu

BF = jnp.bfloat16
F32 = jnp.float32

SEQ, D, H, DH = 2048, 576, 32, 18
NSEG, L, FF = 4, 512, 4608
HPG = 7
NG = 5
GN = (7, 7, 7, 7, 4)
GW = (128, 128, 128, 128, 80)
GP = 592
ZR = (126, 126, 126, 126, 78)
QSCALE = (DH ** -0.5) * 1.4426950408889634
NT_DIMS = (((1,), (1,)), ((), ()))
MOE_DMA = 2304
NMC = FF // MOE_DMA
OUT_ROWS = 192
NEG = -1e30
SCORE_LIMIT = 40.0
KTS = tuple((128 * k, min(128 * (k + 1), D)) for k in range(5))


def _dot(a, b):
    return jnp.dot(a, b, preferred_element_type=F32)


def _dot_nt(a, b):
    return lax.dot_general(a, b, NT_DIMS, preferred_element_type=F32)


def _iota(shape, dim):
    return lax.broadcasted_iota(jnp.int32, shape, dim)


def _phi(t):
    return jnp.where(t > 0, t + 1.0, jnp.exp(t))


def _sigmoid(t):
    return 1.0 / (1.0 + jnp.exp(-t))


def _div18(i):
    return (i * 57) >> 10


def _blk(t, size=128):
    if isinstance(t, int):
        return slice(size * t, size * (t + 1))
    return pl.ds(pl.multiple_of(t * size, size), size)


def _rows(start, size, align):
    if isinstance(start, int):
        return slice(start, start + size)
    return pl.ds(pl.multiple_of(start, align), size)


def _kernel(x_hbm, wq_hbm, wk_hbm, wv_hbm, wo_hbm, beta_hbm, wr_hbm, wg_hbm, wu_hbm, wd_hbm,
            out_hbm,
            x_v, xn_v, stat_v, wraw, w_t, wo_t, beta_v, wr_v, wr_b, wg_v, wu_v, wd_v,
            q_t, pq_t, v_t, k_n, pk_t, o_t, p_buf, am_t, den_t, m_t, r_row, gate_t, out_v,
            sem_in, sem_moe, sem_out):

    def x_copy(s, tt=None):
        if tt is None:
            c0, n, k = s * L, L, 3 + s
        else:
            c0, n, k = tt * 128, 128, tt
        return pltpu.make_async_copy(x_hbm.at[0, :, pl.ds(c0, n)], x_v.at[:, pl.ds(c0, n)],
                                     sem_in.at[k])

    def w_copy(i, cb):
        src = (wq_hbm, wk_hbm, wv_hbm)[i]
        n = 128 if cb < 4 else 64
        return pltpu.make_async_copy(src.at[:, pl.ds(128 * cb, n)], wraw.at[i, :, pl.ds(128 * cb, n)],
                                     sem_in.at[7 + 5 * i + cb])

    wo_copy = pltpu.make_async_copy(wo_hbm, wraw.at[3], sem_in.at[22])
    beta_copy = pltpu.make_async_copy(beta_hbm, beta_v, sem_in.at[23])
    wr_copy = pltpu.make_async_copy(wr_hbm, wr_v, sem_in.at[24])

    def moe_copy(i, c):
        src, dst = ((wg_hbm, wg_v), (wu_hbm, wu_v), (wd_hbm, wd_v))[i]
        cs = pl.ds(c * MOE_DMA, MOE_DMA)
        return pltpu.make_async_copy(src.at[:, cs], dst.at[:, cs], sem_moe.at[i * NMC + c])

    def out_copy(t):
        cs = pl.ds(t * 128 if isinstance(t, int) else pl.multiple_of(t * 128, 128), 128)
        return pltpu.make_async_copy(out_v.at[t], out_hbm.at[0, :, cs], sem_out.at[t])

    wr_copy.start()
    x_copy(0, 0).start()
    for i in range(3):
        w_copy(i, 0).start()
    beta_copy.start()
    for tt in range(1, 4):
        x_copy(0, tt).start()
    for cb in range(1, 5):
        for i in range(3):
            w_copy(i, cb).start()
    x_copy(1).start()
    x_copy(2).start()
    x_copy(3).start()
    wo_copy.start()

    pace = {}

    def paced(row, lanes=128):
        tok = pace.get("tok")
        return row if tok is None else row + tok[:, :lanes] * 0.0

    def ln_stats(t):
        cols = _blk(t)
        shift = paced(x_v[0:16, cols].astype(F32)[0:1])
        s1 = [None] * 2
        s2 = [None] * 2
        for u in range(D // 16):
            d = x_v[16 * u:16 * (u + 1), cols].astype(F32) - shift
            d = d.reshape(2, 8, 128)
            for k in range(2):
                s1[k] = d[k] if u == 0 else s1[k] + d[k]
                s2[k] = d[k] * d[k] if u == 0 else s2[k] + d[k] * d[k]
        m1 = jnp.sum(s1[0] + s1[1], axis=0, keepdims=True) * (1.0 / D)
        m2 = jnp.sum(s2[0] + s2[1], axis=0, keepdims=True) * (1.0 / D)
        var = jnp.maximum(m2 - m1 * m1, 0.0)
        stat_v[0:1, cols] = m1 + shift
        stat_v[8:9, cols] = lax.rsqrt(var + 1e-5)

    def ln_apply(t):
        cols = _blk(t)
        mean = paced(stat_v[0:1, cols])
        rstd = stat_v[8:9, cols]
        for u in range(D // 48):
            rows = slice(48 * u, 48 * (u + 1))
            xn_v[t, rows, :] = ((x_v[rows, cols].astype(F32) - mean) * rstd).astype(BF)

    def router(t):
        r = _dot(wr_b[...], xn_v[t])
        r_row[:, _blk(t)] = r[0:1].astype(BF).astype(F32)

    def layernorm(t):
        ln_stats(t)
        ln_apply(t)
        router(t)

    def prep_wr():
        wr = wr_v[...].reshape(1, D)
        wr_b[...] = jnp.broadcast_to(wr.astype(F32), (16, D)).astype(BF)

    def prep_wt(cb, which):
        nb = 128 if cb < 4 else 64
        n = DH * GN[cb]
        t = wraw[which, :, 128 * cb:128 * cb + nb].T
        r0 = 384 * cb + which * GW[cb]
        k = min(n - 2 * cb, nb)
        w_t[r0 + 2 * cb:r0 + 2 * cb + k, :] = t[0:k]
        w_t[r0 + n:r0 + GW[cb], :] = jnp.zeros((GW[cb] - n, D), BF)
        if cb < 4:
            r1 = 384 * (cb + 1) + which * GW[cb + 1]
            w_t[r1:r1 + 2 * (cb + 1), :] = t[128 - 2 * (cb + 1):128]

    def prep_wo(g):
        n = DH * GN[g]
        wo_t[:, 128 * g:128 * g + n] = wraw[3, 126 * g:126 * g + n, :].T
        wo_t[:, 128 * g + n:128 * g + GW[g]] = jnp.zeros((D, GW[g] - n), BF)

    def prep_gates():
        b = beta_v[...].astype(F32).reshape(1, H)
        sig = jnp.concatenate([_sigmoid(b), jnp.zeros((1, 128 - H), F32)], axis=1)
        rows = jnp.broadcast_to(sig, (128, 128)).T
        for g in range(NG):
            gate_t[g] = rows[HPG * g:HPG * g + 8]

    def proj_qkv(s, tt, g, need_pq=True, need_pk=True):
        w = GW[g]
        rows = slice(128 * g, 128 * g + w)
        r = _dot(w_t[384 * g:384 * g + 3 * w, :], xn_v[4 * s + tt])
        q, k, v = r[:w], r[w:2 * w], r[2 * w:]
        q_t[s, tt, rows, :] = (q * QSCALE).astype(BF)
        if need_pq:
            pq_t[s, tt, rows, :] = _phi(q).astype(BF)
        k_n[s, g, _blk(tt), :w] = k.astype(BF).T
        if need_pk:
            pk_t[s, tt, rows, :] = _phi(k).astype(BF)
        v = jnp.where(_iota((w, 128), 0) == ZR[g], 1.0, v)
        v_t[s, tt, rows, :] = v.astype(BF)

    def mem_update(s, g, first):
        w = GW[g]
        rows = slice(128 * g, 128 * g + w)
        r = _dot_nt(v_t[s, 0, rows, :], pk_t[s, 0, rows, :])
        for tt in range(1, 4):
            r = r + _dot_nt(v_t[s, tt, rows, :], pk_t[s, tt, rows, :])
        rr, cc = _iota((w, w), 0), _iota((w, w), 1)
        keep = (cc < DH * GN[g]) & ((_div18(rr) == _div18(cc)) | (rr == ZR[g]))
        r = jnp.where(keep, r, 0.0)
        if not first:
            r = r + m_t[g, :w, :w]
        m_t[g, :w, :w] = r

    def mem_read(s, g):
        w = GW[g]
        rows = slice(128 * g, 128 * g + w)
        m = m_t[g, :w, :w]
        z = m[ZR[g]:ZR[g] + 1, :]
        zrows = jnp.where(_iota((16, w), 0) == _div18(_iota((16, w), 1)), z, 0.0)
        lhs = jnp.concatenate([m, zrows], axis=0).astype(BF)
        for tt in range(4):
            cols = slice(128 * tt, 128 * (tt + 1))
            r = _dot(lhs, pq_t[s, tt, rows, :])
            am_t[s, rows, cols] = r[:w]
            den_t[s, 16 * g:16 * (g + 1), cols] = r[w:]

    def proj_out(s, tt, fb, by_group=False):
        f0 = OUT_ROWS * fb
        f1 = f0 + OUT_ROWS
        if by_group:
            p = None
            for g in range(NG):
                r = _dot(wo_t[f0:f1, 128 * g:128 * g + GW[g]], o_t[s, tt, 128 * g:128 * g + GW[g], :])
                p = r if p is None else p + r
        else:
            p = _dot(wo_t[f0:f1, :], o_t[s, tt])
        t = 4 * s + tt
        res = x_v[f0:f1, _blk(t)].astype(F32) + xn_v[t, f0:f1, :].astype(F32)
        out_v[t, f0:f1, :] = (p + res).astype(BF)

    moe = {}

    def moe_select():
        r = r_row[...]
        io = _iota((1, SEQ), 1)
        m1 = jnp.max(r)
        i1 = jnp.min(jnp.where(r == m1, io, SEQ - 1))
        r2 = jnp.where(io == i1, -jnp.inf, r)
        m2 = jnp.max(r2)
        i2 = jnp.min(jnp.where((r2 == m2) & (io != i1), io, SEQ - 1))
        rows = []
        for i in (i1, i2):
            xb = xn_v[i // 128].T.astype(F32)
            rows.append(jnp.sum(jnp.where(_iota((128, D), 0) == i % 128, xb, 0.0), axis=0, keepdims=True))
        rr = _iota((16, D), 0)
        xs = jnp.where(rr == 0, rows[0], jnp.where(rr == 1, rows[1], 0.0))
        moe["x"] = xs.astype(BF)
        moe["w"] = _sigmoid(jnp.where(_iota((16, 1), 0) == 0, m1, m2))
        sel = jnp.where(_iota((2, 128), 0) == 0, i1, i2)
        for t in range(4 * NSEG):
            tok = _iota((2, 128), 1) + 128 * t
            o_t[t // 4, t % 4, 126:128, :] = jnp.where(tok == sel, 1.0, 0.0).astype(BF)

    def moe_up(name, ref, f, k):
        k0, k1 = KTS[k]
        r = _dot(moe["x"][:, k0:k1], ref[k0:k1, _blk(f)])
        moe[name] = r if k == 0 else moe[name] + r

    def moe_hidden(f):
        g = moe["g"]
        moe[("h", f if isinstance(f, int) else 0)] = (g * _sigmoid(g) * moe["u"]).astype(BF)

    def moe_down(f, n, first):
        n0, n1 = KTS[n]
        r = _dot_nt(moe[("h", f if isinstance(f, int) else 0)], wd_v[n0:n1, _blk(f)])
        moe[("y", n)] = r if first else moe[("y", n)] + r

    def moe_up_tasks(fs):
        tasks = []
        for f in fs:
            tasks += [lambda f=f, k=k: moe_up("g", wg_v, f, k) for k in range(5)]
            tasks += [lambda f=f, k=k: moe_up("u", wu_v, f, k) for k in range(4)]
            tasks.append(lambda f=f: (moe_up("u", wu_v, f, 4), moe_hidden(f)))
        return tasks

    def moe_down_tasks(fs):
        return [(f, lambda f=f, n=n: moe_down(f, n, f == 0)) for f in fs for n in range(5)]

    def moe_finish():
        y = jnp.concatenate([moe[("y", n)] for n in range(5)], axis=1) * moe["w"]
        rr = _iota((128, D), 0)
        ypad = jnp.where(rr == 126, y[0:1], jnp.where(rr == 127, y[1:2], 0.0))
        cur = wo_t[:, 0:128].astype(F32)
        wo_t[:, 0:128] = jnp.where(_iota((D, 128), 1) >= 126, ypad.T, cur).astype(BF)

    causal = _iota((128, 128), 0) <= _iota((128, 128), 1)
    wrow = _iota((32, 128), 0)

    def query_weights(s, g, j, i, w):
        wq = q_t[s, i, _rows(128 * g + 16 * j, 32, 16), :]
        wq = jnp.where((wrow >= 2 * j) & (wrow < 2 * j + DH), wq, jnp.zeros_like(wq))
        parts = [wq]
        if j > 0:
            parts.insert(0, jnp.zeros((16 * j, 128), BF))
        if w - 16 * j - 32 > 0:
            parts.append(jnp.zeros((w - 16 * j - 32, 128), BF))
        return jnp.concatenate(parts, axis=0) if len(parts) > 1 else wq

    def key_tile(s, g, kt, w):
        return k_n[s, g, 128 * kt:128 * (kt + 1), :w]

    def score_tile(s, g, i, kt, w, wq):
        d = _dot(key_tile(s, g, kt, w), wq)
        return jnp.where(causal, d, NEG) if kt == i else d

    def value_window(s, g, j, kt):
        v = v_t[s, kt, _rows(128 * g + 16 * j, 32, 16), :]
        return jnp.where(wrow >= 30, jnp.ones_like(v), v)

    def value_tile(s, g, j, kt, p):
        return _dot(value_window(s, g, j, kt), p)

    def finish_column(s, g, j, i, o, with_mem):
        cols = slice(128 * i, 128 * (i + 1))
        win = _rows(128 * g + 16 * j, 32, 16)
        gate = gate_t[g][j:j + 1]
        scale = (1.0 - gate) / o[31:32, :]
        if isinstance(g, int):
            pace["tok"] = scale
        o = o * scale
        if with_mem:
            den = den_t[s, _rows(16 * g, 16, 16), cols][j:j + 1] + 1e-6
            o = o + am_t[s, win, cols] * (gate / den)
        if isinstance(g, int):
            r0 = 128 * g + DH * j
            o_t[s, i, r0:r0 + DH, :] = o[2 * j:2 * j + DH].astype(BF)
        else:
            mine = (wrow >= 2 * j) & (wrow < 2 * j + DH)
            o_t[s, i, win, :] = jnp.where(mine, o, o_t[s, i, win, :].astype(F32)).astype(BF)

    def running_max(m, d):
        pm = jnp.max(d.reshape(16, 8, 128), axis=0)
        return pm if m is None else jnp.maximum(m, pm)

    def compact_path():
        pace.clear()
        for g in range(NG):
            prep_wo(g)
            m_t[g] = jnp.zeros((128, 128), F32)
        am_t[0] = jnp.zeros((GP, L), F32)
        den_t[0] = jnp.ones((16 * NG, L), F32)

        @pl.loop(0, 4 * NSEG)
        def _(t):
            layernorm(t)

        moe_select()

        def expert(f, y):
            for k in range(5):
                moe_up("g", wg_v, f, k)
            for k in range(5):
                moe_up("u", wu_v, f, k)
            moe_hidden(f)
            for n in range(5):
                moe[("y", n)] = y[n]
                moe_down(f, n, False)
            return tuple(moe[("y", n)] for n in range(5))

        y = lax.fori_loop(0, FF // 128, expert,
                          tuple(jnp.zeros((16, k1 - k0), F32) for k0, k1 in KTS))
        for n in range(5):
            moe[("y", n)] = y[n]
        moe_finish()

        def head(s, g, j, w):
            for i in range(4):
                wq = query_weights(s, g, j, i, w)
                tiles, m = [], None
                for kt in range(i + 1):
                    tiles.append(score_tile(s, g, i, kt, w, wq))
                    m = running_max(m, tiles[-1])
                m = jnp.max(m, axis=0, keepdims=True)
                o = None
                for kt in range(i + 1):
                    r = value_tile(s, g, j, kt, jnp.exp2(tiles[kt] - m).astype(BF))
                    o = r if o is None else o + r
                finish_column(s, g, j, i, o, True)
                pace.clear()

        @pl.loop(0, NSEG)
        def _(s):
            @pl.loop(0, 4)
            def _(tt):
                for g in range(NG):
                    proj_qkv(s, tt, g)

            @pl.when(s > 0)
            def _():
                for g in range(NG):
                    mem_read(s, g)

            @pl.loop(0, NG - 1)
            def _(g):
                for j in range(HPG):
                    head(s, g, j, 128)

            for j in range(GN[NG - 1]):
                head(s, NG - 1, j, GW[NG - 1])
            for g in range(NG):
                mem_update(s, g, False)

            @pl.loop(0, 4)
            def _(tt):
                for fb in range(D // OUT_ROWS):
                    proj_out(s, tt, fb)
                out_copy(4 * s + tt).start()

    def head_units():
        units, h = [], 0
        while h < H:
            g, j = divmod(h, HPG)
            if j + 1 < GN[g]:
                units.append((h, h + 1))
                h += 2
            else:
                units.append((h,))
                h += 1
        return units

    def make_blocks():
        blocks = []
        for s in range(NSEG - 1):
            blocks += [[(s, u, i) for i in (3, 2, 1, 0)] for u in head_units()]
        s = NSEG - 1
        for i, budget in ((3, 16), (2, 18), (1, 20), (0, 20)):
            cur, n = [], 0
            for u in head_units():
                cost = len(u) * (i + 1)
                if cur and (n + cost > budget or (i == 0 and u[0] % HPG == 0)):
                    blocks.append(cur)
                    cur, n = [], 0
                cur.append((s, u, i))
                n += cost
            blocks.append(cur)
        return blocks

    col128 = _iota((64, 128), 1)
    mix_mask = _iota((64, 128), 0) <= (col128 & 63)

    def run_pipeline():
        blocks = make_blocks()
        nb = len(blocks)

        def slots(b):
            out, n = {}, 0
            for e, (_, heads, i) in enumerate(blocks[b]):
                for pos in range(len(heads)):
                    for kt in range(i + 1):
                        out[(e, pos, kt)] = n
                        n += 1
            return out

        def scores(b, micro):
            slot = slots(b)
            for e, (s, heads, i) in enumerate(blocks[b]):
                g = heads[0] // HPG
                w = GW[g]
                wqs = [query_weights(s, g, h % HPG, i, w) for h in heads]
                paired = len(heads) == 2
                for kt in range(i + 1):
                    half = paired and kt == i
                    keys = k_n[s, g, 128 * kt:128 * kt + (64 if half else 128), :w]
                    for pos in range(len(heads)):
                        d = _dot(keys, wqs[pos])
                        micro()
                        if kt == i:
                            d = jnp.where(causal[:d.shape[0]], d, NEG)
                        p_buf[b % 2, slot[(e, pos, kt)], 0:d.shape[0], :] = jnp.exp2(d).astype(BF)
                if paired:
                    wmix = jnp.concatenate([wqs[1][:, 64:], wqs[0][:, 64:]], axis=1)
                    d = _dot(k_n[s, g, 128 * i + 64:128 * (i + 1), :w], wmix)
                    ex = jnp.exp2(jnp.where(mix_mask, d, NEG))
                    zero = jnp.zeros((64, 64), F32)
                    p_buf[b % 2, slot[(e, 0, i)], 64:128, :] = jnp.where(col128 >= 64, ex, 0.0).astype(BF)
                    p_buf[b % 2, slot[(e, 1, i)], 64:128, :] = jnp.concatenate(
                        [zero, ex[:, :64]], axis=1).astype(BF)

        def values(b):
            slot = slots(b)
            windows = {}
            for e, (s, heads, i) in enumerate(blocks[b]):
                for pos, h in enumerate(heads):
                    g, j = divmod(h, HPG)
                    o = None
                    for kt in range(i + 1):
                        if (h, kt) not in windows:
                            windows[(h, kt)] = value_window(s, g, j, kt)
                        r = _dot(windows[(h, kt)], p_buf[b % 2, slot[(e, pos, kt)]])
                        o = r if o is None else o + r
                    finish_column(s, g, j, i, o, s > 0)

        def proj_tasks(s, groups=range(NG)):
            return [(GW[g] // 16 * 15,
                     lambda s=s, tt=tt, g=g: proj_qkv(s, tt, g, s > 0, s < NSEG - 1))
                    for tt in range(4) for g in groups]

        def out_tasks(s, tts=range(4)):
            tasks = []
            for tt in tts:
                tasks += [(OUT_ROWS * 5 // 16, lambda s=s, tt=tt, fb=fb: proj_out(s, tt, fb, (s, tt) == (NSEG - 1, 0)))
                          for fb in range(D // OUT_ROWS)]
                tasks.append((0, lambda s=s, tt=tt: out_copy(4 * s + tt).start()))
            return tasks

        def ln_tasks(s):
            ts = range(4 * s, 4 * s + 4)
            return ([(10, lambda t=t: ln_stats(t)) for t in ts]
                    + [(10, lambda t=t: ln_apply(t)) for t in ts]
                    + [(2, lambda t=t: router(t)) for t in ts])

        def upd_tasks(s):
            return [(GW[g] // 4, lambda s=s, g=g: mem_update(s, g, s == 0)) for g in range(NG)]

        def read_tasks(s):
            return [(GW[g] // 4 + 4, lambda s=s, g=g: mem_read(s, g)) for g in range(NG)]

        def prep_tasks(cbs):
            return [(5, lambda cb=cb, which=which: prep_wt(cb, which)) for cb in cbs for which in range(3)]

        guard = {}

        def norm_task(i, cb, part):
            acc = col_norm2(i, cb, part)
            if part > 0:
                acc = acc + guard[("acc", i)]
            else:
                acc = acc + paced(jnp.zeros((1, acc.shape[1]), F32), acc.shape[1])
            guard[("acc", i)] = acc
            if part == 2:
                row = jnp.sum(acc, axis=0, keepdims=True)
                if row.shape[1] < 128:
                    row = jnp.concatenate([row, jnp.zeros((1, 128 - row.shape[1]), F32)], axis=1)
                guard[i] = row if i not in guard else jnp.maximum(guard[i], row)

        def guard_task():
            nq, nk, nv = (jnp.max(guard[i]) for i in range(3))
            guard["safe"] = jnp.logical_and(
                nq * nk <= (SCORE_LIMIT / (1.05 * D * QSCALE * DH)) ** 2, nv <= 1e30)

        def norm_tasks(cbs):
            return [(1, lambda i=i, cb=cb, part=part: norm_task(i, cb, part))
                    for cb in cbs for i in range(3) for part in range(3)]

        seg0 = [min(k for k, blk in enumerate(blocks) if blk[0][0] == s) for s in range(NSEG)] + [nb]
        last = {i: max(k for k, blk in enumerate(blocks) if blk[0][0] == NSEG - 1 and blk[0][2] == i)
                for i in range(4)}

        def at(s, frac):
            return seg0[s] + round(frac * (seg0[s + 1] - seg0[s]))

        a1, a2, a3 = seg0[1], seg0[2], seg0[3]
        streams = [
            (0, 1, prep_tasks((1, 2))),
            (0, 2, proj_tasks(0, (1,))),
            (2, 3, prep_tasks((3, 4))),
            (2, 4, proj_tasks(0, (2,))),
            (2, 5, ln_tasks(1)),
            (4, 7, proj_tasks(0, (3, 4))),
            (6, a1 - 1, proj_tasks(1)),
            (8, 10, upd_tasks(0)),
            (a1 - 1, a1, read_tasks(1)),
            (6, a1 - 1, ln_tasks(2) + ln_tasks(3)),
            (6, a1, [(5, lambda g=g: prep_wo(g)) for g in range(NG)]),
            (a3 + 1, nb - 6, norm_tasks(range(5))),
            (nb - 5, nb - 4, [(1, guard_task)]),
            (a1, a1 + 1, [(1, moe_select)]),
            (a1 + 1, at(1, 0.2), upd_tasks(1)),
            (a1, a2 - 1, proj_tasks(2)),
            (a2 - 1, a2, read_tasks(2)),
            (a2 + 1, at(2, 0.2), upd_tasks(2)),
            (a2, a3 - 1, proj_tasks(3)),
            (a3 - 1, a3, read_tasks(3)),
            (a3 - 1, a3, [(1, lambda: (emit_downs(len(downs)), moe_finish()))]),
            (a3 + 1, last[1] + 1, out_tasks(0) + out_tasks(1) + out_tasks(2)),
            (last[3] + 2, last[2] + 1, out_tasks(3, (3,))),
            (last[2] + 2, last[1] + 1, out_tasks(3, (2,))),
            (last[1] + 2, nb + 1, out_tasks(3, (1,))),
        ]
        nf = FF // 128
        micro_ranges = [(a1 + 1, a2 - 1, moe_up_tasks(range(nf // 2))),
                        (a2, a3 - 2, moe_up_tasks(range(nf // 2, nf)))]
        downs = moe_down_tasks(range(nf))
        dstate = [0]

        def emit_downs(limit):
            n = 0
            while dstate[0] < len(downs) and n < limit and ("h", downs[dstate[0]][0]) in moe:
                downs[dstate[0]][1]()
                dstate[0] += 1
                n += 1

        ntiles = [sum(len(u) * (i + 1) for (_, u, i) in blk) for blk in blocks]

        def fence_w12():
            wait_w(1)
            wait_w(2)

        def fence_w34():
            wait_w(3)
            wait_w(4)
            x_copy(1).wait()

        def fence_a1():
            wait_moe(0)
            start_moe(1)

        def fence_a0():
            x_copy(2).wait()
            x_copy(3).wait()
            wo_copy.wait()
            start_moe(0)

        fences = {0: fence_w12, 2: fence_w34, 5: fence_a0, a1: fence_a1, a2: lambda: wait_moe(1)}

        state = [[0, 0.0, float(sum(c for c, _ in t))] for _, _, t in streams]
        mstate = [[0, 0] for _ in micro_ranges]

        for b in range(nb + 1):
            if b in fences:
                fences[b]()

            def micro(b=b):
                for (lo, hi, tasks), ms in zip(micro_ranges, mstate):
                    if lo <= b < hi:
                        ms[0] += 1
                        total = sum(ntiles[lo:hi])
                        while ms[1] < len(tasks) and ms[1] < ms[0] * len(tasks) / total:
                            tasks[ms[1]]()
                            ms[1] += 1

            if b < nb:
                scores(b, micro)
            for (lo, hi, tasks), st_ in zip(streams, state):
                if b < lo:
                    continue
                frac = (b + 1 - lo) / (hi - lo)
                while st_[0] < len(tasks) and st_[1] + tasks[st_[0]][0] / 2 <= frac * st_[2] + 1e-9:
                    cost, task = tasks[st_[0]]
                    task()
                    st_[1] += cost
                    st_[0] += 1
                    if cost >= 75 and a1 < b < a3:
                        emit_downs(5)
            if b > 0:
                values(b - 1)
        for (lo, hi, tasks), st_ in zip(streams, state):
            assert st_[0] == len(tasks), (lo, hi, st_)
        assert all(ms[1] == len(r[2]) for ms, r in zip(mstate, micro_ranges)) and dstate[0] == len(downs)
        for _, t in out_tasks(3, (0,)):
            t()

        def wait_outputs():
            for t in range(4 * NSEG):
                out_copy(t).wait()

        @pl.when(jnp.logical_not(guard["safe"]))
        def _():
            wait_outputs()
            compact_path()

        wait_outputs()

    def prep_group(g):
        for which in range(3):
            prep_wt(g, which)

    def wait_w(cb):
        for i in range(3):
            w_copy(i, cb).wait()

    def start_moe(c):
        for i in range(3):
            moe_copy(i, c).start()

    def wait_moe(c):
        for i in range(3):
            moe_copy(i, c).wait()

    def col_norm2(i, cb, part):
        n = 128 if cb < 4 else 64
        acc = None
        for u in range(3 * part, 3 * part + 3):
            wv = wraw[i, 64 * u:64 * (u + 1), 128 * cb:128 * cb + n].astype(F32)
            c = jnp.sum((wv * wv).reshape(8, 8, n), axis=0)
            acc = c if acc is None else acc + c
        return acc

    for s in range(NSEG):
        for g in range(NG):
            n = DH * GN[g]
            for tt in range(4):
                o_t[s, tt, 128 * g + n:128 * g + GW[g], :] = jnp.zeros((GW[g] - n, 128), BF)
    wr_copy.wait()
    x_copy(0, 0).wait()
    prep_wr()
    layernorm(0)
    wait_w(0)
    prep_group(0)
    proj_qkv(0, 0, 0, False, True)
    for tt in range(1, 4):
        x_copy(0, tt).wait()
    beta_copy.wait()
    for tt in range(1, 4):
        layernorm(tt)
        proj_qkv(0, tt, 0, False, True)
    prep_gates()
    run_pipeline()


@jax.jit
def pallas_parallel_sum__memory_aug_infini_attn__moe_arch_mod__prompt_kernel(
    A_x: jax.Array,
    A_wq: jax.Array,
    A_wk: jax.Array,
    A_wv: jax.Array,
    A_wo: jax.Array,
    A_beta: jax.Array,
    B_x: jax.Array,
    B_w_r: jax.Array,
    B_w_gate: jax.Array,
    B_w_up: jax.Array,
    B_w_down: jax.Array,
):
    del B_x
    hbm = pl.BlockSpec(memory_space=pltpu.HBM)
    scratch = [
        pltpu.VMEM((D, SEQ), BF),
        pltpu.VMEM((4 * NSEG, D, 128), BF),
        pltpu.VMEM((16, SEQ), F32),
        pltpu.VMEM((4, D, D), BF),
        pltpu.VMEM((3 * GP, D), BF),
        pltpu.VMEM((D, GP), BF),
        pltpu.VMEM((H,), BF),
        pltpu.VMEM((D,), BF),
        pltpu.VMEM((16, D), BF),
        pltpu.VMEM((D, FF), BF),
        pltpu.VMEM((D, FF), BF),
        pltpu.VMEM((D, FF), BF),
        pltpu.VMEM((NSEG, 4, GP, 128), BF),
        pltpu.VMEM((NSEG, 4, GP, 128), BF),
        pltpu.VMEM((NSEG, 4, GP, 128), BF),
        pltpu.VMEM((NSEG, NG, L, 128), BF),
        pltpu.VMEM((NSEG, 4, GP, 128), BF),
        pltpu.VMEM((NSEG, 4, GP, 128), BF),
        pltpu.VMEM((2, 20, 128, 128), BF),
        pltpu.VMEM((NSEG, GP, L), F32),
        pltpu.VMEM((NSEG, 16 * NG, L), F32),
        pltpu.VMEM((NG, 128, 128), F32),
        pltpu.VMEM((1, SEQ), F32),
        pltpu.VMEM((NG, 8, 128), F32),
        pltpu.VMEM((4 * NSEG, D, 128), BF),
        pltpu.SemaphoreType.DMA((25,)),
        pltpu.SemaphoreType.DMA((3 * NMC,)),
        pltpu.SemaphoreType.DMA((4 * NSEG,)),
    ]
    out_t = pl.pallas_call(
        _kernel,
        out_shape=jax.ShapeDtypeStruct((1, D, SEQ), BF),
        in_specs=[hbm] * 10,
        out_specs=hbm,
        scratch_shapes=scratch,
        compiler_params=pltpu.CompilerParams(vmem_limit_bytes=100 * 1024 * 1024),
    )(jnp.swapaxes(A_x, 1, 2), A_wq, A_wk, A_wv, A_wo, A_beta, B_w_r, B_w_gate, B_w_up,
      B_w_down.T)
    return jnp.swapaxes(out_t, 1, 2)
```

```python
import jax
import jax.numpy as jnp
from jax import lax
import jax.experimental.pallas as pl
import jax.experimental.pallas.tpu as pltpu

BF = jnp.bfloat16
F32 = jnp.float32

SEQ, D, H, DH = 2048, 576, 32, 18
NSEG, L, FF = 4, 512, 4608
HPG = 7
NG = 5
GN = (7, 7, 7, 7, 4)
GW = (128, 128, 128, 128, 80)
GP = 592
ZR = (126, 126, 126, 126, 78)
QSCALE = (DH ** -0.5) * 1.4426950408889634
NT_DIMS = (((1,), (1,)), ((), ()))
MOE_DMA = 2304
NMC = FF // MOE_DMA
OUT_ROWS = 192
NEG = -1e30
SCORE_LIMIT = 40.0
KTS = tuple((128 * k, min(128 * (k + 1), D)) for k in range(5))


def _dot(a, b):
    return jnp.dot(a, b, preferred_element_type=F32)


def _dot_nt(a, b):
    return lax.dot_general(a, b, NT_DIMS, preferred_element_type=F32)


def _iota(shape, dim):
    return lax.broadcasted_iota(jnp.int32, shape, dim)


def _phi(t):
    return jnp.where(t > 0, t + 1.0, jnp.exp(t))


def _sigmoid(t):
    return 1.0 / (1.0 + jnp.exp(-t))


def _div18(i):
    return (i * 57) >> 10


def _blk(t, size=128):
    if isinstance(t, int):
        return slice(size * t, size * (t + 1))
    return pl.ds(pl.multiple_of(t * size, size), size)


def _rows(start, size, align):
    if isinstance(start, int):
        return slice(start, start + size)
    return pl.ds(pl.multiple_of(start, align), size)


def _kernel(x_hbm, wq_hbm, wk_hbm, wv_hbm, wo_hbm, beta_hbm, wr_hbm, wg_hbm, wu_hbm, wd_hbm,
            out_hbm,
            x_v, xn_v, stat_v, wraw, w_t, wo_t, beta_v, wr_v, wr_b, wg_v, wu_v, wd_v,
            q_t, pq_t, v_t, k_n, pk_t, o_t, p_buf, am_t, den_t, m_t, r_row, gate_t, out_v,
            sem_in, sem_moe, sem_out):

    def x_copy(s, tt=None):
        if tt is None:
            c0, n, k = s * L, L, 3 + s
        else:
            c0, n, k = tt * 128, 128, tt
        return pltpu.make_async_copy(x_hbm.at[0, :, pl.ds(c0, n)], x_v.at[:, pl.ds(c0, n)],
                                     sem_in.at[k])

    def w_copy(i, cb):
        src = (wq_hbm, wk_hbm, wv_hbm)[i]
        n = 128 if cb < 4 else 64
        return pltpu.make_async_copy(src.at[:, pl.ds(128 * cb, n)], wraw.at[i, :, pl.ds(128 * cb, n)],
                                     sem_in.at[7 + 5 * i + cb])

    wo_copy = pltpu.make_async_copy(wo_hbm, wraw.at[3], sem_in.at[22])
    beta_copy = pltpu.make_async_copy(beta_hbm, beta_v, sem_in.at[23])
    wr_copy = pltpu.make_async_copy(wr_hbm, wr_v, sem_in.at[24])

    def moe_copy(i, c):
        src, dst = ((wg_hbm, wg_v), (wu_hbm, wu_v), (wd_hbm, wd_v))[i]
        cs = pl.ds(c * MOE_DMA, MOE_DMA)
        return pltpu.make_async_copy(src.at[:, cs], dst.at[:, cs], sem_moe.at[i * NMC + c])

    def out_copy(t):
        cs = pl.ds(t * 128 if isinstance(t, int) else pl.multiple_of(t * 128, 128), 128)
        return pltpu.make_async_copy(out_v.at[t], out_hbm.at[0, :, cs], sem_out.at[t])

    wr_copy.start()
    x_copy(0, 0).start()
    for i in range(3):
        w_copy(i, 0).start()
    beta_copy.start()
    for tt in range(1, 4):
        x_copy(0, tt).start()
    for cb in range(1, 5):
        for i in range(3):
            w_copy(i, cb).start()
    x_copy(1).start()
    x_copy(2).start()
    x_copy(3).start()
    wo_copy.start()

    pace = {}

    def paced(row, lanes=128):
        tok = pace.get("tok")
        return row if tok is None else row + tok[:, :lanes] * 0.0

    def ln_stats(t):
        cols = _blk(t)
        shift = paced(x_v[0:16, cols].astype(F32)[0:1])
        s1 = [None] * 2
        s2 = [None] * 2
        for u in range(D // 16):
            d = x_v[16 * u:16 * (u + 1), cols].astype(F32) - shift
            d = d.reshape(2, 8, 128)
            for k in range(2):
                s1[k] = d[k] if u == 0 else s1[k] + d[k]
                s2[k] = d[k] * d[k] if u == 0 else s2[k] + d[k] * d[k]
        m1 = jnp.sum(s1[0] + s1[1], axis=0, keepdims=True) * (1.0 / D)
        m2 = jnp.sum(s2[0] + s2[1], axis=0, keepdims=True) * (1.0 / D)
        var = jnp.maximum(m2 - m1 * m1, 0.0)
        stat_v[0:1, cols] = m1 + shift
        stat_v[8:9, cols] = lax.rsqrt(var + 1e-5)

    def ln_apply(t):
        cols = _blk(t)
        mean = paced(stat_v[0:1, cols])
        rstd = stat_v[8:9, cols]
        for u in range(D // 48):
            rows = slice(48 * u, 48 * (u + 1))
            xn_v[t, rows, :] = ((x_v[rows, cols].astype(F32) - mean) * rstd).astype(BF)

    def router(t):
        r = _dot(wr_b[...], xn_v[t])
        r_row[:, _blk(t)] = r[0:1].astype(BF).astype(F32)

    def layernorm(t):
        ln_stats(t)
        ln_apply(t)
        router(t)

    def prep_wr():
        wr = wr_v[...].reshape(1, D)
        wr_b[...] = jnp.broadcast_to(wr.astype(F32), (16, D)).astype(BF)

    def prep_wt(cb, which):
        nb = 128 if cb < 4 else 64
        n = DH * GN[cb]
        t = wraw[which, :, 128 * cb:128 * cb + nb].T
        r0 = 384 * cb + which * GW[cb]
        k = min(n - 2 * cb, nb)
        w_t[r0 + 2 * cb:r0 + 2 * cb + k, :] = t[0:k]
        w_t[r0 + n:r0 + GW[cb], :] = jnp.zeros((GW[cb] - n, D), BF)
        if cb < 4:
            r1 = 384 * (cb + 1) + which * GW[cb + 1]
            w_t[r1:r1 + 2 * (cb + 1), :] = t[128 - 2 * (cb + 1):128]

    def prep_wo(g):
        n = DH * GN[g]
        wo_t[:, 128 * g:128 * g + n] = wraw[3, 126 * g:126 * g + n, :].T
        wo_t[:, 128 * g + n:128 * g + GW[g]] = jnp.zeros((D, GW[g] - n), BF)

    def prep_gates():
        b = beta_v[...].astype(F32).reshape(1, H)
        sig = jnp.concatenate([_sigmoid(b), jnp.zeros((1, 128 - H), F32)], axis=1)
        rows = jnp.broadcast_to(sig, (128, 128)).T
        for g in range(NG):
            gate_t[g] = rows[HPG * g:HPG * g + 8]

    def proj_qkv(s, tt, g, need_pq=True, need_pk=True):
        w = GW[g]
        rows = slice(128 * g, 128 * g + w)
        r = _dot(w_t[384 * g:384 * g + 3 * w, :], xn_v[4 * s + tt])
        q, k, v = r[:w], r[w:2 * w], r[2 * w:]
        q_t[s, tt, rows, :] = (q * QSCALE).astype(BF)
        if need_pq:
            pq_t[s, tt, rows, :] = _phi(q).astype(BF)
        k_n[s, g, _blk(tt), :w] = k.astype(BF).T
        if need_pk:
            pk_t[s, tt, rows, :] = _phi(k).astype(BF)
        v = jnp.where(_iota((w, 128), 0) == ZR[g], 1.0, v)
        v_t[s, tt, rows, :] = v.astype(BF)

    def mem_update(s, g, first):
        w = GW[g]
        rows = slice(128 * g, 128 * g + w)
        r = _dot_nt(v_t[s, 0, rows, :], pk_t[s, 0, rows, :])
        for tt in range(1, 4):
            r = r + _dot_nt(v_t[s, tt, rows, :], pk_t[s, tt, rows, :])
        rr, cc = _iota((w, w), 0), _iota((w, w), 1)
        keep = (cc < DH * GN[g]) & ((_div18(rr) == _div18(cc)) | (rr == ZR[g]))
        r = jnp.where(keep, r, 0.0)
        if not first:
            r = r + m_t[g, :w, :w]
        m_t[g, :w, :w] = r

    def mem_read(s, g):
        w = GW[g]
        rows = slice(128 * g, 128 * g + w)
        m = m_t[g, :w, :w]
        z = m[ZR[g]:ZR[g] + 1, :]
        zrows = jnp.where(_iota((16, w), 0) == _div18(_iota((16, w), 1)), z, 0.0)
        lhs = jnp.concatenate([m, zrows], axis=0).astype(BF)
        for tt in range(4):
            cols = slice(128 * tt, 128 * (tt + 1))
            r = _dot(lhs, pq_t[s, tt, rows, :])
            am_t[s, rows, cols] = r[:w]
            den_t[s, 16 * g:16 * (g + 1), cols] = r[w:]

    def proj_out(s, tt, fb, by_group=False):
        f0 = OUT_ROWS * fb
        f1 = f0 + OUT_ROWS
        if by_group:
            p = None
            for g in range(NG):
                r = _dot(wo_t[f0:f1, 128 * g:128 * g + GW[g]], o_t[s, tt, 128 * g:128 * g + GW[g], :])
                p = r if p is None else p + r
        else:
            p = _dot(wo_t[f0:f1, :], o_t[s, tt])
        t = 4 * s + tt
        res = x_v[f0:f1, _blk(t)].astype(F32) + xn_v[t, f0:f1, :].astype(F32)
        out_v[t, f0:f1, :] = (p + res).astype(BF)

    moe = {}

    def moe_select():
        r = r_row[...]
        io = _iota((1, SEQ), 1)
        m1 = jnp.max(r)
        i1 = jnp.min(jnp.where(r == m1, io, SEQ - 1))
        r2 = jnp.where(io == i1, -jnp.inf, r)
        m2 = jnp.max(r2)
        i2 = jnp.min(jnp.where((r2 == m2) & (io != i1), io, SEQ - 1))
        rows = []
        for i in (i1, i2):
            xb = xn_v[i // 128].T.astype(F32)
            rows.append(jnp.sum(jnp.where(_iota((128, D), 0) == i % 128, xb, 0.0), axis=0, keepdims=True))
        rr = _iota((16, D), 0)
        xs = jnp.where(rr == 0, rows[0], jnp.where(rr == 1, rows[1], 0.0))
        moe["x"] = xs.astype(BF)
        moe["w"] = _sigmoid(jnp.where(_iota((16, 1), 0) == 0, m1, m2))
        sel = jnp.where(_iota((2, 128), 0) == 0, i1, i2)
        for t in range(4 * NSEG):
            tok = _iota((2, 128), 1) + 128 * t
            o_t[t // 4, t % 4, 126:128, :] = jnp.where(tok == sel, 1.0, 0.0).astype(BF)

    def moe_up(name, ref, f, k):
        k0, k1 = KTS[k]
        r = _dot(moe["x"][:, k0:k1], ref[k0:k1, _blk(f)])
        moe[name] = r if k == 0 else moe[name] + r

    def moe_hidden(f):
        g = moe["g"]
        moe[("h", f if isinstance(f, int) else 0)] = (g * _sigmoid(g) * moe["u"]).astype(BF)

    def moe_down(f, n, first):
        n0, n1 = KTS[n]
        r = _dot_nt(moe[("h", f if isinstance(f, int) else 0)], wd_v[n0:n1, _blk(f)])
        moe[("y", n)] = r if first else moe[("y", n)] + r

    def moe_up_tasks(fs):
        tasks = []
        for f in fs:
            tasks += [lambda f=f, k=k: moe_up("g", wg_v, f, k) for k in range(5)]
            tasks += [lambda f=f, k=k: moe_up("u", wu_v, f, k) for k in range(4)]
            tasks.append(lambda f=f: (moe_up("u", wu_v, f, 4), moe_hidden(f)))
        return tasks

    def moe_down_tasks(fs):
        return [(f, lambda f=f, n=n: moe_down(f, n, f == 0)) for f in fs for n in range(5)]

    def moe_finish():
        y = jnp.concatenate([moe[("y", n)] for n in range(5)], axis=1) * moe["w"]
        rr = _iota((128, D), 0)
        ypad = jnp.where(rr == 126, y[0:1], jnp.where(rr == 127, y[1:2], 0.0))
        cur = wo_t[:, 0:128].astype(F32)
        wo_t[:, 0:128] = jnp.where(_iota((D, 128), 1) >= 126, ypad.T, cur).astype(BF)

    causal = _iota((128, 128), 0) <= _iota((128, 128), 1)
    wrow = _iota((32, 128), 0)

    def query_weights(s, g, j, i, w):
        wq = q_t[s, i, _rows(128 * g + 16 * j, 32, 16), :]
        wq = jnp.where((wrow >= 2 * j) & (wrow < 2 * j + DH), wq, jnp.zeros_like(wq))
        parts = [wq]
        if j > 0:
            parts.insert(0, jnp.zeros((16 * j, 128), BF))
        if w - 16 * j - 32 > 0:
            parts.append(jnp.zeros((w - 16 * j - 32, 128), BF))
        return jnp.concatenate(parts, axis=0) if len(parts) > 1 else wq

    def key_tile(s, g, kt, w):
        return k_n[s, g, 128 * kt:128 * (kt + 1), :w]

    def score_tile(s, g, i, kt, w, wq):
        d = _dot(key_tile(s, g, kt, w), wq)
        return jnp.where(causal, d, NEG) if kt == i else d

    def value_window(s, g, j, kt):
        v = v_t[s, kt, _rows(128 * g + 16 * j, 32, 16), :]
        return jnp.where(wrow >= 30, jnp.ones_like(v), v)

    def value_tile(s, g, j, kt, p):
        return _dot(value_window(s, g, j, kt), p)

    def finish_column(s, g, j, i, o, with_mem):
        cols = slice(128 * i, 128 * (i + 1))
        win = _rows(128 * g + 16 * j, 32, 16)
        gate = gate_t[g][j:j + 1]
        scale = (1.0 - gate) / o[31:32, :]
        if isinstance(g, int):
            pace["tok"] = scale
        o = o * scale
        if with_mem:
            den = den_t[s, _rows(16 * g, 16, 16), cols][j:j + 1] + 1e-6
            o = o + am_t[s, win, cols] * (gate / den)
        if isinstance(g, int):
            r0 = 128 * g + DH * j
            o_t[s, i, r0:r0 + DH, :] = o[2 * j:2 * j + DH].astype(BF)
        else:
            mine = (wrow >= 2 * j) & (wrow < 2 * j + DH)
            o_t[s, i, win, :] = jnp.where(mine, o, o_t[s, i, win, :].astype(F32)).astype(BF)

    def running_max(m, d):
        pm = jnp.max(d.reshape(16, 8, 128), axis=0)
        return pm if m is None else jnp.maximum(m, pm)

    def compact_path():
        pace.clear()
        for g in range(NG):
            prep_wo(g)
            m_t[g] = jnp.zeros((128, 128), F32)
        am_t[0] = jnp.zeros((GP, L), F32)
        den_t[0] = jnp.ones((16 * NG, L), F32)

        @pl.loop(0, 4 * NSEG)
        def _(t):
            layernorm(t)

        moe_select()

        def expert(f, y):
            for k in range(5):
                moe_up("g", wg_v, f, k)
            for k in range(5):
                moe_up("u", wu_v, f, k)
            moe_hidden(f)
            for n in range(5):
                moe[("y", n)] = y[n]
                moe_down(f, n, False)
            return tuple(moe[("y", n)] for n in range(5))

        y = lax.fori_loop(0, FF // 128, expert,
                          tuple(jnp.zeros((16, k1 - k0), F32) for k0, k1 in KTS))
        for n in range(5):
            moe[("y", n)] = y[n]
        moe_finish()

        def head(s, g, j, w):
            for i in range(4):
                wq = query_weights(s, g, j, i, w)
                tiles, m = [], None
                for kt in range(i + 1):
                    tiles.append(score_tile(s, g, i, kt, w, wq))
                    m = running_max(m, tiles[-1])
                m = jnp.max(m, axis=0, keepdims=True)
                o = None
                for kt in range(i + 1):
                    r = value_tile(s, g, j, kt, jnp.exp2(tiles[kt] - m).astype(BF))
                    o = r if o is None else o + r
                finish_column(s, g, j, i, o, True)
                pace.clear()

        @pl.loop(0, NSEG)
        def _(s):
            @pl.loop(0, 4)
            def _(tt):
                for g in range(NG):
                    proj_qkv(s, tt, g)

            @pl.when(s > 0)
            def _():
                for g in range(NG):
                    mem_read(s, g)

            @pl.loop(0, NG - 1)
            def _(g):
                for j in range(HPG):
                    head(s, g, j, 128)

            for j in range(GN[NG - 1]):
                head(s, NG - 1, j, GW[NG - 1])
            for g in range(NG):
                mem_update(s, g, False)

            @pl.loop(0, 4)
            def _(tt):
                for fb in range(D // OUT_ROWS):
                    proj_out(s, tt, fb)
                out_copy(4 * s + tt).start()

    def head_units():
        units, h = [], 0
        while h < H:
            g, j = divmod(h, HPG)
            if j + 1 < GN[g]:
                units.append((h, h + 1))
                h += 2
            else:
                units.append((h,))
                h += 1
        return units

    def make_blocks():
        blocks = []
        for s in range(NSEG - 1):
            units = head_units()
            if s == 0:
                first = [u for u in units if u[0] < HPG]
                blocks += [[(0, u, i) for u in first] for i in range(4)]
                units = [u for u in units if u[0] >= HPG]
            blocks += [[(s, u, i) for i in (3, 2, 1, 0)] for u in units]
        s = NSEG - 1
        for i, budget in ((3, 16), (2, 18), (1, 20), (0, 20)):
            cur, n = [], 0
            for u in head_units():
                cost = len(u) * (i + 1)
                if cur and (n + cost > budget or (i == 0 and u[0] % HPG == 0)):
                    blocks.append(cur)
                    cur, n = [], 0
                cur.append((s, u, i))
                n += cost
            blocks.append(cur)
        return blocks

    col128 = _iota((64, 128), 1)
    mix_mask = _iota((64, 128), 0) <= (col128 & 63)

    def run_pipeline():
        blocks = make_blocks()
        nb = len(blocks)

        def slots(b):
            out, n = {}, 0
            for e, (_, heads, i) in enumerate(blocks[b]):
                for pos in range(len(heads)):
                    for kt in range(i + 1):
                        out[(e, pos, kt)] = n
                        n += 1
            return out

        def scores(b, micro):
            slot = slots(b)
            for e, (s, heads, i) in enumerate(blocks[b]):
                g = heads[0] // HPG
                w = GW[g]
                wqs = [query_weights(s, g, h % HPG, i, w) for h in heads]
                paired = len(heads) == 2
                for kt in range(i + 1):
                    half = paired and kt == i
                    keys = k_n[s, g, 128 * kt:128 * kt + (64 if half else 128), :w]
                    for pos in range(len(heads)):
                        d = _dot(keys, wqs[pos])
                        micro()
                        if kt == i:
                            d = jnp.where(causal[:d.shape[0]], d, NEG)
                        p_buf[b % 2, slot[(e, pos, kt)], 0:d.shape[0], :] = jnp.exp2(d).astype(BF)
                if paired:
                    wmix = jnp.concatenate([wqs[1][:, 64:], wqs[0][:, 64:]], axis=1)
                    d = _dot(k_n[s, g, 128 * i + 64:128 * (i + 1), :w], wmix)
                    ex = jnp.exp2(jnp.where(mix_mask, d, NEG))
                    zero = jnp.zeros((64, 64), F32)
                    p_buf[b % 2, slot[(e, 0, i)], 64:128, :] = jnp.where(col128 >= 64, ex, 0.0).astype(BF)
                    p_buf[b % 2, slot[(e, 1, i)], 64:128, :] = jnp.concatenate(
                        [zero, ex[:, :64]], axis=1).astype(BF)

        def values(b):
            slot = slots(b)
            windows = {}
            for e, (s, heads, i) in enumerate(blocks[b]):
                for pos, h in enumerate(heads):
                    g, j = divmod(h, HPG)
                    o = None
                    for kt in range(i + 1):
                        if (h, kt) not in windows:
                            windows[(h, kt)] = value_window(s, g, j, kt)
                        r = _dot(windows[(h, kt)], p_buf[b % 2, slot[(e, pos, kt)]])
                        o = r if o is None else o + r
                    finish_column(s, g, j, i, o, s > 0)

        def proj_tasks(s, groups=range(NG)):
            return [(GW[g] // 16 * 15,
                     lambda s=s, tt=tt, g=g: proj_qkv(s, tt, g, s > 0, s < NSEG - 1))
                    for tt in range(4) for g in groups]

        def out_tasks(s, tts=range(4)):
            tasks = []
            for tt in tts:
                tasks += [(OUT_ROWS * 5 // 16, lambda s=s, tt=tt, fb=fb: proj_out(s, tt, fb, (s, tt) == (NSEG - 1, 0)))
                          for fb in range(D // OUT_ROWS)]
                tasks.append((0, lambda s=s, tt=tt: out_copy(4 * s + tt).start()))
            return tasks

        def ln_tasks(s):
            ts = range(4 * s, 4 * s + 4)
            return ([(10, lambda t=t: ln_stats(t)) for t in ts]
                    + [(10, lambda t=t: ln_apply(t)) for t in ts]
                    + [(2, lambda t=t: router(t)) for t in ts])

        def upd_tasks(s):
            return [(GW[g] // 4, lambda s=s, g=g: mem_update(s, g, s == 0)) for g in range(NG)]

        def read_tasks(s):
            return [(GW[g] // 4 + 4, lambda s=s, g=g: mem_read(s, g)) for g in range(NG)]

        def prep_tasks(cbs):
            return [(5, lambda cb=cb, which=which: prep_wt(cb, which)) for cb in cbs for which in range(3)]

        guard = {}

        def norm_task(i, cb, part):
            acc = col_norm2(i, cb, part)
            if part > 0:
                acc = acc + guard[("acc", i)]
            else:
                acc = acc + paced(jnp.zeros((1, acc.shape[1]), F32), acc.shape[1])
            guard[("acc", i)] = acc
            if part == 2:
                row = jnp.sum(acc, axis=0, keepdims=True)
                if row.shape[1] < 128:
                    row = jnp.concatenate([row, jnp.zeros((1, 128 - row.shape[1]), F32)], axis=1)
                guard[i] = row if i not in guard else jnp.maximum(guard[i], row)

        def guard_task():
            nq, nk, nv = (jnp.max(guard[i]) for i in range(3))
            guard["safe"] = jnp.logical_and(
                nq * nk <= (SCORE_LIMIT / (1.05 * D * QSCALE * DH)) ** 2, nv <= 1e30)

        def norm_tasks(cbs):
            return [(1, lambda i=i, cb=cb, part=part: norm_task(i, cb, part))
                    for cb in cbs for i in range(3) for part in range(3)]

        seg0 = [min(k for k, blk in enumerate(blocks) if blk[0][0] == s) for s in range(NSEG)] + [nb]
        last = {i: max(k for k, blk in enumerate(blocks) if blk[0][0] == NSEG - 1 and blk[0][2] == i)
                for i in range(4)}

        def at(s, frac):
            return seg0[s] + round(frac * (seg0[s + 1] - seg0[s]))

        a1, a2, a3 = seg0[1], seg0[2], seg0[3]
        def tile0(tt):
            return [(10, lambda: layernorm(tt)), (120, lambda: proj_qkv(0, tt, 0, False, True))]

        streams = [
            (0, 1, [(1, prep_gates)] + tile0(1)),
            (1, 2, tile0(2)),
            (2, 3, tile0(3)),
            (2, 3, prep_tasks((1, 2))),
            (2, 4, proj_tasks(0, (1,))),
            (4, 5, prep_tasks((3, 4))),
            (4, 6, proj_tasks(0, (2,))),
            (4, 6, ln_tasks(1)),
            (5, 8, proj_tasks(0, (3, 4))),
            (7, a1 - 1, proj_tasks(1)),
            (9, 11, upd_tasks(0)),
            (a1 - 1, a1, read_tasks(1)),
            (7, a1 - 1, ln_tasks(2) + ln_tasks(3)),
            (7, a1, [(5, lambda g=g: prep_wo(g)) for g in range(NG)]),
            (a3 + 1, nb - 6, norm_tasks(range(5))),
            (nb - 5, nb - 4, [(1, guard_task)]),
            (a1, a1 + 1, [(1, moe_select)]),
            (a1 + 1, at(1, 0.2), upd_tasks(1)),
            (a1, a2 - 1, proj_tasks(2)),
            (a2 - 1, a2, read_tasks(2)),
            (a2 + 1, at(2, 0.2), upd_tasks(2)),
            (a2, a3 - 1, proj_tasks(3)),
            (a3 - 1, a3, read_tasks(3)),
            (a3 - 1, a3, [(1, lambda: (emit_downs(len(downs)), moe_finish()))]),
            (a3 + 1, last[1] + 1, out_tasks(0) + out_tasks(1) + out_tasks(2)),
            (last[3] + 2, last[2] + 1, out_tasks(3, (3,))),
            (last[2] + 2, last[1] + 1, out_tasks(3, (2,))),
            (last[1] + 2, nb + 1, out_tasks(3, (1,))),
        ]
        nf = FF // 128
        micro_ranges = [(a1 + 1, a2 - 1, moe_up_tasks(range(nf // 2))),
                        (a2, a3 - 2, moe_up_tasks(range(nf // 2, nf)))]
        downs = moe_down_tasks(range(nf))
        dstate = [0]

        def emit_downs(limit):
            n = 0
            while dstate[0] < len(downs) and n < limit and ("h", downs[dstate[0]][0]) in moe:
                downs[dstate[0]][1]()
                dstate[0] += 1
                n += 1

        ntiles = [sum(len(u) * (i + 1) for (_, u, i) in blk) for blk in blocks]

        def fence_w12():
            wait_w(1)
            wait_w(2)

        def fence_w34():
            wait_w(3)
            wait_w(4)
            x_copy(1).wait()

        def fence_a1():
            wait_moe(0)
            start_moe(1)

        def fence_a0():
            x_copy(2).wait()
            x_copy(3).wait()
            wo_copy.wait()
            start_moe(0)

        def fence_x0():
            for tt in range(1, 4):
                x_copy(0, tt).wait()
            beta_copy.wait()

        fences = {0: fence_x0, 2: fence_w12, 4: fence_w34, 6: fence_a0, a1: fence_a1,
                  a2: lambda: wait_moe(1)}

        state = [[0, 0.0, float(sum(c for c, _ in t))] for _, _, t in streams]
        mstate = [[0, 0] for _ in micro_ranges]

        for b in range(nb + 1):
            if b in fences:
                fences[b]()

            def micro(b=b):
                for (lo, hi, tasks), ms in zip(micro_ranges, mstate):
                    if lo <= b < hi:
                        ms[0] += 1
                        total = sum(ntiles[lo:hi])
                        while ms[1] < len(tasks) and ms[1] < ms[0] * len(tasks) / total:
                            tasks[ms[1]]()
                            ms[1] += 1

            if b < nb:
                scores(b, micro)
            for (lo, hi, tasks), st_ in zip(streams, state):
                if b < lo:
                    continue
                frac = (b + 1 - lo) / (hi - lo)
                while st_[0] < len(tasks) and st_[1] + tasks[st_[0]][0] / 2 <= frac * st_[2] + 1e-9:
                    cost, task = tasks[st_[0]]
                    task()
                    st_[1] += cost
                    st_[0] += 1
                    if cost >= 75 and a1 < b < a3:
                        emit_downs(5)
            if b > 0:
                values(b - 1)
        for (lo, hi, tasks), st_ in zip(streams, state):
            assert st_[0] == len(tasks), (lo, hi, st_)
        assert all(ms[1] == len(r[2]) for ms, r in zip(mstate, micro_ranges)) and dstate[0] == len(downs)
        for _, t in out_tasks(3, (0,)):
            t()

        def wait_outputs():
            for t in range(4 * NSEG):
                out_copy(t).wait()

        @pl.when(jnp.logical_not(guard["safe"]))
        def _():
            wait_outputs()
            compact_path()

        wait_outputs()

    def prep_group(g):
        for which in range(3):
            prep_wt(g, which)

    def wait_w(cb):
        for i in range(3):
            w_copy(i, cb).wait()

    def start_moe(c):
        for i in range(3):
            moe_copy(i, c).start()

    def wait_moe(c):
        for i in range(3):
            moe_copy(i, c).wait()

    def col_norm2(i, cb, part):
        n = 128 if cb < 4 else 64
        acc = None
        for u in range(3 * part, 3 * part + 3):
            wv = wraw[i, 64 * u:64 * (u + 1), 128 * cb:128 * cb + n].astype(F32)
            c = jnp.sum((wv * wv).reshape(8, 8, n), axis=0)
            acc = c if acc is None else acc + c
        return acc

    for s in range(NSEG):
        for g in range(NG):
            n = DH * GN[g]
            for tt in range(4):
                o_t[s, tt, 128 * g + n:128 * g + GW[g], :] = jnp.zeros((GW[g] - n, 128), BF)
    wr_copy.wait()
    x_copy(0, 0).wait()
    prep_wr()
    layernorm(0)
    wait_w(0)
    prep_group(0)
    proj_qkv(0, 0, 0, False, True)
    run_pipeline()


@jax.jit
def pallas_parallel_sum__memory_aug_infini_attn__moe_arch_mod__prompt_kernel(
    A_x: jax.Array,
    A_wq: jax.Array,
    A_wk: jax.Array,
    A_wv: jax.Array,
    A_wo: jax.Array,
    A_beta: jax.Array,
    B_x: jax.Array,
    B_w_r: jax.Array,
    B_w_gate: jax.Array,
    B_w_up: jax.Array,
    B_w_down: jax.Array,
):
    del B_x
    hbm = pl.BlockSpec(memory_space=pltpu.HBM)
    scratch = [
        pltpu.VMEM((D, SEQ), BF),
        pltpu.VMEM((4 * NSEG, D, 128), BF),
        pltpu.VMEM((16, SEQ), F32),
        pltpu.VMEM((4, D, D), BF),
        pltpu.VMEM((3 * GP, D), BF),
        pltpu.VMEM((D, GP), BF),
        pltpu.VMEM((H,), BF),
        pltpu.VMEM((D,), BF),
        pltpu.VMEM((16, D), BF),
        pltpu.VMEM((D, FF), BF),
        pltpu.VMEM((D, FF), BF),
        pltpu.VMEM((D, FF), BF),
        pltpu.VMEM((NSEG, 4, GP, 128), BF),
        pltpu.VMEM((NSEG, 4, GP, 128), BF),
        pltpu.VMEM((NSEG, 4, GP, 128), BF),
        pltpu.VMEM((NSEG, NG, L, 128), BF),
        pltpu.VMEM((NSEG, 4, GP, 128), BF),
        pltpu.VMEM((NSEG, 4, GP, 128), BF),
        pltpu.VMEM((2, 28, 128, 128), BF),
        pltpu.VMEM((NSEG, GP, L), F32),
        pltpu.VMEM((NSEG, 16 * NG, L), F32),
        pltpu.VMEM((NG, 128, 128), F32),
        pltpu.VMEM((1, SEQ), F32),
        pltpu.VMEM((NG, 8, 128), F32),
        pltpu.VMEM((4 * NSEG, D, 128), BF),
        pltpu.SemaphoreType.DMA((25,)),
        pltpu.SemaphoreType.DMA((3 * NMC,)),
        pltpu.SemaphoreType.DMA((4 * NSEG,)),
    ]
    out_t = pl.pallas_call(
        _kernel,
        out_shape=jax.ShapeDtypeStruct((1, D, SEQ), BF),
        in_specs=[hbm] * 10,
        out_specs=hbm,
        scratch_shapes=scratch,
        compiler_params=pltpu.CompilerParams(vmem_limit_bytes=100 * 1024 * 1024),
    )(jnp.swapaxes(A_x, 1, 2), A_wq, A_wk, A_wv, A_wo, A_beta, B_w_r, B_w_gate, B_w_up,
      B_w_down.T)
    return jnp.swapaxes(out_t, 1, 2)
```
